```python
import jax
import jax.numpy as jnp

def _softmax(x, axis=-1):
    return jax.nn.softmax(x, axis=axis)

def _gelu(x):
    return jax.nn.gelu(x, approximate=True)

def _silu(x):
    return jax.nn.silu(x)

def _sigmoid(x):
    return jax.nn.sigmoid(x)

def _layernorm(x, axis=-1, eps=1e-05):
    m = jnp.mean(x, axis=axis, keepdims=True)
    v = jnp.var(x, axis=axis, keepdims=True)
    return (x - m) / jnp.sqrt(v + eps)

def _scatter_add(tgt, idx, src, axis=0):
    return tgt.at[idx].add(src)

def _segment_sum(src, seg, n):
    return jax.ops.segment_sum(src, seg, n)

class _Rng:

    def __init__(self, key):
        self._k = key

    def _next(self):
        self._k, sub = jax.random.split(self._k)
        return sub

    def normal(self, shape):
        return jax.random.normal(self._next(), shape, dtype=jnp.bfloat16)

    def randint(self, lo, hi, shape):
        return jax.random.randint(self._next(), shape, lo, hi, dtype=jnp.int32)

    def uniform(self, shape, lo=0.0, hi=1.0):
        return jax.random.uniform(self._next(), shape, jnp.bfloat16, lo, hi)

    def permutation(self, n):
        return jax.random.permutation(self._next(), n)
kernel_name = 'adaLN_cond__gqa_block_cached__moe_arch_mod__prompt'

def setup_inputs():
    _rng = _Rng(jax.random.key(int.from_bytes(__import__("os").urandom(4), "little")))
    _w = lambda a: (lambda t: t.astype(jnp.bfloat16) if jnp.issubdtype(t.dtype, jnp.floating) else t)(jnp.asarray(a))

    def _A_setup():
        B, Sq, D = (1, 2048, 576)
        Hq, Hkv, Sk, Dh = (32, 16, 2048, 128)
        assert Hq % Hkv == 0, (Hq, Hkv)
        return {'x': _w((lambda *s: _rng.normal(s) * 0.05)(B, Sq, D)), 'k_cache': _w((lambda *s: _rng.normal(s) * 0.05)(B, Hkv, Sk, Dh)), 'v_cache': _w((lambda *s: _rng.normal(s) * 0.05)(B, Hkv, Sk, Dh)), 'wq': _w((lambda *s: _rng.normal(s) * 0.05)(D, Hq * Dh) * D ** (-0.5)), 'wo': _w((lambda *s: _rng.normal(s) * 0.05)(Hq * Dh, D) * (Hq * Dh) ** (-0.5))}
    _A_in = _A_setup()

    def _B_setup():
        B, S, D, F, C = (1, 2048, 576, 4608, 8)
        return {'x': _w((lambda *s: _rng.normal(s) * 0.05)(B, S, D)), 'w_r': _w((lambda *s: _rng.normal(s) * 0.05)(D)), 'w_gate': _w((lambda *s: _rng.normal(s) * 0.05)(D, F)), 'w_up': _w((lambda *s: _rng.normal(s) * 0.05)(D, F)), 'w_down': _w((lambda *s: _rng.normal(s) * 0.05)(F, D))}
    _B_in = _B_setup()
    return {'A_x': _A_in['x'], 'A_k_cache': _A_in['k_cache'], 'A_v_cache': _A_in['v_cache'], 'A_wq': _A_in['wq'], 'A_wo': _A_in['wo'], 'B_x': _B_in['x'], 'B_w_r': _B_in['w_r'], 'B_w_gate': _B_in['w_gate'], 'B_w_up': _B_in['w_up'], 'B_w_down': _B_in['w_down'], 'c': _w((lambda *s: _rng.normal(s) * 0.05)(1, 576)), 'w_mod': _w((lambda *s: _rng.normal(s) * 0.05)(576, 6 * 576) * 576 ** (-0.5))}

def reference(A_x, A_k_cache, A_v_cache, A_wq, A_wo, B_x, B_w_r, B_w_gate, B_w_up, B_w_down, c, w_mod):

    def _A_ref(x, k_cache, v_cache, wq, wo):
        B, Sq, D = x.shape
        Hq, Dh = (32, 128)
        Hkv = k_cache.shape[1]
        rep = Hq // Hkv
        q = (lambda x, *d: x.transpose(*d))((x @ wq).reshape(B, Sq, Hq, Dh), 0, 2, 1, 3)
        k = jnp.repeat(k_cache, rep, axis=1)
        v = jnp.repeat(v_cache, rep, axis=1)
        scores = jnp.einsum('bhqd,bhkd->bhqk', q, k) * Dh ** (-0.5)
        p = _softmax(scores, axis=-1)
        o = jnp.einsum('bhqk,bhkd->bhqd', p, v)
        return (lambda x, *d: x.transpose(*d))(o, 0, 2, 1, 3).reshape(B, Sq, Hq * Dh) @ wo

    def _B_ref(x, w_r, w_gate, w_up, w_down):
        B, S, D = x.shape
        C = 8
        r = x @ w_r
        idx = jnp.argsort(-r, axis=-1)[:, :C]
        idx_e = jnp.repeat(idx.reshape(B, C, 1), D, axis=2)
        x_sel = jnp.take_along_axis(x, idx_e, axis=1)
        g = _silu(x_sel @ w_gate)
        u = x_sel @ w_up
        y = g * u @ w_down
        r_sel = _sigmoid(jnp.take_along_axis(r, idx, axis=1))
        y = y * r_sel.reshape(B, C, 1)
        b_off = (jnp.arange(B) * S).reshape(B, 1)
        flat_idx = (idx + b_off).reshape(B * C)
        zero = (x * 0.0).reshape(B * S, D)
        upd = _scatter_add(zero, flat_idx, y.reshape(B * C, D), axis=0)
        return x + upd.reshape(B, S, D)
    x = A_x
    mod = (_silu(c) @ w_mod).reshape(c.shape[0], 6, 1, -1)
    sa, ca, ga, sb, cb, gb = (mod[:, 0].copy(), mod[:, 1].copy(), mod[:, 2].copy(), mod[:, 3].copy(), mod[:, 4].copy(), mod[:, 5].copy())
    h = _layernorm(x, axis=-1) * (1 + ca) + sa
    x = x + ga * _A_ref(h, A_k_cache, A_v_cache, A_wq, A_wo)
    h = _layernorm(x, axis=-1) * (1 + cb) + sb
    x = x + gb * _B_ref(h, B_w_r, B_w_gate, B_w_up, B_w_down)
    return x
```

```python
import functools

import jax
import jax.numpy as jnp
from jax import lax
import jax.experimental.pallas as pl
import jax.experimental.pallas.tpu as pltpu

BF = jnp.bfloat16
F32 = jnp.float32
NT = (((1,), (1,)), ((), ()))
LOG2E = 1.4426950408889634
EPS = 1e-5
TOPC = 8
LANES = 128


def _build(S, SK, D, HKV, DH, F, T, CK, flags, opts):
    REP = 2
    R = REP * T
    NB = S // T
    TPB = T // LANES
    NTILE = S // LANES
    NC = SK // CK
    HD = REP * DH
    assert HKV % 2 == 0 and T % LANES == 0 and NC >= 2
    qscale = (DH ** -0.5) * LOG2E
    round_x2 = opts.get('round_x2', True)

    def kernel(xT_hbm, k_hbm, v_hbm, wq_hbm, woT_hbm, wr_ref, wg_hbm, wu_hbm, wdT_hbm, c_ref, wm_hbm,
               outT_hbm,
               xT_v, k_v, v_v, wq_v, woT_v, wg_v, wu_v, wdT_v, wm_v,
               modr_s, colf_s, wr_s, h_s, s_s0, s_s1, m_s0, m_s1, acc_s, out0_s, h2_s, r_s, outT_v,
               sem_head, sem_misc, sem_out):
        s_s = (s_s0, s_s1)
        m_s = (m_s0, m_s1)

        def cp_wq(g):
            return pltpu.make_async_copy(wq_hbm.at[:, pl.ds(g * HD, HD)], wq_v.at[g], sem_head.at[g, 0])

        def cp_k(g):
            return pltpu.make_async_copy(k_hbm.at[g], k_v.at[g], sem_head.at[g, 1])

        def cp_v(g):
            return pltpu.make_async_copy(v_hbm.at[g], v_v.at[g], sem_head.at[g, 2])

        def cp_wo(g):
            return pltpu.make_async_copy(woT_hbm.at[:, pl.ds(g * HD, HD)], woT_v.at[g], sem_head.at[g, 3])

        def head_copies(g):
            return (cp_wq(g), cp_k(g), cp_v(g), cp_wo(g))

        cp_wm1 = pltpu.make_async_copy(wm_hbm.at[:, pl.ds(0, 2 * D)], wm_v.at[:, pl.ds(0, 2 * D)], sem_misc.at[0])
        cp_wm2 = pltpu.make_async_copy(wm_hbm.at[:, pl.ds(2 * D, 4 * D)], wm_v.at[:, pl.ds(2 * D, 4 * D)],
                                       sem_misc.at[1])
        cp_x0 = pltpu.make_async_copy(xT_hbm.at[:, pl.ds(0, T)], xT_v.at[:, pl.ds(0, T)], sem_misc.at[2])
        cp_x1 = pltpu.make_async_copy(xT_hbm.at[:, pl.ds(T, S - T)], xT_v.at[:, pl.ds(T, S - T)], sem_misc.at[3])
        cp_wg = pltpu.make_async_copy(wg_hbm, wg_v, sem_misc.at[4])
        cp_wu = pltpu.make_async_copy(wu_hbm, wu_v, sem_misc.at[5])
        cp_wd = pltpu.make_async_copy(wdT_hbm, wdT_v, sem_misc.at[6])

        cp_wm1.start()
        cp_x0.start()
        cp_wq(0).start()
        cp_k(0).start()
        cp_v(0).start()
        cp_wo(0).start()
        cp_wq(1).start()
        cp_k(1).start()
        cp_x1.start()
        cp_v(1).start()
        cp_wo(1).start()
        for g0 in (2, 3):
            for cp in head_copies(g0):
                cp.start()

        acc_s[...] = jnp.zeros(acc_s.shape, F32)

        cc = jnp.broadcast_to(c_ref[...].astype(F32), (8, D))
        sc = (cc * jax.nn.sigmoid(cc)).astype(BF)
        wr_s[...] = jnp.broadcast_to(wr_ref[...].reshape(1, D), (16, D))
        cp_wm1.wait()
        mod1 = jnp.dot(sc, wm_v[:, pl.ds(0, 2 * D)], preferred_element_type=F32)
        modr_s[0] = mod1[:, 0:D]
        modr_s[1] = mod1[:, D:2 * D] + 1.0

        def ln1_tile(tile_src, row_dst):
            col = pl.multiple_of(tile_src * LANES, LANES)
            xs = xT_v[:, pl.ds(col, LANES)].astype(F32)
            mu = jnp.mean(xs, axis=0, keepdims=True)
            xc = xs - mu
            var = jnp.mean(xc * xc, axis=0, keepdims=True)
            hn = (xc * lax.rsqrt(var + EPS)).T
            hh = hn * modr_s[1, 0:1, :] + modr_s[0, 0:1, :]
            h_s[pl.ds(pl.multiple_of(row_dst, LANES), LANES), :] = hh.astype(BF)

        def ln2_tile(tile):
            col = pl.multiple_of(tile * LANES, LANES)
            slot = (tile // TPB) % 2
            acol = pl.multiple_of((tile % TPB) * LANES, LANES)
            xs = xT_v[:, pl.ds(col, LANES)].astype(F32)
            av = acc_s[slot, :, pl.ds(acol, LANES)]
            acc_s[slot, :, pl.ds(acol, LANES)] = jnp.zeros((D, LANES), F32)
            x2 = xs + colf_s[0] * av
            if round_x2:
                x2 = x2.astype(BF).astype(F32)
            mu = jnp.mean(x2, axis=0, keepdims=True)
            xc = x2 - mu
            var = jnp.mean(xc * xc, axis=0, keepdims=True)
            h2 = (xc * lax.rsqrt(var + EPS) * colf_s[2] + colf_s[1]).astype(BF)
            h2_s[:, pl.ds(col, LANES)] = h2
            out0_s[:, pl.ds(col, LANES)] = x2 + colf_s[3] * h2.astype(F32)
            rr = jnp.dot(wr_s[...], h2, preferred_element_type=F32)
            r_s[tile] = rr[0:8, :]

        def step(ta, ga, tb, gb, slot_a, do_a=True, do_b=True, extra=None):
            slot_b = 1 - slot_a
            extra = extra or {}
            if do_a:
                hrow = pl.multiple_of((ta % 2) * T, T)
                hh = h_s[pl.ds(hrow, T), :]
                qf = jnp.dot(hh, wq_v[ga], preferred_element_type=F32) * qscale
                qb = qf.astype(BF)
                q2 = jnp.concatenate([qb[:, r * DH:(r + 1) * DH] for r in range(REP)], axis=0)
                mrun = None
            if do_b:
                mrow = jnp.max(m_s[slot_b][...], axis=-1, keepdims=True)
                lrun = None
                oacc = None
            for c in range(NC):
                if do_b:
                    sv = s_s[slot_b][:, pl.ds(c * CK, CK)]
                    p = jnp.exp2(sv - mrow)
                    ll = p[:, 0:LANES]
                    for jj in range(1, CK // LANES):
                        ll = ll + p[:, jj * LANES:(jj + 1) * LANES]
                    lrun = ll if lrun is None else lrun + ll
                    o = jnp.dot(p.astype(BF), v_v[gb, pl.ds(c * CK, CK), :], preferred_element_type=F32)
                    oacc = o if oacc is None else oacc + o
                if do_a:
                    s = lax.dot_general(q2, k_v[ga, pl.ds(c * CK, CK), :], NT, preferred_element_type=F32)
                    s_s[slot_a][:, pl.ds(c * CK, CK)] = s
                    mm = s[:, 0:LANES]
                    for jj in range(1, CK // LANES):
                        mm = jnp.maximum(mm, s[:, jj * LANES:(jj + 1) * LANES])
                    mrun = mm if mrun is None else jnp.maximum(mrun, mm)
                if c in extra:
                    extra[c]()
            if do_b:
                lsum = jnp.sum(lrun, axis=-1, keepdims=True)
                ob = (oacc * pltpu.reciprocal(lsum, approx=False, full_range=False)).astype(BF)
                o2 = jnp.concatenate([ob[r * T:(r + 1) * T, :] for r in range(REP)], axis=1)
                y = lax.dot_general(woT_v[gb], o2, NT, preferred_element_type=F32)
                acc_s[tb % 2] = acc_s[tb % 2] + y
            if do_a:
                m_s[slot_a][...] = mrun

        cp_x0.wait()

        def ln1_first(i, carry):
            ln1_tile(i, i * LANES)
            return carry
        lax.fori_loop(0, TPB, ln1_first, 0)

        def ln1_next(t):
            tn = jnp.minimum(t + 1, NB - 1)
            return {
                2 * i * (NC // (2 * TPB)): functools.partial(
                    ln1_tile, tn * TPB + i, ((t + 1) % 2) * T + i * LANES)
                for i in range(TPB)}

        def ln2_prev(t):
            return {
                2 * i * (NC // (2 * TPB)): functools.partial(ln2_tile, (t - 1) * TPB + i)
                for i in range(TPB)}

        def block(t, carry):
            @pl.when(t == 0)
            def _():
                cp_wq(0).wait()
                cp_k(0).wait()
                step(0, 0, None, None, 0, do_b=False)
                cp_v(0).wait()
                cp_wo(0).wait()
                cp_wq(1).wait()
                cp_k(1).wait()
                cp_x1.wait()
                step(0, 1, 0, 0, 1, extra=ln1_next(0))

            @pl.when(t > 0)
            def _():
                step(t, 0, t - 1, HKV - 1, 0, extra=ln1_next(t))
                step(t, 1, t, 0, 1, extra=ln2_prev(t))

            def pair(b, carry2):
                g = 2 * b + 2

                @pl.when(t == 0)
                def _():
                    cp_v(g - 1).wait()
                    cp_wo(g - 1).wait()
                    for cp in head_copies(g):
                        cp.wait()
                    cp_wq(g + 1).wait()
                    cp_k(g + 1).wait()

                    @pl.when(g + 2 < HKV)
                    def _():
                        for cp in head_copies(g + 2) + head_copies(g + 3):
                            cp.start()

                    @pl.when(g + 2 == HKV)
                    def _():
                        cp_v(HKV - 1).wait()
                        cp_wo(HKV - 1).wait()
                        cp_wm2.start()
                        cp_wg.start()
                        cp_wu.start()
                        cp_wd.start()

                step(t, g, t, g - 1, 0)
                step(t, g + 1, t, g, 1)
                return carry2

            lax.fori_loop(0, HKV // 2 - 1, pair, 0)

            @pl.when(t == 0)
            def _():
                cp_wm2.wait()
                mod2 = jnp.dot(sc, wm_v[:, pl.ds(2 * D, 4 * D)], preferred_element_type=F32)
                for i in range(4):
                    row = mod2[0:1, i * D:(i + 1) * D]
                    if i == 2:
                        row = row + 1.0
                    colf_s[i] = jnp.broadcast_to(row, (LANES, D)).T
            return carry

        lax.fori_loop(0, NB, block, 0)
        step(None, None, NB - 1, HKV - 1, 1 - 1, do_a=False)

        def ln2_tail(i, carry):
            ln2_tile((NB - 1) * TPB + i)
            return carry
        lax.fori_loop(0, TPB, ln2_tail, 0)

        lane = lax.broadcasted_iota(jnp.int32, (8, LANES), 1)
        sub = lax.broadcasted_iota(jnp.int32, (8, LANES), 0)
        keys = []
        for tl in range(NTILE):
            rv = r_s[tl]
            tok = lane + tl * LANES
            code = jnp.where(rv < 0.0, tok, (S - 1) - tok)
            mag = jnp.maximum(jnp.abs(rv), 1.1754944e-38)
            bits = lax.bitcast_convert_type(mag, jnp.int32)
            bits = (bits & jnp.int32(-S)) | code
            kf = lax.bitcast_convert_type(bits, F32)
            keys.append(jnp.where(rv < 0.0, -kf, kf))
        keys0 = list(keys)
        msel = jnp.zeros((8, LANES), F32)
        for i in range(TOPC):
            mm = keys[0]
            tree = list(keys)
            while len(tree) > 1:
                tree = [jnp.maximum(tree[2 * a], tree[2 * a + 1]) for a in range(len(tree) // 2)] + \
                    ([tree[-1]] if len(tree) % 2 else [])
            mx = jnp.max(tree[0], axis=1, keepdims=True)
            msel = jnp.where(sub == i, mx, msel)
            if i + 1 < TOPC:
                keys = [jnp.where(kk == mx, -jnp.inf, kk) for kk in keys]
        oht = jnp.concatenate([jnp.where(kk == msel, 1.0, 0.0) for kk in keys0], axis=1).astype(BF)
        rsel = lax.bitcast_convert_type(
            lax.bitcast_convert_type(msel[:, 0:1], jnp.int32) & jnp.int32(-S), F32)

        xsel = lax.dot_general(oht, h2_s[...], NT, preferred_element_type=F32).astype(BF)
        cp_wg.wait()
        cp_wu.wait()
        cp_wd.wait()
        gg = jnp.dot(xsel, wg_v[...], preferred_element_type=F32)
        uu = jnp.dot(xsel, wu_v[...], preferred_element_type=F32)
        act = (gg * jax.nn.sigmoid(gg) * uu).astype(BF)
        yy = lax.dot_general(act, wdT_v[...], NT, preferred_element_type=F32)
        yy = yy * jax.nn.sigmoid(rsel)
        yT = yy.T.astype(BF)

        def out_copy(i):
            cs = pl.ds(i * T, T)
            return pltpu.make_async_copy(outT_v.at[:, cs], outT_hbm.at[:, cs], sem_out.at[i])

        for i in range(NB):
            cs = pl.ds(i * T, T)
            upd = jnp.dot(yT, oht[:, i * T:(i + 1) * T], preferred_element_type=F32)
            gbc = jnp.concatenate([colf_s[3]] * TPB, axis=1)
            outT_v[:, cs] = (out0_s[:, cs] + gbc * upd).astype(BF)
            out_copy(i).start()
        for i in range(NB):
            out_copy(i).wait()

    scratch = [
        pltpu.VMEM((D, S), BF),
        pltpu.VMEM((HKV, SK, DH), BF),
        pltpu.VMEM((HKV, SK, DH), BF),
        pltpu.VMEM((HKV, D, HD), BF),
        pltpu.VMEM((HKV, D, HD), BF),
        pltpu.VMEM((D, F), BF),
        pltpu.VMEM((D, F), BF),
        pltpu.VMEM((D, F), BF),
        pltpu.VMEM((D, 6 * D), BF),
        pltpu.VMEM((2, 8, D), F32),
        pltpu.VMEM((4, D, LANES), F32),
        pltpu.VMEM((16, D), BF),
        pltpu.VMEM((2 * T, D), BF),
        pltpu.VMEM((R, SK), F32),
        pltpu.VMEM((R, SK), F32),
        pltpu.VMEM((R, LANES), F32),
        pltpu.VMEM((R, LANES), F32),
        pltpu.VMEM((2, D, T), F32),
        pltpu.VMEM((D, S), F32),
        pltpu.VMEM((D, S), BF),
        pltpu.VMEM((NTILE, 8, LANES), F32),
        pltpu.VMEM((D, S), BF),
        pltpu.SemaphoreType.DMA((HKV, 4)),
        pltpu.SemaphoreType.DMA((8,)),
        pltpu.SemaphoreType.DMA((NB,)),
    ]
    anyspec = pl.BlockSpec(memory_space=pl.ANY)
    vm = pl.BlockSpec(memory_space=pltpu.VMEM)
    return pl.pallas_call(
        kernel,
        in_specs=[anyspec, anyspec, anyspec, anyspec, anyspec, vm, anyspec, anyspec, anyspec, vm, anyspec],
        out_specs=anyspec,
        out_shape=jax.ShapeDtypeStruct((D, S), BF),
        scratch_shapes=scratch,
        compiler_params=pltpu.CompilerParams(vmem_limit_bytes=opts.get('vmem', 110) * 1024 * 1024, flags=flags),
        name='adaln_gqa_moe',
        interpret=opts.get('interpret', False),
    )


def build_fn(T=256, CK=512, flags=None, **opts):
    def fn(A_x, A_k_cache, A_v_cache, A_wq, A_wo, B_x, B_w_r, B_w_gate, B_w_up, B_w_down, c, w_mod):
        B, S, D = A_x.shape
        _, HKV, SK, DH = A_k_cache.shape
        F = B_w_gate.shape[1]
        call = _build(S, SK, D, HKV, DH, F, T, CK, flags, opts)
        outT = call(
            A_x.reshape(S, D).T, A_k_cache.reshape(HKV, SK, DH), A_v_cache.reshape(HKV, SK, DH),
            A_wq, A_wo.T, B_w_r, B_w_gate, B_w_up, B_w_down.T, c, w_mod)
        return outT.T.reshape(B, S, D)
    return fn


_IMPL = build_fn(flags={"XLA_TPU_FORCE_LP_LLO_SCHEDULER": True})


@jax.jit
def pallas_adaLN_cond__gqa_block_cached__moe_arch_mod__prompt_kernel(
        A_x, A_k_cache, A_v_cache, A_wq, A_wo, B_x, B_w_r, B_w_gate, B_w_up, B_w_down, c, w_mod):
    return _IMPL(A_x, A_k_cache, A_v_cache, A_wq, A_wo, B_x, B_w_r, B_w_gate, B_w_up, B_w_down, c, w_mod)
```

```python
import functools

import jax
import jax.numpy as jnp
from jax import lax
import jax.experimental.pallas as pl
import jax.experimental.pallas.tpu as pltpu

BF = jnp.bfloat16
F32 = jnp.float32
NT = (((1,), (1,)), ((), ()))
LOG2E = 1.4426950408889634
EPS = 1e-5
TOPC = 8
LANES = 128


def _build(S, SK, D, HKV, DH, F, T, CK, flags, opts):
    REP = 2
    R = REP * T
    NB = S // T
    TPB = T // LANES
    NTILE = S // LANES
    NC = SK // CK
    HD = REP * DH
    assert HKV % 2 == 0 and T % LANES == 0 and NC >= 2
    qscale = (DH ** -0.5) * LOG2E
    round_x2 = opts.get('round_x2', True)
    ANCH = opts.get('anch', 1)
    PH = opts.get('ph', [1, 1, 1, 1, 1, 1, 1, 0])
    assert TPB == 2 and NC == 4

    def kernel(xT_hbm, k_hbm, v_hbm, wq_hbm, woT_hbm, wr_ref, wg_hbm, wu_hbm, wdT_hbm, c_ref, wm_hbm,
               outT_hbm,
               xT_v, k_v, v_v, wq_v, woT_v, wg_v, wu_v, wdT_v, wm_v,
               modr_s, colf_s, wr_s, h_s, s_s0, s_s1, m_s0, m_s1, o_s0, o_s1, acc_s, zero_s, out0_s, h2_s, r_s, outT_v,
               sem_head, sem_misc, sem_out):
        s_s = (s_s0, s_s1)
        m_s = (m_s0, m_s1)
        o_s = (o_s0, o_s1)

        def cp_wq(g):
            return pltpu.make_async_copy(wq_hbm.at[:, pl.ds(g * HD, HD)], wq_v.at[g], sem_head.at[g, 0])

        def cp_k(g):
            return pltpu.make_async_copy(k_hbm.at[g], k_v.at[g], sem_head.at[g, 1])

        def cp_v(g):
            return pltpu.make_async_copy(v_hbm.at[g], v_v.at[g], sem_head.at[g, 2])

        def cp_wo(g):
            return pltpu.make_async_copy(woT_hbm.at[:, pl.ds(g * HD, HD)], woT_v.at[g], sem_head.at[g, 3])

        def cols(src, dst, lo, n, sem):
            return pltpu.make_async_copy(src.at[:, pl.ds(lo, n)], dst.at[:, pl.ds(lo, n)], sem)

        cp_wm1 = cols(wm_hbm, wm_v, 0, 2 * D, sem_misc.at[0])
        cp_wm2 = cols(wm_hbm, wm_v, 2 * D, 4 * D, sem_misc.at[1])
        cp_x0 = cols(xT_hbm, xT_v, 0, T, sem_misc.at[2])
        cp_x1 = cols(xT_hbm, xT_v, T, T, sem_misc.at[3])
        cp_x2 = cols(xT_hbm, xT_v, 2 * T, S - 2 * T, sem_misc.at[4])
        cp_wg = pltpu.make_async_copy(wg_hbm, wg_v, sem_misc.at[5])
        cp_wu = pltpu.make_async_copy(wu_hbm, wu_v, sem_misc.at[6])
        cp_wd = pltpu.make_async_copy(wdT_hbm, wdT_v, sem_misc.at[7])

        cp_wm1.start()
        cp_x0.start()
        for g0 in range(HKV + 2):
            if g0 < HKV:
                cp_wq(g0).start()
                cp_k(g0).start()
            if 0 <= g0 - 1 < HKV:
                cp_v(g0 - 1).start()
            if g0 == 1:
                cp_x1.start()
            if 0 <= g0 - 2 < HKV:
                cp_wo(g0 - 2).start()
        LATE = opts.get('late', 0)

        zero_s[0] = 0
        acc_s[0:2] = jnp.zeros((2, D, T), F32)
        colf_s[0:4] = jnp.zeros((4, D, LANES), F32)

        cc = jnp.broadcast_to(c_ref[...].astype(F32), (8, D))
        sc = (cc * jax.nn.sigmoid(cc)).astype(BF)
        wr_s[...] = jnp.broadcast_to(wr_ref[...].reshape(1, D), (16, D))
        cp_wm1.wait()
        mod1 = jnp.dot(sc, wm_v[:, pl.ds(0, 2 * D)], preferred_element_type=F32)
        modr_s[0] = mod1[:, 0:D]
        modr_s[1] = mod1[:, D:2 * D] + 1.0

        FC = opts.get('fc', 48)
        assert D % FC == 0 and FC % 16 == 0

        def fold(a):
            n = a.shape[0]
            while n > 8:
                if n % 16 == 0:
                    n //= 2
                    a = a[0:n] + a[n:2 * n]
                else:
                    r = a[0:8]
                    for i in range(1, n // 8):
                        r = r + a[8 * i:8 * i + 8]
                    a, n = r, 8
            return a

        def total(a):
            return jnp.sum(a, axis=0, keepdims=True) * (1.0 / D)

        def x_rows(lo, n, tile):
            col = pl.ds(pl.multiple_of(tile * LANES, LANES), LANES)
            return xT_v[pl.ds(lo, n), col].astype(F32)

        def stat_pieces(load_a, load_b, st):
            def sum_piece(lo):
                def run():
                    part = fold(load_a(lo, FC))
                    st['s'] = part if lo == 0 else st['s'] + part
                    if lo + FC == D:
                        st['mu'] = total(st['s'])
                return run

            def var_piece(lo):
                def run():
                    xc = load_b(lo, FC) - st['mu']
                    part = fold(xc * xc)
                    st['q'] = part if lo == 0 else st['q'] + part
                    if lo + FC == D:
                        st['rstd'] = lax.rsqrt(total(st['q']) + EPS)
                return run
            return [sum_piece(lo) for lo in range(0, D, FC)] + [var_piece(lo) for lo in range(0, D, FC)]

        def ln1_pieces(tile, row_dst):
            st = {}
            row = pl.ds(pl.multiple_of(row_dst, LANES), LANES)
            ld = lambda lo, n: x_rows(lo, n, tile)

            def apply_piece(lo):
                def run():
                    n = min(LANES, D - lo)
                    hn = ((ld(lo, n) - st['mu']) * st['rstd']).T
                    hh = hn * modr_s[1, 0:1, pl.ds(lo, n)] + modr_s[0, 0:1, pl.ds(lo, n)]
                    h_s[row, pl.ds(lo, n)] = hh.astype(BF)
                return run
            return stat_pieces(ld, ld, st) + [apply_piece(lo) for lo in range(0, D, LANES)]

        def ln2_pieces(tile, xs):
            st = {}
            col = pl.ds(pl.multiple_of(tile * LANES, LANES), LANES)
            slot = (tile // TPB) % 2
            acol = pl.ds(pl.multiple_of((tile % TPB) * LANES, LANES), LANES)

            def load_a(lo, n):
                rows = pl.ds(lo, n)
                x2 = x_rows(lo, n, tile) + colf_s[0, rows, :] * acc_s[slot, rows, acol]
                acc_s[slot, rows, acol] = jnp.zeros((n, LANES), F32)
                if round_x2:
                    x2 = x2.astype(BF).astype(F32)
                colf_s[5 + xs, rows, :] = x2
                return x2

            def apply_piece(lo):
                def run():
                    rows = pl.ds(lo, FC)
                    x2 = colf_s[5 + xs, rows, :]
                    h2 = ((x2 - st['mu']) * st['rstd'] * colf_s[2, rows, :] + colf_s[1, rows, :]).astype(BF)
                    h2_s[rows, col] = h2
                    out0_s[rows, col] = x2 + colf_s[3, rows, :] * h2.astype(F32)
                return run
            return (stat_pieces(load_a, lambda lo, n: colf_s[5 + xs, pl.ds(lo, n), :], st)
                    + [apply_piece(lo) for lo in range(0, D, FC)])

        def interleave(a, b):
            return [f for pair_ in zip(a, b) for f in pair_]

        def run_all(pieces):
            for f in pieces:
                f()

        def anchor(v, z):
            xT_v[0:16, pl.ds(pl.multiple_of(S + z * LANES, LANES), LANES)] = v.astype(BF)
            colf_s[4 + z, 0:8, :] = v[0:8]
            if ANCH > 1:
                acc_s[2 + z, 0:8, 0:LANES] = v[0:8]

        def r_tile(tile):
            col = pl.multiple_of(tile * LANES, LANES)
            rr = jnp.dot(wr_s[...], h2_s[:, pl.ds(col, LANES)], preferred_element_type=F32)
            r_s[tile] = rr[0:8, :]

        def step(ua, up, uo, par, extra=None, pieces=None):
            extra = extra or {}
            pieces = list(pieces or [])
            phases = [ph for ph in range(2 * NC) if PH[ph]]

            def place(v, ph):
                if not pieces or ph not in phases:
                    return
                left = len([q for q in phases if q >= ph])
                npc = -(-len(pieces) // left)
                mine = [pieces.pop(0) for _ in range(npc)]
                for i, f in enumerate(mine):
                    r0 = ((i * R // len(mine)) // 16) * 16
                    anchor(v[r0:r0 + 16, 0:LANES], zero_s[0])
                    f()

            if ua is not None:
                ta, ga = ua
                hrow = pl.multiple_of((ta % 2) * T, T)
                qf = jnp.dot(h_s[pl.ds(hrow, T), :], wq_v[ga], preferred_element_type=F32) * qscale
                qb = qf.astype(BF)
                q2 = jnp.concatenate([qb[:, r * DH:(r + 1) * DH] for r in range(REP)], axis=0)
                mrun = None
            if uo is not None:
                to, go = uo
                y = lax.dot_general(woT_v[go], o_s[par][...], NT, preferred_element_type=F32)
                acc_s[to % 2] = acc_s[to % 2] + y
            if up is not None:
                tp, gp = up
                mrow = jnp.max(m_s[1 - par][...], axis=-1, keepdims=True)
                lrun = None
                oacc = None
            for c in range(NC):
                if up is not None:
                    sv = s_s[1 - par][:, pl.ds(c * CK, CK)]
                    p = jnp.exp2(sv - mrow)
                    ll = p[:, 0:LANES]
                    for jj in range(1, CK // LANES):
                        ll = ll + p[:, jj * LANES:(jj + 1) * LANES]
                    lrun = ll if lrun is None else lrun + ll
                    o = jnp.dot(p.astype(BF), v_v[gp, pl.ds(c * CK, CK), :], preferred_element_type=F32)
                    oacc = o if oacc is None else oacc + o
                    place(o, 2 * c)
                if ua is not None:
                    s = lax.dot_general(q2, k_v[ga, pl.ds(c * CK, CK), :], NT, preferred_element_type=F32)
                    s_s[par][:, pl.ds(c * CK, CK)] = s
                    mm = s[:, 0:LANES]
                    for jj in range(1, CK // LANES):
                        mm = jnp.maximum(mm, s[:, jj * LANES:(jj + 1) * LANES])
                    mrun = mm if mrun is None else jnp.maximum(mrun, mm)
                    place(s, 2 * c + 1)
            if up is not None:
                lsum = jnp.sum(lrun, axis=-1, keepdims=True)
                ob = (oacc * pltpu.reciprocal(lsum, approx=False, full_range=False)).astype(BF)
                for r in range(REP):
                    o_s[1 - par][:, r * DH:(r + 1) * DH] = ob[r * T:(r + 1) * T, :]
            if ua is not None:
                m_s[par][...] = mrun
            if NC in extra:
                extra[NC]()

        cp_x0.wait()

        def ln1_first(i, carry):
            run_all(ln1_pieces(i, i * LANES))
            return carry
        lax.fori_loop(0, TPB, ln1_first, 0)
        if LATE < 2:
            cp_x2.start()
            cp_wm2.start()
        if LATE < 1:
            cp_wg.start()
            cp_wu.start()
            cp_wd.start()

        cp_wq(0).wait()
        cp_k(0).wait()
        step((0, 0), None, None, 0)
        cp_wq(1).wait()
        cp_k(1).wait()
        cp_v(0).wait()
        cp_x1.wait()
        step((0, 1), (0, 0), None, 1)

        def wait_pair(first, g):
            def run(i, carry):
                @pl.when(g < HKV)
                def _():
                    cp_wq(g).wait()
                    cp_k(g).wait()
                    cp_wq(g + 1).wait()
                    cp_k(g + 1).wait()
                    cp_v(g).wait()
                cp_v(g - 1).wait()
                cp_wo(g - 2).wait()
                cp_wo(g - 1).wait()
                return carry
            if not opts.get('nowait'):
                lax.fori_loop(0, first, run, 0)

        def unit(t, g):
            return (t + g // HKV, g % HKV)

        def spread(fns):
            stride = max(NC // len(fns), 1)
            return {i * stride: f for i, f in enumerate(fns)}

        def block(t, carry):
            first = (t == 0).astype(jnp.int32)
            tn = jnp.minimum(t + 1, NB - 1)
            tp = jnp.maximum(t - 1, 0)
            wait_pair(first, 2)
            a0, a1 = tn * TPB, tn * TPB + 1
            r0 = ((t + 1) % 2) * T
            b0, b1 = tp * TPB, tp * TPB + 1
            step((t, 2), (t, 1), (t, 0), 0, pieces=interleave(ln1_pieces(a0, r0), ln1_pieces(a1, r0 + LANES)))
            step((t, 3), (t, 2), (t, 1), 1, pieces=interleave(ln2_pieces(b0, 0), ln2_pieces(b1, 1)),
                 extra={NC: lambda: (r_tile(b0), r_tile(b1))})

            def pair(b, carry2):
                g = 2 * b + 4
                wait_pair(first, g)
                step(unit(t, g), unit(t, g - 1), unit(t, g - 2), 0)
                step(unit(t, g + 1), unit(t, g), unit(t, g - 1), 1)
                return carry2

            lax.fori_loop(0, HKV // 2 - 1 - (t == NB - 1).astype(jnp.int32), pair, 0)

            def mod_rest(i, carry2):
                if LATE >= 2:
                    cp_x2.start()
                    cp_wm2.start()
                if LATE >= 1:
                    cp_wg.start()
                    cp_wu.start()
                    cp_wd.start()
                cp_x2.wait()
                cp_wm2.wait()
                mod2 = jnp.dot(sc, wm_v[:, pl.ds(2 * D, 4 * D)], preferred_element_type=F32)
                for k2 in range(4):
                    row = mod2[0:1, k2 * D:(k2 + 1) * D]
                    if k2 == 2:
                        row = row + 1.0
                    colf_s[k2] = jnp.broadcast_to(row, (LANES, D)).T
                return carry2
            lax.fori_loop(0, first, mod_rest, 0)
            return carry

        lax.fori_loop(0, NB, block, 0)
        step(None, (NB - 1, HKV - 1), (NB - 1, HKV - 2), 0)
        step(None, None, (NB - 1, HKV - 1), 1)
        if opts.get('nowait'):
            for g0 in range(2, HKV):
                cp_wq(g0).wait()
                cp_k(g0).wait()
            for g0 in range(1, HKV):
                cp_v(g0).wait()
            for g0 in range(0, HKV):
                cp_wo(g0).wait()

        def ln2_tail(i, carry):
            run_all(ln2_pieces((NB - 1) * TPB + i, 0))
            r_tile((NB - 1) * TPB + i)
            return carry
        lax.fori_loop(0, TPB, ln2_tail, 0)

        lane = lax.broadcasted_iota(jnp.int32, (8, LANES), 1)
        sub = lax.broadcasted_iota(jnp.int32, (8, LANES), 0)
        keys = []
        for tl in range(NTILE):
            rv = r_s[tl]
            tok = lane + tl * LANES
            code = jnp.where(rv < 0.0, tok, (S - 1) - tok)
            mag = jnp.maximum(jnp.abs(rv), 1.1754944e-38)
            bits = lax.bitcast_convert_type(mag, jnp.int32)
            bits = (bits & jnp.int32(-S)) | code
            kf = lax.bitcast_convert_type(bits, F32)
            keys.append(jnp.where(rv < 0.0, -kf, kf))
        keys0 = list(keys)
        msel = jnp.zeros((8, LANES), F32)
        for i in range(TOPC):
            mm = keys[0]
            tree = list(keys)
            while len(tree) > 1:
                tree = [jnp.maximum(tree[2 * a], tree[2 * a + 1]) for a in range(len(tree) // 2)] + \
                    ([tree[-1]] if len(tree) % 2 else [])
            mx = jnp.max(tree[0], axis=1, keepdims=True)
            msel = jnp.where(sub == i, mx, msel)
            if i + 1 < TOPC:
                keys = [jnp.where(kk == mx, -jnp.inf, kk) for kk in keys]
        oht = jnp.concatenate([jnp.where(kk == msel, 1.0, 0.0) for kk in keys0], axis=1).astype(BF)
        rsel = lax.bitcast_convert_type(
            lax.bitcast_convert_type(msel[:, 0:1], jnp.int32) & jnp.int32(-S), F32)

        xsel = lax.dot_general(oht, h2_s[...], NT, preferred_element_type=F32).astype(BF)
        cp_wg.wait()
        cp_wu.wait()
        cp_wd.wait()
        gg = jnp.dot(xsel, wg_v[...], preferred_element_type=F32)
        uu = jnp.dot(xsel, wu_v[...], preferred_element_type=F32)
        act = (gg * jax.nn.sigmoid(gg) * uu).astype(BF)
        yy = lax.dot_general(act, wdT_v[...], NT, preferred_element_type=F32)
        yy = yy * jax.nn.sigmoid(rsel)
        yT = yy.T.astype(BF)

        def out_copy(i):
            cs = pl.ds(i * T, T)
            return pltpu.make_async_copy(outT_v.at[:, cs], outT_hbm.at[:, cs], sem_out.at[i])

        for i in range(NB):
            cs = pl.ds(i * T, T)
            upd = jnp.dot(yT, oht[:, i * T:(i + 1) * T], preferred_element_type=F32)
            gbc = jnp.concatenate([colf_s[3]] * TPB, axis=1)
            outT_v[:, cs] = (out0_s[:, cs] + gbc * upd).astype(BF)
            out_copy(i).start()
        for i in range(NB):
            out_copy(i).wait()

    scratch = [
        pltpu.VMEM((D, S + LANES), BF),
        pltpu.VMEM((HKV, SK, DH), BF),
        pltpu.VMEM((HKV, SK, DH), BF),
        pltpu.VMEM((HKV, D, HD), BF),
        pltpu.VMEM((HKV, D, HD), BF),
        pltpu.VMEM((D, F), BF),
        pltpu.VMEM((D, F), BF),
        pltpu.VMEM((D, F), BF),
        pltpu.VMEM((D, 6 * D), BF),
        pltpu.VMEM((2, 8, D), F32),
        pltpu.VMEM((7, D, LANES), F32),
        pltpu.VMEM((16, D), BF),
        pltpu.VMEM((2 * T, D), BF),
        pltpu.VMEM((R, SK), F32),
        pltpu.VMEM((R, SK), F32),
        pltpu.VMEM((R, LANES), F32),
        pltpu.VMEM((R, LANES), F32),
        pltpu.VMEM((T, HD), BF),
        pltpu.VMEM((T, HD), BF),
        pltpu.VMEM((3, D, T), F32),
        pltpu.SMEM((1,), jnp.int32),
        pltpu.VMEM((D, S), F32),
        pltpu.VMEM((D, S), BF),
        pltpu.VMEM((NTILE, 8, LANES), F32),
        pltpu.VMEM((D, S), BF),
        pltpu.SemaphoreType.DMA((HKV, 4)),
        pltpu.SemaphoreType.DMA((8,)),
        pltpu.SemaphoreType.DMA((NB,)),
    ]
    anyspec = pl.BlockSpec(memory_space=pl.ANY)
    vm = pl.BlockSpec(memory_space=pltpu.VMEM)
    return pl.pallas_call(
        kernel,
        in_specs=[anyspec, anyspec, anyspec, anyspec, anyspec, vm, anyspec, anyspec, anyspec, vm, anyspec],
        out_specs=anyspec,
        out_shape=jax.ShapeDtypeStruct((D, S), BF),
        scratch_shapes=scratch,
        compiler_params=pltpu.CompilerParams(vmem_limit_bytes=opts.get('vmem', 110) * 1024 * 1024, flags=flags),
        name='adaln_gqa_moe',
        interpret=opts.get('interpret', False),
    )


def build_fn(T=256, CK=512, flags=None, **opts):
    def fn(A_x, A_k_cache, A_v_cache, A_wq, A_wo, B_x, B_w_r, B_w_gate, B_w_up, B_w_down, c, w_mod):
        B, S, D = A_x.shape
        _, HKV, SK, DH = A_k_cache.shape
        F = B_w_gate.shape[1]
        call = _build(S, SK, D, HKV, DH, F, T, CK, flags, opts)
        outT = call(
            A_x.reshape(S, D).T, A_k_cache.reshape(HKV, SK, DH), A_v_cache.reshape(HKV, SK, DH),
            A_wq, A_wo.T, B_w_r, B_w_gate, B_w_up, B_w_down.T, c, w_mod)
        return outT.T.reshape(B, S, D)
    return fn


_IMPL = build_fn(flags={"XLA_TPU_FORCE_LP_LLO_SCHEDULER": True}, )


@jax.jit
def pallas_adaLN_cond__gqa_block_cached__moe_arch_mod__prompt_kernel(
        A_x, A_k_cache, A_v_cache, A_wq, A_wo, B_x, B_w_r, B_w_gate, B_w_up, B_w_down, c, w_mod):
    return _IMPL(A_x, A_k_cache, A_v_cache, A_wq, A_wo, B_x, B_w_r, B_w_gate, B_w_up, B_w_down, c, w_mod)
```

```python
import functools

import jax
import jax.numpy as jnp
from jax import lax
import jax.experimental.pallas as pl
import jax.experimental.pallas.tpu as pltpu

BF = jnp.bfloat16
F32 = jnp.float32
NT = (((1,), (1,)), ((), ()))
LOG2E = 1.4426950408889634
EPS = 1e-5
TOPC = 8
LANES = 128


def _build(S, SK, D, HKV, DH, F, T, CK, flags, opts):
    REP = 2
    R = REP * T
    NB = S // T
    TPB = T // LANES
    NTILE = S // LANES
    NC = SK // CK
    HD = REP * DH
    NP = HKV // 2
    qscale = (DH ** -0.5) * LOG2E
    PH = opts.get('ph', [1, 1, 1, 1, 1, 1, 1, 0])
    FC = opts.get('fc', 48)
    assert HKV % 2 == 0 and TPB == 2 and NC == 4 and D % FC == 0 and FC % 16 == 0 and NB >= 3
    assert S & (S - 1) == 0 and NP & (NP - 1) == 0
    LOG_NP = NP.bit_length() - 1

    def kernel(xT_hbm, k_hbm, v_hbm, wq_hbm, woT_hbm, wr_hbm, wg_hbm, wu_hbm, wdT_hbm, c_hbm, wm_hbm,
               outT_hbm,
               xT_v, k_v, v_v, wq_v, woT_v, wg_v, wu_v, wdT_v, wm_v, c_v, wr_v,
               modr_s, colf_s, wr_s, h_s, s_s0, s_s1, m_s0, m_s1, o_s0, o_s1, acc_s, zero_s, out0_s, h2_s, r_s,
               outT_v, flag_s,
               sem_w, sem_misc, sem_out):
        s_s = (s_s0, s_s1)
        m_s = (m_s0, m_s1)
        o_s = (o_s0, o_s1)
        if opts.get('prof'):
            scope = jax.named_scope
        else:
            import contextlib
            scope = lambda name: contextlib.nullcontext()

        def cp_wq(p):
            return pltpu.make_async_copy(wq_hbm.at[:, pl.ds(p * 2 * HD, 2 * HD)], wq_v.at[p], sem_w.at[0, p])

        def cp_k(p):
            return pltpu.make_async_copy(k_hbm.at[pl.ds(2 * p, 2)], k_v.at[pl.ds(2 * p, 2)], sem_w.at[1, p])

        def cp_v(p):
            return pltpu.make_async_copy(v_hbm.at[pl.ds(2 * p, 2)], v_v.at[pl.ds(2 * p, 2)], sem_w.at[2, p])

        def cp_wo(p):
            return pltpu.make_async_copy(woT_hbm.at[:, pl.ds(p * 2 * HD, 2 * HD)], woT_v.at[p], sem_w.at[3, p])

        def cols(src, dst, lo, n, sem):
            return pltpu.make_async_copy(src.at[:, pl.ds(lo, n)], dst.at[:, pl.ds(lo, n)], sem)

        def head(src, dst, g, sem):
            return pltpu.make_async_copy(src.at[pl.ds(g, 1)], dst.at[pl.ds(g, 1)], sem)

        cp_wq0 = [cols(wq_hbm, wq_v.at[0], i * HD, HD, sem_misc.at[8 + i]) for i in range(2)]
        cp_k0 = [head(k_hbm, k_v, i, sem_misc.at[10 + i]) for i in range(2)]
        cp_v0 = [head(v_hbm, v_v, i, sem_misc.at[12 + i]) for i in range(2)]
        cp_wm1 = cols(wm_hbm, wm_v, 0, 2 * D, sem_misc.at[0])
        cp_wm2 = cols(wm_hbm, wm_v, 2 * D, 4 * D, sem_misc.at[1])
        cp_x0 = cols(xT_hbm, xT_v, 0, T, sem_misc.at[2])
        cp_x1 = cols(xT_hbm, xT_v, T, T, sem_misc.at[3])
        cp_x2 = cols(xT_hbm, xT_v, 2 * T, S - 2 * T, sem_misc.at[4])
        cp_wg = pltpu.make_async_copy(wg_hbm, wg_v, sem_misc.at[5])
        cp_wu = pltpu.make_async_copy(wu_hbm, wu_v, sem_misc.at[6])
        cp_wd = pltpu.make_async_copy(wdT_hbm, wdT_v, sem_misc.at[7])
        cp_c = pltpu.make_async_copy(c_hbm, c_v, sem_misc.at[14])
        cp_wr = pltpu.make_async_copy(wr_hbm, wr_v, sem_misc.at[15])

        def cp_out(t):
            cs = pl.ds(pl.multiple_of(t * T, T), T)
            return pltpu.make_async_copy(outT_v.at[:, cs], outT_hbm.at[:, cs], sem_out.at[t])

        def cp_fix(tl):
            cs = pl.ds(tl * LANES, LANES)
            return pltpu.make_async_copy(outT_v.at[:, cs], outT_hbm.at[:, cs], sem_out.at[NB + tl])

        def in_own_block(fn):
            def body(i, carry):
                fn()
                return carry
            lax.fori_loop(0, zero_s[0] + 1, body, 0)

        zero_s[0] = 0
        for cp in (cp_c, cp_wr, cp_x0, cp_wm1, cp_wq0[0], cp_k0[0], cp_wq0[1], cp_k0[1], cp_v0[0], cp_x1,
                   cp_v0[1]):
            cp.start()

        def request_pairs():
            for p0 in range(1, NP):
                cp_wq(p0).start()
                cp_k(p0).start()
                cp_wo(p0 - 1).start()
                cp_v(p0).start()
            cp_wo(NP - 1).start()
        in_own_block(request_pairs)

        def fold(a):
            n = a.shape[0]
            while n > 8:
                if n % 16 == 0:
                    n //= 2
                    a = a[0:n] + a[n:2 * n]
                else:
                    r = a[0:8]
                    for i in range(1, n // 8):
                        r = r + a[8 * i:8 * i + 8]
                    a, n = r, 8
            return a

        def total(a):
            return jnp.sum(a, axis=0, keepdims=True) * (1.0 / D)

        def x_rows(lo, n, tile):
            col = pl.ds(pl.multiple_of(tile * LANES, LANES), LANES)
            return xT_v[pl.ds(lo, n), col].astype(F32)

        def stat_pieces(load_a, load_b, st):
            def sum_piece(lo):
                def run():
                    part = fold(load_a(lo, FC))
                    st['s'] = part if lo == 0 else st['s'] + part
                    if lo + FC == D:
                        st['mu'] = total(st['s'])
                return run

            def var_piece(lo):
                def run():
                    xc = load_b(lo, FC) - st['mu']
                    part = fold(xc * xc)
                    st['q'] = part if lo == 0 else st['q'] + part
                    if lo + FC == D:
                        st['rstd'] = lax.rsqrt(total(st['q']) + EPS)
                return run
            return [sum_piece(lo) for lo in range(0, D, FC)] + [var_piece(lo) for lo in range(0, D, FC)]

        def ln1_pieces(tile, row_dst):
            st = {}
            row = pl.ds(pl.multiple_of(row_dst, LANES), LANES)
            ld = lambda lo, n: x_rows(lo, n, tile)

            def apply_piece(lo):
                def run():
                    n = min(LANES, D - lo)
                    hn = ((ld(lo, n) - st['mu']) * st['rstd']).T
                    hh = hn * modr_s[1, 0:1, pl.ds(lo, n)] + modr_s[0, 0:1, pl.ds(lo, n)]
                    h_s[row, pl.ds(lo, n)] = hh.astype(BF)
                return run
            return stat_pieces(ld, ld, st), [apply_piece(lo) for lo in range(0, D, LANES)]

        def ln2_pieces(tile, slot, half):
            st = {}
            col = pl.ds(pl.multiple_of(tile * LANES, LANES), LANES)
            acol = pl.ds(half * LANES, LANES)

            def load_a(lo, n):
                rows = pl.ds(lo, n)
                x2 = x_rows(lo, n, tile) + colf_s[0, rows, :] * acc_s[slot, rows, acol]
                acc_s[slot, rows, acol] = jnp.zeros((n, LANES), F32)
                x2 = x2.astype(BF).astype(F32)
                colf_s[5 + half, rows, :] = x2
                return x2

            def apply_piece(lo):
                def run():
                    rows = pl.ds(lo, FC)
                    x2 = colf_s[5 + half, rows, :]
                    h2 = ((x2 - st['mu']) * st['rstd'] * colf_s[2, rows, :] + colf_s[1, rows, :]).astype(BF)
                    h2_s[rows, col] = h2
                    o0 = x2 + colf_s[3, rows, :] * h2.astype(F32)
                    out0_s[rows, col] = o0
                    outT_v[rows, col] = o0.astype(BF)
                return run
            return (stat_pieces(load_a, lambda lo, n: colf_s[5 + half, pl.ds(lo, n), :], st)
                    + [apply_piece(lo) for lo in range(0, D, FC)])

        def interleave(a, b):
            return [f for pair_ in zip(a, b) for f in pair_]

        def run_all(pieces):
            for f in pieces:
                f()

        def anchor(v, z):
            xT_v[0:16, pl.ds(pl.multiple_of(S + z * LANES, LANES), LANES)] = v.astype(BF)
            colf_s[4 + z, 0:8, :] = v[0:8]

        def r_tile(tile):
            col = pl.multiple_of(tile * LANES, LANES)
            rr = jnp.dot(wr_s[...], h2_s[:, pl.ds(col, LANES)], preferred_element_type=F32)
            r_s[tile] = rr[0:8, :]

        def step(ua, up, uo, par, extra=None, pieces=None):
            pieces = list(pieces or [])
            phases = [ph for ph in range(2 * NC) if PH[ph]]

            def place(v, ph):
                if not pieces or ph not in phases:
                    return
                left = len([q for q in phases if q >= ph])
                npc = -(-len(pieces) // left)
                mine = [pieces.pop(0) for _ in range(npc)]
                for i, f in enumerate(mine):
                    r0 = ((i * R // len(mine)) // 16) * 16
                    anchor(v[r0:r0 + 16, 0:LANES], zero_s[0])
                    f()

            if ua is not None:
                hslot, pa = ua
                hrow = pl.multiple_of(hslot * T, T)
                qf = jnp.dot(h_s[pl.ds(hrow, T), :], wq_v[pa, :, pl.ds(par * HD, HD)],
                             preferred_element_type=F32) * qscale
                qb = qf.astype(BF)
                q2 = jnp.concatenate([qb[:, r * DH:(r + 1) * DH] for r in range(REP)], axis=0)
                mrun = None
            if uo is not None:
                aslot, po = uo
                y = lax.dot_general(woT_v[po, :, pl.ds(par * HD, HD)], o_s[par][...], NT,
                                    preferred_element_type=F32)
                acc_s[aslot] = acc_s[aslot] + y
            if up is not None:
                mrow = jnp.max(m_s[1 - par][...], axis=-1, keepdims=True)
                lrun = None
                oacc = None
            for c in range(NC):
                keys = pl.ds(c * CK, CK)
                if up is not None:
                    sv = s_s[1 - par][:, keys]
                    p = jnp.exp2(sv - mrow)
                    ll = p[:, 0:LANES]
                    for jj in range(1, CK // LANES):
                        ll = ll + p[:, jj * LANES:(jj + 1) * LANES]
                    lrun = ll if lrun is None else lrun + ll
                    o = jnp.dot(p.astype(BF), v_v[up, keys, :], preferred_element_type=F32)
                    oacc = o if oacc is None else oacc + o
                    place(o, 2 * c)
                if ua is not None:
                    s = lax.dot_general(q2, k_v[2 * pa + par, keys, :], NT, preferred_element_type=F32)
                    s_s[par][:, keys] = s
                    mm = s[:, 0:LANES]
                    for jj in range(1, CK // LANES):
                        mm = jnp.maximum(mm, s[:, jj * LANES:(jj + 1) * LANES])
                    mrun = mm if mrun is None else jnp.maximum(mrun, mm)
                    place(s, 2 * c + 1)
            if up is not None:
                lsum = jnp.sum(lrun, axis=-1, keepdims=True)
                ob = (oacc * pltpu.reciprocal(lsum, approx=False, full_range=False)).astype(BF)
                for r in range(REP):
                    o_s[1 - par][:, r * DH:(r + 1) * DH] = ob[r * T:(r + 1) * T, :]
            if ua is not None:
                m_s[par][...] = mrun
            if extra is not None:
                extra()

        acc_s[...] = jnp.zeros(acc_s.shape, F32)

        cp_c.wait()
        cp_wr.wait()
        cc = jnp.broadcast_to(c_v[...].astype(F32), (8, D))
        sc = (cc * jax.nn.sigmoid(cc)).astype(BF)
        wr_s[...] = jnp.broadcast_to(wr_v[...].reshape(1, D), (16, D))

        with scope('ln1_first'):
            cp_x0.wait()
            first_ln = [ln1_pieces(i, i * LANES) for i in range(TPB)]
            run_all(interleave(first_ln[0][0], first_ln[1][0]))
            cp_wm1.wait()
            mod1 = jnp.dot(sc, wm_v[:, pl.ds(0, 2 * D)], preferred_element_type=F32)
            modr_s[0] = mod1[:, 0:D]
            modr_s[1] = mod1[:, D:2 * D] + 1.0
            run_all(interleave(first_ln[0][1], first_ln[1][1]))

        in_own_block(lambda: [cp.start() for cp in (cp_x2, cp_wm2, cp_wg, cp_wu, cp_wd)])

        def pair_units(t, p):
            return ((t + (p >> LOG_NP)) & 1, p & (NP - 1)), (t & 1, p - 1)

        def pair(t, p, pieces=(None, None), extra=None):
            ua, uo = pair_units(t, p)
            step(ua, 2 * p - 1, uo, 0, pieces=pieces[0])
            step(ua, (2 * p) & (HKV - 1), uo, 1, pieces=pieces[1], extra=extra)

        def ln1_block(tsrc, tdst):
            la = [ln1_pieces(tsrc * TPB + i, (tdst & 1) * T + i * LANES) for i in range(TPB)]
            return interleave(la[0][0] + la[0][1], la[1][0] + la[1][1])

        with scope('fill'):
            cp_wq0[0].wait()
            cp_k0[0].wait()
            step((0, 0), None, None, 0)
            cp_wq0[1].wait()
            cp_k0[1].wait()
            cp_v0[0].wait()
            step((0, 0), 0, None, 1)
            ua, uo = pair_units(0, 1)
            cp_x1.wait()
            cp_v0[1].wait()
            cp_wq(1).wait()
            cp_k(1).wait()
            cp_wo(0).wait()
            step(ua, 1, uo, 0, pieces=ln1_block(1, 1))
            cp_v(1).wait()
            step(ua, 2, uo, 1)

        def block(t, carry):
            def inner(b, carry2):
                p = b + 2
                first = t == 0

                @pl.when(jnp.logical_and(first, p < NP))
                def _():
                    cp_wq(p).wait()
                    cp_k(p).wait()
                    cp_v(p).wait()

                @pl.when(first)
                def _():
                    cp_wo(p - 1).wait()

                pair(t, p)
                return carry2

            with scope('inner'):
                lax.fori_loop(0, NP - 1 - (t == NB - 1).astype(jnp.int32), inner, 0)

            def mod_rest(i, carry2):
                cp_x2.wait()
                cp_wm2.wait()
                mod2 = jnp.dot(sc, wm_v[:, pl.ds(2 * D, 4 * D)], preferred_element_type=F32)
                for k2 in range(4):
                    row = mod2[0:1, k2 * D:(k2 + 1) * D]
                    if k2 == 2:
                        row = row + 1.0
                    colf_s[k2] = jnp.broadcast_to(row, (LANES, D)).T
                return carry2
            with scope('mod_rest'):
                lax.fori_loop(0, (t == 0).astype(jnp.int32), mod_rest, 0)

            @pl.when(t < NB - 1)
            def _():
                with scope('peeled'):
                    p1 = ln1_block(jnp.minimum(t + 2, NB - 1), t)
                    p2 = interleave(*[ln2_pieces(t * TPB + i, t & 1, i) for i in range(TPB)])
                    pair(t + 1, 1, pieces=(p1, p2), extra=lambda: [r_tile(t * TPB + i) for i in range(TPB)])
                    cp_out(t).start()
            return carry

        lax.fori_loop(0, NB, block, 0)
        with scope('drain'):
            tl = NB - 1
            step(None, HKV - 1, ((NB - 1) % 2, NP - 1), 0)
            step(None, None, ((NB - 1) % 2, NP - 1), 1)

        with scope('ln2_tail'):
            run_all(interleave(*[ln2_pieces(tl * TPB + i, (NB - 1) % 2, i) for i in range(TPB)]))
            cp_out(tl).start()
            for i in range(TPB):
                r_tile(tl * TPB + i)

        with scope('topk'):
            lane = lax.broadcasted_iota(jnp.int32, (8, LANES), 1)
            sub = lax.broadcasted_iota(jnp.int32, (8, LANES), 0)
            keys = []
            for i in range(NTILE):
                rv = r_s[i]
                tok = lane + i * LANES
                code = jnp.where(rv < 0.0, tok, (S - 1) - tok)
                mag = jnp.maximum(jnp.abs(rv), 1.1754944e-38)
                bits = (lax.bitcast_convert_type(mag, jnp.int32) & jnp.int32(-S)) | code
                kf = lax.bitcast_convert_type(bits, F32)
                keys.append(jnp.where(rv < 0.0, -kf, kf))
            keys0 = list(keys)
            msel = jnp.zeros((8, LANES), F32)
            for i in range(TOPC):
                tree = list(keys)
                while len(tree) > 1:
                    tree = [jnp.maximum(tree[2 * a], tree[2 * a + 1]) for a in range(len(tree) // 2)]
                mx = jnp.max(tree[0], axis=1, keepdims=True)
                msel = jnp.where(sub == i, mx, msel)
                if i + 1 < TOPC:
                    keys = [jnp.where(kk == mx, -jnp.inf, kk) for kk in keys]
            hot = [jnp.where(kk == msel, 1.0, 0.0) for kk in keys0]
            oht = jnp.concatenate(hot, axis=1).astype(BF)
            mbits = lax.bitcast_convert_type(msel, jnp.int32)
            rsel = lax.bitcast_convert_type(mbits & jnp.int32(-S), F32)[:, 0:1]
            code = mbits & jnp.int32(S - 1)
            tile_of = jnp.where(msel < 0.0, code, (S - 1) - code) // LANES
            for i in range(TOPC):
                flag_s[NTILE + i] = jnp.max(tile_of[i:i + 1, 0:1])
            for i in range(NTILE):
                hit = flag_s[NTILE] == i
                for j in range(1, TOPC):
                    hit = jnp.logical_or(hit, flag_s[NTILE + j] == i)
                flag_s[i] = hit.astype(jnp.int32)

        with scope('ffn'):
            xsel = lax.dot_general(oht, h2_s[...], NT, preferred_element_type=F32).astype(BF)
            cp_wg.wait()
            cp_wu.wait()
            cp_wd.wait()
            gg = jnp.dot(xsel, wg_v[...], preferred_element_type=F32)
            uu = jnp.dot(xsel, wu_v[...], preferred_element_type=F32)
            act = (gg * jax.nn.sigmoid(gg) * uu).astype(BF)
            yy = lax.dot_general(act, wdT_v[...], NT, preferred_element_type=F32)
            yy = yy * jax.nn.sigmoid(rsel)
            yT = yy.T.astype(BF)

        with scope('final'):
            for i in range(NB):
                cp_out(i).wait()
            for i in range(NTILE):
                @pl.when(flag_s[i] > 0)
                def _():
                    cs = pl.ds(i * LANES, LANES)
                    upd = jnp.dot(yT, hot[i].astype(BF), preferred_element_type=F32)
                    outT_v[:, cs] = (out0_s[:, cs] + colf_s[3] * upd).astype(BF)
                    cp_fix(i).start()
            for i in range(NTILE):
                @pl.when(flag_s[i] > 0)
                def _():
                    cp_fix(i).wait()

    scratch = [
        pltpu.VMEM((D, S + LANES), BF),
        pltpu.VMEM((HKV, SK, DH), BF),
        pltpu.VMEM((HKV, SK, DH), BF),
        pltpu.VMEM((NP, D, 2 * HD), BF),
        pltpu.VMEM((NP, D, 2 * HD), BF),
        pltpu.VMEM((D, F), BF),
        pltpu.VMEM((D, F), BF),
        pltpu.VMEM((D, F), BF),
        pltpu.VMEM((D, 6 * D), BF),
        pltpu.VMEM((1, D), BF),
        pltpu.VMEM((D,), BF),
        pltpu.VMEM((2, 8, D), F32),
        pltpu.VMEM((7, D, LANES), F32),
        pltpu.VMEM((16, D), BF),
        pltpu.VMEM((2 * T, D), BF),
        pltpu.VMEM((R, SK), F32),
        pltpu.VMEM((R, SK), F32),
        pltpu.VMEM((R, LANES), F32),
        pltpu.VMEM((R, LANES), F32),
        pltpu.VMEM((T, HD), BF),
        pltpu.VMEM((T, HD), BF),
        pltpu.VMEM((2, D, T), F32),
        pltpu.SMEM((1,), jnp.int32),
        pltpu.VMEM((D, S), F32),
        pltpu.VMEM((D, S), BF),
        pltpu.VMEM((NTILE, 8, LANES), F32),
        pltpu.VMEM((D, S), BF),
        pltpu.SMEM((NTILE + TOPC,), jnp.int32),
        pltpu.SemaphoreType.DMA((4, NP)),
        pltpu.SemaphoreType.DMA((16,)),
        pltpu.SemaphoreType.DMA((NB + NTILE,)),
    ]
    anyspec = pl.BlockSpec(memory_space=pl.ANY)
    return pl.pallas_call(
        kernel,
        in_specs=[anyspec] * 11,
        out_specs=anyspec,
        out_shape=jax.ShapeDtypeStruct((D, S), BF),
        scratch_shapes=scratch,
        compiler_params=pltpu.CompilerParams(vmem_limit_bytes=opts.get('vmem', 110) * 1024 * 1024, flags=flags),
        name='adaln_gqa_moe',
        interpret=opts.get('interpret', False),
    )


def build_fn(T=256, CK=512, flags=None, **opts):
    def fn(A_x, A_k_cache, A_v_cache, A_wq, A_wo, B_x, B_w_r, B_w_gate, B_w_up, B_w_down, c, w_mod):
        B, S, D = A_x.shape
        _, HKV, SK, DH = A_k_cache.shape
        F = B_w_gate.shape[1]
        call = _build(S, SK, D, HKV, DH, F, T, CK, flags, opts)
        outT = call(
            A_x.reshape(S, D).T, A_k_cache.reshape(HKV, SK, DH), A_v_cache.reshape(HKV, SK, DH),
            A_wq, A_wo.T, B_w_r, B_w_gate, B_w_up, B_w_down.T, c, w_mod)
        return outT.T.reshape(B, S, D)
    return fn


_IMPL = build_fn(flags={"XLA_TPU_FORCE_LP_LLO_SCHEDULER": True}, )


@jax.jit
def pallas_adaLN_cond__gqa_block_cached__moe_arch_mod__prompt_kernel(
        A_x, A_k_cache, A_v_cache, A_wq, A_wo, B_x, B_w_r, B_w_gate, B_w_up, B_w_down, c, w_mod):
    return _IMPL(A_x, A_k_cache, A_v_cache, A_wq, A_wo, B_x, B_w_r, B_w_gate, B_w_up, B_w_down, c, w_mod)
```

```python
import functools

import jax
import jax.numpy as jnp
from jax import lax
import jax.experimental.pallas as pl
import jax.experimental.pallas.tpu as pltpu

BF = jnp.bfloat16
F32 = jnp.float32
NT = (((1,), (1,)), ((), ()))
LOG2E = 1.4426950408889634
EPS = 1e-5
TOPC = 8
LANES = 128


def _build(S, SK, D, HKV, DH, F, T, CK, flags, opts):
    REP = 2
    R = REP * T
    NB = S // T
    TPB = T // LANES
    NTILE = S // LANES
    NC = SK // CK
    HD = REP * DH
    NP = HKV // 2
    qscale = (DH ** -0.5) * LOG2E
    PH = opts.get('ph', [1] * 7 + [0])
    NL = opts.get('nl', 1)
    FC = opts.get('fc', 48)
    assert HKV % 2 == 0 and TPB == 2 and D % FC == 0 and FC % 16 == 0 and NB >= 3
    assert S & (S - 1) == 0 and NP & (NP - 1) == 0
    LOG_NP = NP.bit_length() - 1

    def kernel(xT_hbm, k_hbm, v_hbm, wq_hbm, woT_hbm, wr_hbm, wg_hbm, wu_hbm, wdT_hbm, c_hbm, wm_hbm,
               outT_hbm,
               xT_v, k_v, v_v, wq_v, woT_v, wg_v, wu_v, wdT_v, wm_v, c_v, wr_v,
               modr_s, colf_s, wr_s, h_s, s_s0, s_s1, m_s0, m_s1, o_s0, o_s1, acc_s, zero_s, out0_s, h2_s, r_s,
               outT_v, flag_s, of_s0, of_s1, l_s0, l_s1,
               sem_w, sem_misc, sem_out):
        s_s = (s_s0, s_s1)
        m_s = (m_s0, m_s1)
        o_s = (o_s0, o_s1)
        of_s = (of_s0, of_s1)
        l_s = (l_s0, l_s1)
        if opts.get('prof'):
            scope = jax.named_scope
        else:
            import contextlib
            scope = lambda name: contextlib.nullcontext()

        def cp_wq(p):
            return pltpu.make_async_copy(wq_hbm.at[:, pl.ds(p * 2 * HD, 2 * HD)], wq_v.at[p], sem_w.at[0, p])

        def cp_k(p):
            return pltpu.make_async_copy(k_hbm.at[pl.ds(2 * p, 2)], k_v.at[pl.ds(2 * p, 2)], sem_w.at[1, p])

        def cp_v(p):
            return pltpu.make_async_copy(v_hbm.at[pl.ds(2 * p, 2)], v_v.at[pl.ds(2 * p, 2)], sem_w.at[2, p])

        def cp_wo(p):
            return pltpu.make_async_copy(woT_hbm.at[:, pl.ds(p * 2 * HD, 2 * HD)], woT_v.at[p], sem_w.at[3, p])

        def cols(src, dst, lo, n, sem):
            return pltpu.make_async_copy(src.at[:, pl.ds(lo, n)], dst.at[:, pl.ds(lo, n)], sem)

        def head(src, dst, g, sem):
            return pltpu.make_async_copy(src.at[pl.ds(g, 1)], dst.at[pl.ds(g, 1)], sem)

        cp_wq0 = [cols(wq_hbm, wq_v.at[0], i * HD, HD, sem_misc.at[8 + i]) for i in range(2)]
        cp_k0 = [head(k_hbm, k_v, i, sem_misc.at[10 + i]) for i in range(2)]
        cp_v0 = [head(v_hbm, v_v, i, sem_misc.at[12 + i]) for i in range(2)]
        cp_wm1 = cols(wm_hbm, wm_v, 0, 2 * D, sem_misc.at[0])
        cp_wm2 = cols(wm_hbm, wm_v, 2 * D, 4 * D, sem_misc.at[1])
        cp_x0 = cols(xT_hbm, xT_v, 0, T, sem_misc.at[2])
        cp_x1 = cols(xT_hbm, xT_v, T, T, sem_misc.at[3])
        cp_x2 = cols(xT_hbm, xT_v, 2 * T, S - 2 * T, sem_misc.at[4])
        cp_wg = pltpu.make_async_copy(wg_hbm, wg_v, sem_misc.at[5])
        cp_wu = pltpu.make_async_copy(wu_hbm, wu_v, sem_misc.at[6])
        cp_wd = pltpu.make_async_copy(wdT_hbm, wdT_v, sem_misc.at[7])
        cp_c = pltpu.make_async_copy(c_hbm, c_v, sem_misc.at[14])
        cp_wr = pltpu.make_async_copy(wr_hbm, wr_v, sem_misc.at[15])

        def cp_out(t):
            cs = pl.ds(pl.multiple_of(t * T, T), T)
            return pltpu.make_async_copy(outT_v.at[:, cs], outT_hbm.at[:, cs], sem_out.at[t])

        def cp_fix(tl):
            cs = pl.ds(tl * LANES, LANES)
            return pltpu.make_async_copy(outT_v.at[:, cs], outT_hbm.at[:, cs], sem_out.at[NB + tl])

        def in_own_block(fn):
            def body(i, carry):
                fn()
                return carry
            lax.fori_loop(0, zero_s[0] + 1, body, 0)

        zero_s[0] = 0
        for cp in (cp_c, cp_wr, cp_x0, cp_wm1, cp_wq0[0], cp_k0[0], cp_wq0[1], cp_k0[1], cp_v0[0], cp_x1,
                   cp_v0[1]):
            cp.start()

        def request_pairs():
            for p0 in range(1, NP):
                cp_wq(p0).start()
                cp_k(p0).start()
                cp_wo(p0 - 1).start()
                cp_v(p0).start()
            cp_wo(NP - 1).start()
        in_own_block(request_pairs)

        def fold(a):
            n = a.shape[0]
            while n > 8:
                if n % 16 == 0:
                    n //= 2
                    a = a[0:n] + a[n:2 * n]
                else:
                    r = a[0:8]
                    for i in range(1, n // 8):
                        r = r + a[8 * i:8 * i + 8]
                    a, n = r, 8
            return a

        def total(a):
            return jnp.sum(a, axis=0, keepdims=True) * (1.0 / D)

        def x_rows(lo, n, tile):
            col = pl.ds(pl.multiple_of(tile * LANES, LANES), LANES)
            return xT_v[pl.ds(lo, n), col].astype(F32)

        def stat_pieces(load_a, load_b, st):
            def sum_piece(lo):
                def run():
                    part = fold(load_a(lo, FC))
                    st['s'] = part if lo == 0 else st['s'] + part
                    if lo + FC == D:
                        st['mu'] = total(st['s'])
                return run

            def var_piece(lo):
                def run():
                    xc = load_b(lo, FC) - st['mu']
                    part = fold(xc * xc)
                    st['q'] = part if lo == 0 else st['q'] + part
                    if lo + FC == D:
                        st['rstd'] = lax.rsqrt(total(st['q']) + EPS)
                return run
            return [sum_piece(lo) for lo in range(0, D, FC)] + [var_piece(lo) for lo in range(0, D, FC)]

        def ln1_pieces(tile, row_dst):
            st = {}
            row = pl.ds(pl.multiple_of(row_dst, LANES), LANES)
            ld = lambda lo, n: x_rows(lo, n, tile)

            def apply_piece(lo):
                def run():
                    n = min(LANES, D - lo)
                    hn = ((ld(lo, n) - st['mu']) * st['rstd']).T
                    hh = hn * modr_s[1, 0:1, pl.ds(lo, n)] + modr_s[0, 0:1, pl.ds(lo, n)]
                    h_s[row, pl.ds(lo, n)] = hh.astype(BF)
                return run
            return stat_pieces(ld, ld, st), [apply_piece(lo) for lo in range(0, D, LANES)]

        def ln2_pieces(tile, slot, half):
            st = {}
            col = pl.ds(pl.multiple_of(tile * LANES, LANES), LANES)
            acol = pl.ds(half * LANES, LANES)

            def load_a(lo, n):
                rows = pl.ds(lo, n)
                x2 = x_rows(lo, n, tile) + colf_s[0, rows, :] * acc_s[slot, rows, acol]
                acc_s[slot, rows, acol] = jnp.zeros((n, LANES), F32)
                x2 = x2.astype(BF).astype(F32)
                colf_s[5 + half, rows, :] = x2
                return x2

            def apply_piece(lo):
                def run():
                    rows = pl.ds(lo, FC)
                    x2 = colf_s[5 + half, rows, :]
                    h2 = ((x2 - st['mu']) * st['rstd'] * colf_s[2, rows, :] + colf_s[1, rows, :]).astype(BF)
                    h2_s[rows, col] = h2
                    o0 = x2 + colf_s[3, rows, :] * h2.astype(F32)
                    out0_s[rows, col] = o0
                    outT_v[rows, col] = o0.astype(BF)
                return run
            return (stat_pieces(load_a, lambda lo, n: colf_s[5 + half, pl.ds(lo, n), :], st)
                    + [apply_piece(lo) for lo in range(0, D, FC)])

        def interleave(a, b):
            return [f for pair_ in zip(a, b) for f in pair_]

        def run_all(pieces):
            for f in pieces:
                f()

        def anchor(v, z):
            xT_v[0:16, pl.ds(pl.multiple_of(S + z * LANES, LANES), LANES)] = v.astype(BF)
            colf_s[4 + z, 0:8, :] = v[0:8]

        def r_tile(tile):
            col = pl.multiple_of(tile * LANES, LANES)
            rr = jnp.dot(wr_s[...], h2_s[:, pl.ds(col, LANES)], preferred_element_type=F32)
            r_s[tile] = rr[0:8, :]

        def step(ua, up, uo, par, extra=None, pieces=None, ck=None, nl_in=None, nl_out=None):
            pieces = list(pieces or [])
            nl_in = NL if nl_in is None else nl_in
            nl_out = NL if nl_out is None else nl_out
            CK = ck or (opts.get('ckp', 512) if pieces else opts.get('cki', 2048))
            NC = SK // CK
            nslot = 2 * SK // 512
            slots = [i for i in range(nslot) if PH[i]]
            state = {'slot': 0}

            def place(v):
                for c0 in range(0, v.shape[1], 512):
                    ph = state['slot']
                    state['slot'] += 1
                    if not pieces or ph not in slots:
                        continue
                    left = len([q for q in slots if q >= ph])
                    npc = -(-len(pieces) // left)
                    mine = [pieces.pop(0) for _ in range(npc)]
                    for i, f in enumerate(mine):
                        r0 = ((i * R // len(mine)) // 16) * 16
                        anchor(v[r0:r0 + 16, c0:c0 + LANES], zero_s[0])
                        f()

            OP = opts.get('opos', 'start')
            st = {}

            def ldkv(ref, g, c):
                if opts.get('u32'):
                    return pltpu.bitcast(ref.bitcast(jnp.uint32)[g, pl.ds(c * (CK // 2), CK // 2), :], BF)
                return ref[g, pl.ds(c * CK, CK), :]

            def do_q():
                hslot, pa = ua
                hrow = pl.multiple_of(hslot * T, T)
                if opts.get('ksplit', 1):
                    k0 = (D // LANES) * LANES
                    qf = jnp.dot(h_s[pl.ds(hrow, T), pl.ds(k0, D - k0)], wq_v[pa, pl.ds(k0, D - k0), pl.ds(par * HD, HD)],
                                 preferred_element_type=F32)
                    qf = qf + jnp.dot(h_s[pl.ds(hrow, T), pl.ds(0, k0)], wq_v[pa, pl.ds(0, k0), pl.ds(par * HD, HD)],
                                      preferred_element_type=F32)
                    qf = qf * qscale
                else:
                    qf = jnp.dot(h_s[pl.ds(hrow, T), :], wq_v[pa, :, pl.ds(par * HD, HD)],
                                 preferred_element_type=F32) * qscale
                qb = qf.astype(BF)
                st['q2'] = jnp.concatenate([qb[:, r * DH:(r + 1) * DH] for r in range(REP)], axis=0)

            def do_o():
                aslot, po = uo
                if nl_in:
                    if nl_in == 1:
                        lsum = jnp.sum(l_s[par][...], axis=-1, keepdims=True)
                    else:
                        lsum = l_s[par][...]
                    ob = (of_s[par][...] * pltpu.reciprocal(lsum, approx=False, full_range=False)).astype(BF)
                    o2 = jnp.concatenate([ob[r * T:(r + 1) * T, :] for r in range(REP)], axis=1)
                else:
                    o2 = o_s[par][...]
                y = lax.dot_general(woT_v[po, :, pl.ds(par * HD, HD)], o2, NT,
                                    preferred_element_type=F32)
                acc_s[aslot] = acc_s[aslot] + y

            def do_m():
                if opts.get('mend'):
                    st['mrow'] = m_s[1 - par][...]
                else:
                    st['mrow'] = jnp.max(m_s[1 - par][...], axis=-1, keepdims=True)

            def do_p(c):
                keys = pl.ds(c * CK, CK)
                sv = s_s[1 - par][:, keys]
                mrow = st['mrow']
                if opts.get('mend'):
                    mrow = jnp.concatenate([mrow] * (CK // LANES), axis=1)
                p = jnp.exp2(sv - mrow)
                ll = p[:, 0:LANES]
                for jj in range(1, CK // LANES):
                    ll = ll + p[:, jj * LANES:(jj + 1) * LANES]
                st['l'] = ll if c == 0 else st['l'] + ll
                o = jnp.dot(p.astype(BF), ldkv(v_v, up, c), preferred_element_type=F32)
                st['o'] = o if c == 0 else st['o'] + o
                place(p if opts.get('anchp', CK > 512) else o)

            def do_s(c):
                keys = pl.ds(c * CK, CK)
                s = lax.dot_general(st['q2'], ldkv(k_v, 2 * ua[1] + par, c), NT, preferred_element_type=F32)
                s_s[par][:, keys] = s
                mm = s[:, 0:LANES]
                for jj in range(1, CK // LANES):
                    mm = jnp.maximum(mm, s[:, jj * LANES:(jj + 1) * LANES])
                st['m'] = mm if c == 0 else jnp.maximum(st['m'], mm)
                place(s)

            def do_norm():
                if nl_out:
                    of_s[1 - par][...] = st['o']
                    if nl_out == 1:
                        l_s[1 - par][...] = st['l']
                    else:
                        l_s[1 - par][...] = jnp.broadcast_to(jnp.sum(st['l'], axis=-1, keepdims=True), (R, LANES))
                    return
                lsum = jnp.sum(st['l'], axis=-1, keepdims=True)
                ob = (st['o'] * pltpu.reciprocal(lsum, approx=False, full_range=False)).astype(BF)
                for r in range(REP):
                    o_s[1 - par][:, r * DH:(r + 1) * DH] = ob[r * T:(r + 1) * T, :]

            if OP == 'first' and uo is not None:
                do_o()
            if opts.get('mfirst') and up is not None:
                do_m()
            if ua is not None:
                do_q()
            if OP == 'start' and uo is not None:
                do_o()
            if not opts.get('mfirst') and up is not None:
                do_m()
            for c in range(NC):
                if opts.get('sfirst') and c > 0:
                    if ua is not None:
                        do_s(c - 1)
                if up is not None:
                    do_p(c)
                if not opts.get('sfirst') and ua is not None:
                    do_s(c)
                if OP == c and uo is not None:
                    do_o()
            if opts.get('sfirst'):
                if opts.get('normlast') and ua is not None:
                    do_s(NC - 1)
                if up is not None:
                    do_norm()
                if not opts.get('normlast') and ua is not None:
                    do_s(NC - 1)
            elif up is not None:
                do_norm()
            if OP == 'end' and uo is not None:
                do_o()
            if ua is not None:
                if opts.get('mend'):
                    m_s[par][...] = jnp.broadcast_to(jnp.max(st['m'], axis=-1, keepdims=True), (R, LANES))
                else:
                    m_s[par][...] = st['m']
            if extra is not None:
                extra()

        acc_s[...] = jnp.zeros(acc_s.shape, F32)

        cp_c.wait()
        cp_wr.wait()
        cc = jnp.broadcast_to(c_v[...].astype(F32), (8, D))
        sc = (cc * jax.nn.sigmoid(cc)).astype(BF)
        wr_s[...] = jnp.broadcast_to(wr_v[...].reshape(1, D), (16, D))

        with scope('ln1_first'):
            cp_x0.wait()
            first_ln = [ln1_pieces(i, i * LANES) for i in range(TPB)]
            run_all(interleave(first_ln[0][0], first_ln[1][0]))
            cp_wm1.wait()
            mod1 = jnp.dot(sc, wm_v[:, pl.ds(0, 2 * D)], preferred_element_type=F32)
            modr_s[0] = mod1[:, 0:D]
            modr_s[1] = mod1[:, D:2 * D] + 1.0
            run_all(interleave(first_ln[0][1], first_ln[1][1]))

        in_own_block(lambda: [cp.start() for cp in (cp_x2, cp_wm2, cp_wg, cp_wu, cp_wd)])

        def pair_units(t, p):
            return ((t + (p >> LOG_NP)) & 1, p & (NP - 1)), (t & 1, p - 1)

        def pair(t, p, pieces=(None, None), extra=None):
            ua, uo = pair_units(t, p)
            step(ua, 2 * p - 1, uo, 0, pieces=pieces[0])
            step(ua, (2 * p) & (HKV - 1), uo, 1, pieces=pieces[1], extra=extra)

        def ln1_block(tsrc, tdst):
            la = [ln1_pieces(tsrc * TPB + i, (tdst & 1) * T + i * LANES) for i in range(TPB)]
            return interleave(la[0][0] + la[0][1], la[1][0] + la[1][1])

        with scope('fill'):
            cp_wq0[0].wait()
            cp_k0[0].wait()
            step((0, 0), None, None, 0)
            cp_wq0[1].wait()
            cp_k0[1].wait()
            cp_v0[0].wait()
            step((0, 0), 0, None, 1)
            ua, uo = pair_units(0, 1)
            cp_x1.wait()
            cp_v0[1].wait()
            cp_wq(1).wait()
            cp_k(1).wait()
            cp_wo(0).wait()
            step(ua, 1, uo, 0, pieces=ln1_block(1, 1))
            cp_v(1).wait()
            step(ua, 2, uo, 1)

        def block(t, carry):
            def inner(b, carry2):
                p = b + 2
                first = t == 0

                @pl.when(jnp.logical_and(first, p < NP))
                def _():
                    cp_wq(p).wait()
                    cp_k(p).wait()
                    cp_v(p).wait()

                @pl.when(first)
                def _():
                    cp_wo(p - 1).wait()

                pair(t, p)
                return carry2

            with scope('inner'):
                lax.fori_loop(0, NP - 1 - (t == NB - 1).astype(jnp.int32), inner, 0)

            def mod_rest(i, carry2):
                cp_x2.wait()
                cp_wm2.wait()
                mod2 = jnp.dot(sc, wm_v[:, pl.ds(2 * D, 4 * D)], preferred_element_type=F32)
                for k2 in range(4):
                    row = mod2[0:1, k2 * D:(k2 + 1) * D]
                    if k2 == 2:
                        row = row + 1.0
                    colf_s[k2] = jnp.broadcast_to(row, (LANES, D)).T
                return carry2
            with scope('mod_rest'):
                lax.fori_loop(0, (t == 0).astype(jnp.int32), mod_rest, 0)

            @pl.when(t < NB - 1)
            def _():
                with scope('peeled'):
                    p1 = ln1_block(jnp.minimum(t + 2, NB - 1), t)
                    p2 = interleave(*[ln2_pieces(t * TPB + i, t & 1, i) for i in range(TPB)])
                    pair(t + 1, 1, pieces=(p1, p2), extra=lambda: [r_tile(t * TPB + i) for i in range(TPB)])
                    cp_out(t).start()
            return carry

        lax.fori_loop(0, NB, block, 0)
        if opts.get('dead'):
            def dead(i, c):
                for u in range(opts['dead']):
                    step(None, None, (0, i), u & 1) if opts.get('small') else step((0, i), 1, (0, i), u & 1)
                return c
            lax.fori_loop(0, zero_s[0], dead, 0)
        with scope('drain'):
            tl = NB - 1
            step(None, HKV - 1, ((NB - 1) % 2, NP - 1), 0, nl_out=0)
            step(None, None, ((NB - 1) % 2, NP - 1), 1, nl_in=0)

        with scope('ln2_tail'):
            run_all(interleave(*[ln2_pieces(tl * TPB + i, (NB - 1) % 2, i) for i in range(TPB)]))
            cp_out(tl).start()
            for i in range(TPB):
                r_tile(tl * TPB + i)

        with scope('topk'):
            lane = lax.broadcasted_iota(jnp.int32, (8, LANES), 1)
            sub = lax.broadcasted_iota(jnp.int32, (8, LANES), 0)
            keys = []
            for i in range(NTILE):
                rv = r_s[i]
                tok = lane + i * LANES
                code = jnp.where(rv < 0.0, tok, (S - 1) - tok)
                mag = jnp.maximum(jnp.abs(rv), 1.1754944e-38)
                bits = (lax.bitcast_convert_type(mag, jnp.int32) & jnp.int32(-S)) | code
                kf = lax.bitcast_convert_type(bits, F32)
                keys.append(jnp.where(rv < 0.0, -kf, kf))
            keys0 = list(keys)
            msel = jnp.zeros((8, LANES), F32)
            for i in range(TOPC):
                tree = list(keys)
                while len(tree) > 1:
                    tree = [jnp.maximum(tree[2 * a], tree[2 * a + 1]) for a in range(len(tree) // 2)]
                mx = jnp.max(tree[0], axis=1, keepdims=True)
                msel = jnp.where(sub == i, mx, msel)
                if i + 1 < TOPC:
                    keys = [jnp.where(kk == mx, -jnp.inf, kk) for kk in keys]
            hot = [jnp.where(kk == msel, 1.0, 0.0) for kk in keys0]
            oht = jnp.concatenate(hot, axis=1).astype(BF)
            mbits = lax.bitcast_convert_type(msel, jnp.int32)
            rsel = lax.bitcast_convert_type(mbits & jnp.int32(-S), F32)[:, 0:1]
            code = mbits & jnp.int32(S - 1)
            tile_of = jnp.where(msel < 0.0, code, (S - 1) - code) // LANES
            for i in range(TOPC):
                flag_s[NTILE + i] = jnp.max(tile_of[i:i + 1, 0:1])
            for i in range(NTILE):
                hit = flag_s[NTILE] == i
                for j in range(1, TOPC):
                    hit = jnp.logical_or(hit, flag_s[NTILE + j] == i)
                flag_s[i] = hit.astype(jnp.int32)

        with scope('ffn'):
            xsel = lax.dot_general(oht, h2_s[...], NT, preferred_element_type=F32).astype(BF)
            cp_wg.wait()
            cp_wu.wait()
            cp_wd.wait()
            gg = jnp.dot(xsel, wg_v[...], preferred_element_type=F32)
            uu = jnp.dot(xsel, wu_v[...], preferred_element_type=F32)
            act = (gg * jax.nn.sigmoid(gg) * uu).astype(BF)
            yy = lax.dot_general(act, wdT_v[...], NT, preferred_element_type=F32)
            yy = yy * jax.nn.sigmoid(rsel)
            yT = yy.T.astype(BF)

        with scope('final'):
            for i in range(NB):
                cp_out(i).wait()
            for i in range(NTILE):
                @pl.when(flag_s[i] > 0)
                def _():
                    cs = pl.ds(i * LANES, LANES)
                    upd = jnp.dot(yT, hot[i].astype(BF), preferred_element_type=F32)
                    outT_v[:, cs] = (out0_s[:, cs] + colf_s[3] * upd).astype(BF)
                    cp_fix(i).start()
            for i in range(NTILE):
                @pl.when(flag_s[i] > 0)
                def _():
                    cp_fix(i).wait()

    scratch = [
        pltpu.VMEM((D, S + LANES), BF),
        pltpu.VMEM((HKV, SK, DH), BF),
        pltpu.VMEM((HKV, SK, DH), BF),
        pltpu.VMEM((NP, D, 2 * HD), BF),
        pltpu.VMEM((NP, D, 2 * HD), BF),
        pltpu.VMEM((D, F), BF),
        pltpu.VMEM((D, F), BF),
        pltpu.VMEM((D, F), BF),
        pltpu.VMEM((D, 6 * D), BF),
        pltpu.VMEM((1, D), BF),
        pltpu.VMEM((D,), BF),
        pltpu.VMEM((2, 8, D), F32),
        pltpu.VMEM((7, D, LANES), F32),
        pltpu.VMEM((16, D), BF),
        pltpu.VMEM((2 * T, D), BF),
        pltpu.VMEM((R, SK), F32),
        pltpu.VMEM((R, SK), F32),
        pltpu.VMEM((R, LANES), F32),
        pltpu.VMEM((R, LANES), F32),
        pltpu.VMEM((T, HD), BF),
        pltpu.VMEM((T, HD), BF),
        pltpu.VMEM((2, D, T), F32),
        pltpu.SMEM((1,), jnp.int32),
        pltpu.VMEM((D, S), F32),
        pltpu.VMEM((D, S), BF),
        pltpu.VMEM((NTILE, 8, LANES), F32),
        pltpu.VMEM((D, S), BF),
        pltpu.SMEM((NTILE + TOPC,), jnp.int32),
        pltpu.VMEM((R, LANES), F32), pltpu.VMEM((R, LANES), F32), pltpu.VMEM((R, LANES), F32), pltpu.VMEM((R, LANES), F32),
        pltpu.SemaphoreType.DMA((4, NP)),
        pltpu.SemaphoreType.DMA((16,)),
        pltpu.SemaphoreType.DMA((NB + NTILE,)),
    ]
    anyspec = pl.BlockSpec(memory_space=pl.ANY)
    return pl.pallas_call(
        kernel,
        in_specs=[anyspec] * 11,
        out_specs=anyspec,
        out_shape=jax.ShapeDtypeStruct((D, S), BF),
        scratch_shapes=scratch,
        compiler_params=pltpu.CompilerParams(vmem_limit_bytes=opts.get('vmem', 110) * 1024 * 1024, flags=flags),
        name='adaln_gqa_moe',
        interpret=opts.get('interpret', False),
    )


def build_fn(T=256, CK=512, flags=None, **opts):
    def fn(A_x, A_k_cache, A_v_cache, A_wq, A_wo, B_x, B_w_r, B_w_gate, B_w_up, B_w_down, c, w_mod):
        B, S, D = A_x.shape
        _, HKV, SK, DH = A_k_cache.shape
        F = B_w_gate.shape[1]
        call = _build(S, SK, D, HKV, DH, F, T, CK, flags, opts)
        outT = call(
            A_x.reshape(S, D).T, A_k_cache.reshape(HKV, SK, DH), A_v_cache.reshape(HKV, SK, DH),
            A_wq, A_wo.T, B_w_r, B_w_gate, B_w_up, B_w_down.T, c, w_mod)
        return outT.T.reshape(B, S, D)
    return fn


_IMPL = build_fn(flags={"XLA_TPU_FORCE_LP_LLO_SCHEDULER": True}, )


@jax.jit
def pallas_adaLN_cond__gqa_block_cached__moe_arch_mod__prompt_kernel(
        A_x, A_k_cache, A_v_cache, A_wq, A_wo, B_x, B_w_r, B_w_gate, B_w_up, B_w_down, c, w_mod):
    return _IMPL(A_x, A_k_cache, A_v_cache, A_wq, A_wo, B_x, B_w_r, B_w_gate, B_w_up, B_w_down, c, w_mod)
```

```python
import functools

import jax
import jax.numpy as jnp
from jax import lax
import jax.experimental.pallas as pl
import jax.experimental.pallas.tpu as pltpu

BF = jnp.bfloat16
F32 = jnp.float32
NT = (((1,), (1,)), ((), ()))
LOG2E = 1.4426950408889634
EPS = 1e-5
TOPC = 8
LANES = 128


def _build(S, SK, D, HKV, DH, F, T, CK, flags, opts):
    REP = 2
    R = REP * T
    NB = S // T
    TPB = T // LANES
    NTILE = S // LANES
    NC = SK // CK
    HD = REP * DH
    NP = HKV // 2
    qscale = (DH ** -0.5) * LOG2E
    PH = opts.get('ph', [1] * 7 + [0])
    NL = opts.get('nl', 0)
    FC = opts.get('fc', 48)
    assert HKV % 2 == 0 and TPB == 2 and D % FC == 0 and FC % 16 == 0 and NB >= 3
    assert S & (S - 1) == 0 and NP & (NP - 1) == 0
    LOG_NP = NP.bit_length() - 1

    def kernel(xT_hbm, k_hbm, v_hbm, wq_hbm, woT_hbm, wr_hbm, wg_hbm, wu_hbm, wdT_hbm, c_hbm, wm_hbm,
               outT_hbm,
               xT_v, k_v, v_v, wq_v, woT_v, wg_v, wu_v, wdT_v, wm_v, c_v, wr_v,
               modr_s, colf_s, h_s, s_s0, s_s1, m_s0, m_s1, o_s0, o_s1, acc_s, zero_s, h2_s, r_s,
               outT_v, flag_s, hot_s, of_s0, of_s1, l_s0, l_s1,
               sem_w, sem_first, sem_misc, sem_out):
        s_s = (s_s0, s_s1)
        m_s = (m_s0, m_s1)
        o_s = (o_s0, o_s1)
        of_s = (of_s0, of_s1)
        l_s = (l_s0, l_s1)
        if opts.get('prof'):
            scope = jax.named_scope
        else:
            import contextlib
            scope = lambda name: contextlib.nullcontext()

        def cp_wq(p):
            return pltpu.make_async_copy(wq_hbm.at[:, pl.ds(p * 2 * HD, 2 * HD)], wq_v.at[p], sem_w.at[0, p])

        def cp_k(p):
            return pltpu.make_async_copy(k_hbm.at[pl.ds(2 * p, 2)], k_v.at[pl.ds(2 * p, 2)], sem_w.at[1, p])

        def cp_v(p):
            return pltpu.make_async_copy(v_hbm.at[pl.ds(2 * p, 2)], v_v.at[pl.ds(2 * p, 2)], sem_w.at[2, p])

        def cp_wo(p):
            return pltpu.make_async_copy(woT_hbm.at[:, pl.ds(p * 2 * HD, 2 * HD)], woT_v.at[p], sem_w.at[3, p])

        def cols(src, dst, lo, n, sem):
            return pltpu.make_async_copy(src.at[:, pl.ds(lo, n)], dst.at[:, pl.ds(lo, n)], sem)

        def head(src, dst, g, sem):
            return pltpu.make_async_copy(src.at[pl.ds(g, 1)], dst.at[pl.ds(g, 1)], sem)

        def half(src, dst, g, sem):
            lo = (g % 2) * HD
            return pltpu.make_async_copy(src.at[:, pl.ds(g * HD, HD)], dst.at[g // 2, :, pl.ds(lo, HD)], sem)

        cp_wq0 = [half(wq_hbm, wq_v, g, sem_first.at[0, g]) for g in range(4)]
        cp_k0 = [head(k_hbm, k_v, g, sem_first.at[1, g]) for g in range(4)]
        cp_v0 = [head(v_hbm, v_v, g, sem_first.at[2, g]) for g in range(4)]
        cp_wo0 = [half(woT_hbm, woT_v, g, sem_first.at[3, g]) for g in range(2)]
        cp_wm1 = cols(wm_hbm, wm_v, 0, 2 * D, sem_misc.at[0])
        cp_wm2 = cols(wm_hbm, wm_v, 2 * D, 4 * D, sem_misc.at[1])
        cp_x0 = cols(xT_hbm, xT_v, 0, T, sem_misc.at[2])
        cp_x1 = cols(xT_hbm, xT_v, T, T, sem_misc.at[3])
        cp_x2 = cols(xT_hbm, xT_v, 2 * T, S - 2 * T, sem_misc.at[4])
        cp_wg = pltpu.make_async_copy(wg_hbm, wg_v, sem_misc.at[5])
        cp_wu = pltpu.make_async_copy(wu_hbm, wu_v, sem_misc.at[6])
        cp_wd = pltpu.make_async_copy(wdT_hbm, wdT_v, sem_misc.at[7])
        cp_c = pltpu.make_async_copy(c_hbm, c_v, sem_misc.at[8])
        cp_wr = pltpu.make_async_copy(wr_hbm, wr_v, sem_misc.at[9])

        def cp_out(t):
            cs = pl.ds(pl.multiple_of(t * T, T), T)
            return pltpu.make_async_copy(outT_v.at[:, cs], outT_hbm.at[:, cs], sem_out.at[t])

        def cp_fix(i, tile):
            cs = pl.ds(pl.multiple_of(tile * LANES, LANES), LANES)
            return pltpu.make_async_copy(outT_v.at[:, cs], outT_hbm.at[:, cs], sem_out.at[NB + i])

        def in_own_block(fn):
            def body(i, carry):
                fn()
                return carry
            lax.fori_loop(0, zero_s[0] + 1, body, 0)

        zero_s[0] = 0
        for cp in (cp_c, cp_wr, cp_x0, cp_wm1, cp_wq0[0], cp_k0[0]):
            cp.start()
        in_own_block(lambda: [cp.start() for cp in (cp_wq0[1], cp_k0[1], cp_v0[0])])
        in_own_block(lambda: [cp.start() for cp in (cp_wq0[2], cp_k0[2], cp_v0[1], cp_wo0[0])])
        in_own_block(lambda: [cp.start() for cp in (cp_x1, cp_wq0[3], cp_k0[3], cp_v0[2], cp_wo0[1], cp_v0[3])])

        def request_pairs():
            for p0 in range(2, NP):
                cp_wq(p0).start()
                cp_k(p0).start()
                cp_wo(p0 - 1).start()
                cp_v(p0).start()
            cp_wo(NP - 1).start()
        in_own_block(request_pairs)

        def fold(a):
            n = a.shape[0]
            while n > 8:
                if n % 16 == 0:
                    n //= 2
                    a = a[0:n] + a[n:2 * n]
                else:
                    r = a[0:8]
                    for i in range(1, n // 8):
                        r = r + a[8 * i:8 * i + 8]
                    a, n = r, 8
            return a

        def total(a):
            return jnp.sum(a, axis=0, keepdims=True) * (1.0 / D)

        def x_rows(lo, n, tile):
            col = pl.ds(pl.multiple_of(tile * LANES, LANES), LANES)
            return xT_v[pl.ds(lo, n), col].astype(F32)

        def stat_pieces(load_a, load_b, st):
            def sum_piece(lo):
                def run():
                    part = fold(load_a(lo, FC))
                    st['s'] = part if lo == 0 else st['s'] + part
                    if lo + FC == D:
                        st['mu'] = total(st['s'])
                return run

            def var_piece(lo):
                def run():
                    xc = load_b(lo, FC) - st['mu']
                    part = fold(xc * xc)
                    st['q'] = part if lo == 0 else st['q'] + part
                    if lo + FC == D:
                        st['rstd'] = lax.rsqrt(total(st['q']) + EPS)
                return run
            return [sum_piece(lo) for lo in range(0, D, FC)] + [var_piece(lo) for lo in range(0, D, FC)]

        def ln1_pieces(tile, row_dst, raw=False):
            st = {}
            row = pl.ds(pl.multiple_of(row_dst, LANES), LANES)
            ld = lambda lo, n: x_rows(lo, n, tile)

            def apply_piece(lo):
                def run():
                    n = min(LANES, D - lo)
                    hn = ((ld(lo, n) - st['mu']) * st['rstd']).T
                    if raw:
                        s_s0[row, pl.ds(lo, n)] = hn
                    else:
                        hh = hn * modr_s[1, 0:1, pl.ds(lo, n)] + modr_s[0, 0:1, pl.ds(lo, n)]
                        h_s[row, pl.ds(lo, n)] = hh.astype(BF)
                return run
            return stat_pieces(ld, ld, st), [apply_piece(lo) for lo in range(0, D, LANES)]

        def ln2_pieces(tile, slot, half, acc_val=None, st=None):
            st = {} if st is None else st
            col = pl.ds(pl.multiple_of(tile * LANES, LANES), LANES)
            acol = pl.ds(half * LANES, LANES)

            def load_a(lo, n):
                rows = pl.ds(lo, n)
                av = acc_s[slot, rows, acol] if acc_val is None else acc_val[lo:lo + n, :]
                x2 = (x_rows(lo, n, tile) + colf_s[0, rows, :] * av).astype(BF)
                xT_v[rows, col] = x2
                return x2.astype(F32)

            def load_b(lo, n):
                return x_rows(lo, n, tile)

            def apply_piece(lo):
                def run():
                    rows = pl.ds(lo, FC)
                    x2 = load_b(lo, FC)
                    h2 = ((x2 - st['mu']) * st['rstd'] * colf_s[2, rows, :] + colf_s[1, rows, :]).astype(BF)
                    h2_s[rows, col] = h2
                    h2 = h2.astype(F32)
                    outT_v[rows, col] = (x2 + colf_s[3, rows, :] * h2).astype(BF)
                    if opts.get('rv', 1):
                        part = fold(h2 * colf_s[4, rows, :])
                        st['r'] = part if lo == 0 else st['r'] + part
                        if lo + FC == D:
                            r_s[tile] = jnp.broadcast_to(jnp.sum(st['r'], axis=0, keepdims=True), (8, LANES))
                return run
            sp = stat_pieces(load_a, load_b, st)
            if acc_val is not None:
                run_all(sp[:D // FC])
                sp = sp[D // FC:]
            return sp + [apply_piece(lo) for lo in range(0, D, FC)]

        def interleave(a, b):
            return [f for pair_ in zip(a, b) for f in pair_]

        def run_all(pieces):
            for f in pieces:
                f()

        def anchor(v, z):
            xT_v[0:16, pl.ds(pl.multiple_of(S + z * LANES, LANES), LANES)] = v.astype(BF)
            colf_s[5 + z, 0:8, :] = v[0:8]

        def r_tile(tile):
            col = pl.multiple_of(tile * LANES, LANES)
            wr16 = jnp.broadcast_to(wr_v[...].reshape(1, D), (16, D))
            rr = jnp.dot(wr16, h2_s[:, pl.ds(col, LANES)], preferred_element_type=F32)
            r_s[tile] = rr[0:8, :]

        def step(ua, up, uo, par, extra=None, pieces=None, ck=None, nl_in=None, nl_out=None, o_sink=None,
                 o_init=False):
            pieces = list(pieces or [])
            nl_in = NL if nl_in is None else nl_in
            nl_out = NL if nl_out is None else nl_out
            CK = ck or (opts.get('ckp', 512) if pieces else opts.get('cki', 2048))
            NC = SK // CK
            nslot = 2 * SK // 512
            slots = [i for i in range(nslot) if PH[i]]
            state = {'slot': 0}

            def place(v):
                for c0 in range(0, v.shape[1], 512):
                    ph = state['slot']
                    state['slot'] += 1
                    if not pieces or ph not in slots:
                        continue
                    left = len([q for q in slots if q >= ph])
                    npc = -(-len(pieces) // left)
                    mine = [pieces.pop(0) for _ in range(npc)]
                    for i, f in enumerate(mine):
                        r0 = ((i * R // len(mine)) // 16) * 16
                        anchor(v[r0:r0 + 16, c0:c0 + LANES], zero_s[0])
                        f()

            OP = opts.get('opos', 'start')
            st = {}

            def ldkv(ref, g, c):
                if opts.get('u32'):
                    return pltpu.bitcast(ref.bitcast(jnp.uint32)[g, pl.ds(c * (CK // 2), CK // 2), :], BF)
                return ref[g, pl.ds(c * CK, CK), :]

            def do_q():
                hslot, pa = ua
                hrow = pl.multiple_of(hslot * T, T)
                if opts.get('ksplit', 1):
                    k0 = (D // LANES) * LANES
                    qf = jnp.dot(h_s[pl.ds(hrow, T), pl.ds(k0, D - k0)], wq_v[pa, pl.ds(k0, D - k0), pl.ds(par * HD, HD)],
                                 preferred_element_type=F32)
                    qf = qf + jnp.dot(h_s[pl.ds(hrow, T), pl.ds(0, k0)], wq_v[pa, pl.ds(0, k0), pl.ds(par * HD, HD)],
                                      preferred_element_type=F32)
                    qf = qf * qscale
                else:
                    qf = jnp.dot(h_s[pl.ds(hrow, T), :], wq_v[pa, :, pl.ds(par * HD, HD)],
                                 preferred_element_type=F32) * qscale
                qb = qf.astype(BF)
                st['q2'] = jnp.concatenate([qb[:, r * DH:(r + 1) * DH] for r in range(REP)], axis=0)

            def do_o():
                aslot, po = uo
                if nl_in:
                    if nl_in == 1:
                        lsum = jnp.sum(l_s[par][...], axis=-1, keepdims=True)
                    else:
                        lsum = l_s[par][...]
                    ob = (of_s[par][...] * pltpu.reciprocal(lsum, approx=False, full_range=False)).astype(BF)
                    o2 = jnp.concatenate([ob[r * T:(r + 1) * T, :] for r in range(REP)], axis=1)
                else:
                    o2 = o_s[par][...]
                y = lax.dot_general(woT_v[po, :, pl.ds(par * HD, HD)], o2, NT,
                                    preferred_element_type=F32)
                if o_init:
                    acc_s[aslot] = y
                elif o_sink is None:
                    acc_s[aslot] = acc_s[aslot] + y
                else:
                    o_sink(acc_s[aslot] + y)

            def do_m():
                if opts.get('mend'):
                    st['mrow'] = m_s[1 - par][...]
                else:
                    st['mrow'] = jnp.max(m_s[1 - par][...], axis=-1, keepdims=True)

            def do_p(c):
                keys = pl.ds(c * CK, CK)
                sv = s_s[1 - par][:, keys]
                mrow = st['mrow']
                if opts.get('mend'):
                    mrow = jnp.concatenate([mrow] * (CK // LANES), axis=1)
                p = jnp.exp2(sv - mrow)
                ll = p[:, 0:LANES]
                for jj in range(1, CK // LANES):
                    ll = ll + p[:, jj * LANES:(jj + 1) * LANES]
                st['l'] = ll if c == 0 else st['l'] + ll
                o = jnp.dot(p.astype(BF), ldkv(v_v, up, c), preferred_element_type=F32)
                st['o'] = o if c == 0 else st['o'] + o
                place(p if opts.get('anchp', CK > 512) else o)

            def do_s(c):
                keys = pl.ds(c * CK, CK)
                s = lax.dot_general(st['q2'], ldkv(k_v, 2 * ua[1] + par, c), NT, preferred_element_type=F32)
                s_s[par][:, keys] = s
                mm = s[:, 0:LANES]
                for jj in range(1, CK // LANES):
                    mm = jnp.maximum(mm, s[:, jj * LANES:(jj + 1) * LANES])
                st['m'] = mm if c == 0 else jnp.maximum(st['m'], mm)
                place(s)

            def do_norm():
                if nl_out:
                    of_s[1 - par][...] = st['o']
                    if nl_out == 1:
                        l_s[1 - par][...] = st['l']
                    else:
                        l_s[1 - par][...] = jnp.broadcast_to(jnp.sum(st['l'], axis=-1, keepdims=True), (R, LANES))
                    return
                lsum = jnp.sum(st['l'], axis=-1, keepdims=True)
                ob = (st['o'] * pltpu.reciprocal(lsum, approx=False, full_range=False)).astype(BF)
                for r in range(REP):
                    o_s[1 - par][:, r * DH:(r + 1) * DH] = ob[r * T:(r + 1) * T, :]

            if OP == 'first' and uo is not None:
                do_o()
            if opts.get('mfirst', 1) and up is not None:
                do_m()
            if ua is not None:
                do_q()
            if OP == 'start' and uo is not None:
                do_o()
            if not opts.get('mfirst', 1) and up is not None:
                do_m()
            for c in range(NC):
                if opts.get('sfirst') and c > 0:
                    if ua is not None:
                        do_s(c - 1)
                if up is not None:
                    do_p(c)
                if not opts.get('sfirst') and ua is not None:
                    do_s(c)
                if OP == c and uo is not None:
                    do_o()
            if opts.get('sfirst'):
                if opts.get('normlast') and ua is not None:
                    do_s(NC - 1)
                if up is not None:
                    do_norm()
                if not opts.get('normlast') and ua is not None:
                    do_s(NC - 1)
            elif up is not None:
                do_norm()
            if OP == 'end' and uo is not None:
                do_o()
            if ua is not None:
                if opts.get('mend'):
                    m_s[par][...] = jnp.broadcast_to(jnp.max(st['m'], axis=-1, keepdims=True), (R, LANES))
                else:
                    m_s[par][...] = st['m']
            if extra is not None:
                extra()


        cp_c.wait()
        cp_wr.wait()
        cc = jnp.broadcast_to(c_v[...].astype(F32), (8, D))
        sc = (cc * jax.nn.sigmoid(cc)).astype(BF)
        colf_s[4] = jnp.broadcast_to(wr_v[...].reshape(1, D).astype(F32), (LANES, D)).T

        with scope('ln1_first'):
            cp_x0.wait()
            first_ln = [ln1_pieces(i, i * LANES, raw=True) for i in range(TPB)]
            run_all(interleave(first_ln[0][0], first_ln[1][0]))
            run_all(interleave(first_ln[0][1], first_ln[1][1]))
            cp_wm1.wait()
            mod1 = jnp.dot(sc, wm_v[:, pl.ds(0, 2 * D)], preferred_element_type=F32)
            sa = mod1[:, 0:D]
            ca1 = mod1[:, D:2 * D] + 1.0
            modr_s[0] = sa
            modr_s[1] = ca1
            h_s[0:T, :] = (s_s0[0:T, 0:D] * ca1[0:1, :] + sa[0:1, :]).astype(BF)

        in_own_block(lambda: [cp.start() for cp in (cp_x2, cp_wm2, cp_wg, cp_wu, cp_wd)])

        def pair_units(t, p):
            return ((t + (p >> LOG_NP)) & 1, p & (NP - 1)), (t & 1, p - 1)

        def pair(t, p, pieces=(None, None), extra=None):
            ua, uo = pair_units(t, p)
            step(ua, 2 * p - 1, uo, 0, pieces=pieces[0], o_init=isinstance(p, int) and p == 1)
            step(ua, (2 * p) & (HKV - 1), uo, 1, pieces=pieces[1], extra=extra)

        def ln1_block(tsrc, tdst):
            la = [ln1_pieces(tsrc * TPB + i, (tdst & 1) * T + i * LANES) for i in range(TPB)]
            return interleave(la[0][0] + la[0][1], la[1][0] + la[1][1])

        with scope('fill'):
            cp_wq0[0].wait()
            cp_k0[0].wait()
            step((0, 0), None, None, 0)
            cp_wq0[1].wait()
            cp_k0[1].wait()
            cp_v0[0].wait()
            step((0, 0), 0, None, 1)
            ua, uo = pair_units(0, 1)
            for cp in (cp_wq0[2], cp_k0[2], cp_v0[1], cp_wo0[0]):
                cp.wait()
            step(ua, 1, uo, 0, o_init=True)
            for cp in (cp_x1, cp_wq0[3], cp_k0[3], cp_v0[2], cp_wo0[1]):
                cp.wait()
            step(ua, 2, uo, 1, pieces=ln1_block(1, 1))
            cp_v0[3].wait()

        def block(t, carry):
            def inner(b, carry2):
                p = b + 2
                first = t == 0

                @pl.when(jnp.logical_and(first, p < NP))
                def _():
                    cp_wq(p).wait()
                    cp_k(p).wait()
                    cp_v(p).wait()

                @pl.when(first)
                def _():
                    cp_wo(p - 1).wait()

                pair(t, p)
                return carry2

            with scope('inner'):
                lax.fori_loop(0, NP - 1 - (t == NB - 1).astype(jnp.int32), inner, 0)

            def mod_rest(i, carry2):
                cp_x2.wait()
                cp_wm2.wait()
                for k2 in range(4):
                    lo = (2 + k2) * D // LANES * LANES
                    hi = -(-((3 + k2) * D) // LANES) * LANES
                    row = jnp.dot(sc, wm_v[:, pl.ds(lo, hi - lo)], preferred_element_type=F32)[0:1, :]
                    if k2 == 2:
                        row = row + 1.0
                    off = (2 + k2) * D - lo
                    colf_s[k2] = jnp.broadcast_to(row, (LANES, hi - lo)).T[off:off + D, :]
                return carry2
            with scope('mod_rest'):
                lax.fori_loop(0, (t == 0).astype(jnp.int32), mod_rest, 0)

            @pl.when(t < NB - 1)
            def _():
                with scope('peeled'):
                    p1 = ln1_block(jnp.minimum(t + 2, NB - 1), t)
                    p2 = interleave(*[ln2_pieces(t * TPB + i, t & 1, i) for i in range(TPB)])
                    pair(t + 1, 1, pieces=(p1, p2),
                         extra=None if opts.get('rv', 1) else (lambda: [r_tile(t * TPB + i) for i in range(TPB)]))
                    cp_out(t).start()
            return carry

        lax.fori_loop(0, NB, block, 0)
        if opts.get('dead'):
            def dead(i, c):
                for u in range(opts['dead']):
                    step(None, None, (0, i), u & 1) if opts.get('small') else step((0, i), 1, (0, i), u & 1)
                return c
            lax.fori_loop(0, zero_s[0], dead, 0)
        with scope('drain'):
            tl = NB - 1
            step(None, HKV - 1, ((NB - 1) % 2, NP - 1), 0, nl_out=0)
            sums = []

            def first_sweep(a):
                for i in range(TPB):
                    st = {}
                    st['rest'] = ln2_pieces(tl * TPB + i, None, i, a[:, i * LANES:(i + 1) * LANES], st)
                    sums.append(st)
            step(None, None, ((NB - 1) % 2, NP - 1), 1, nl_in=0, o_sink=first_sweep)

        with scope('ln2_tail'):
            if not opts.get('tloop', 1):
                run_all(interleave(sums[0]['rest'], sums[1]['rest']))
            else:
                TC = opts.get('tc', 96)
                cols_ = [pl.ds((tl * TPB + i) * LANES, LANES) for i in range(TPB)]
                mus = [st['mu'] for st in sums]

                def var_body(k, qs):
                    rows = pl.ds(pl.multiple_of(k * TC, TC), TC)
                    out = []
                    for i in range(TPB):
                        xc = xT_v[rows, cols_[i]].astype(F32) - mus[i]
                        out.append(qs[i] + fold(xc * xc))
                    return tuple(out)
                qs = lax.fori_loop(0, D // TC, var_body, (jnp.zeros((8, LANES), F32),) * TPB)
                rstds = [lax.rsqrt(total(q) + EPS) for q in qs]

                def apply_body(k, rs):
                    rows = pl.ds(pl.multiple_of(k * TC, TC), TC)
                    out = []
                    for i in range(TPB):
                        x2 = xT_v[rows, cols_[i]].astype(F32)
                        h2 = ((x2 - mus[i]) * rstds[i] * colf_s[2, rows, :] + colf_s[1, rows, :]).astype(BF)
                        h2_s[rows, cols_[i]] = h2
                        h2 = h2.astype(F32)
                        outT_v[rows, cols_[i]] = (x2 + colf_s[3, rows, :] * h2).astype(BF)
                        out.append(rs[i] + fold(h2 * colf_s[4, rows, :]))
                    return tuple(out)
                rs = lax.fori_loop(0, D // TC, apply_body, (jnp.zeros((8, LANES), F32),) * TPB)
                for i in range(TPB):
                    r_s[tl * TPB + i] = jnp.broadcast_to(jnp.sum(rs[i], axis=0, keepdims=True), (8, LANES))
            cp_out(tl).start()

        with scope('topk'):
            lane = lax.broadcasted_iota(jnp.int32, (8, LANES), 1)
            sub = lax.broadcasted_iota(jnp.int32, (8, LANES), 0)
            keys = []
            for i in range(NTILE):
                rv = r_s[i]
                tok = lane + i * LANES
                code = jnp.where(rv < 0.0, tok, (S - 1) - tok)
                mag = jnp.clip(jnp.abs(rv), 1.1754944e-38, 3.0e38)
                bits = (lax.bitcast_convert_type(mag, jnp.int32) & jnp.int32(-S)) | code
                kf = lax.bitcast_convert_type(bits, F32)
                keys.append(jnp.where(rv < 0.0, -kf, kf))
            keys0 = list(keys)
            msel = jnp.zeros((8, LANES), F32)
            for i in range(TOPC):
                tree = list(keys)
                while len(tree) > 1:
                    tree = [jnp.maximum(tree[2 * a], tree[2 * a + 1]) for a in range(len(tree) // 2)]
                mx = jnp.max(tree[0], axis=1, keepdims=True)
                msel = jnp.where(sub == i, mx, msel)
                if i + 1 < TOPC:
                    keys = [jnp.where(kk == mx, -jnp.inf, kk) for kk in keys]
            hot = [jnp.where(kk == msel, 1.0, 0.0) for kk in keys0]
            oht = jnp.concatenate(hot, axis=1).astype(BF)
            mbits = lax.bitcast_convert_type(msel, jnp.int32)
            rsel = lax.bitcast_convert_type(mbits & jnp.int32(-S), F32)[:, 0:1]
            code = mbits & jnp.int32(S - 1)
            tile_of = jnp.where(msel < 0.0, code, (S - 1) - code) // LANES
            for i in range(TOPC):
                flag_s[NTILE + i] = jnp.max(tile_of[i:i + 1, 0:1])
            for i in range(TOPC):
                fresh = jnp.int32(1)
                for j in range(i):
                    fresh = fresh & (flag_s[NTILE + j] != flag_s[NTILE + i]).astype(jnp.int32)
                flag_s[i] = fresh
            for i in range(NTILE):
                hot_s[i] = jnp.concatenate([hot[i], hot[i]], axis=0).astype(BF)[0:16]

        with scope('ffn'):
            xsel = lax.dot_general(oht, h2_s[...], NT, preferred_element_type=F32).astype(BF)
            cp_wg.wait()
            cp_wu.wait()
            cp_wd.wait()
            gg = jnp.dot(xsel, wg_v[...], preferred_element_type=F32)
            uu = jnp.dot(xsel, wu_v[...], preferred_element_type=F32)
            act = (gg * jax.nn.sigmoid(gg) * uu).astype(BF)
            yy = lax.dot_general(act, wdT_v[...], NT, preferred_element_type=F32)
            yy = yy * jax.nn.sigmoid(rsel)
            yT = yy.T.astype(BF)

        with scope('final'):
            for i in range(NB):
                cp_out(i).wait()
            yT2 = jnp.concatenate([yT, jnp.zeros_like(yT)], axis=1)

            for i in range(TOPC):
                @pl.when(flag_s[i] > 0)
                def _():
                    tile = flag_s[NTILE + i]
                    cs = pl.ds(pl.multiple_of(tile * LANES, LANES), LANES)
                    upd = jnp.dot(yT2, hot_s[tile], preferred_element_type=F32)
                    outT_v[:, cs] = (xT_v[:, cs].astype(F32)
                                     + colf_s[3] * (h2_s[:, cs].astype(F32) + upd)).astype(BF)
                    cp_fix(i, tile).start()
            for i in range(TOPC):
                @pl.when(flag_s[i] > 0)
                def _():
                    cp_fix(i, flag_s[NTILE + i]).wait()

    scratch = [
        pltpu.VMEM((D, S + LANES), BF),
        pltpu.VMEM((HKV, SK, DH), BF),
        pltpu.VMEM((HKV, SK, DH), BF),
        pltpu.VMEM((NP, D, 2 * HD), BF),
        pltpu.VMEM((NP, D, 2 * HD), BF),
        pltpu.VMEM((D, F), BF),
        pltpu.VMEM((D, F), BF),
        pltpu.VMEM((D, F), BF),
        pltpu.VMEM((D, 6 * D), BF),
        pltpu.VMEM((1, D), BF),
        pltpu.VMEM((D,), BF),
        pltpu.VMEM((2, 8, D), F32),
        pltpu.VMEM((6, D, LANES), F32),
        pltpu.VMEM((2 * T, D), BF),
        pltpu.VMEM((R, SK), F32),
        pltpu.VMEM((R, SK), F32),
        pltpu.VMEM((R, LANES), F32),
        pltpu.VMEM((R, LANES), F32),
        pltpu.VMEM((T, HD), BF),
        pltpu.VMEM((T, HD), BF),
        pltpu.VMEM((2, D, T), F32),
        pltpu.SMEM((1,), jnp.int32),
        pltpu.VMEM((D, S), BF),
        pltpu.VMEM((NTILE, 8, LANES), F32),
        pltpu.VMEM((D, S), BF),
        pltpu.SMEM((NTILE + TOPC,), jnp.int32),
        pltpu.VMEM((NTILE, 16, LANES), BF),
        pltpu.VMEM((R, LANES), F32), pltpu.VMEM((R, LANES), F32), pltpu.VMEM((R, LANES), F32), pltpu.VMEM((R, LANES), F32),
        pltpu.SemaphoreType.DMA((4, NP)),
        pltpu.SemaphoreType.DMA((4, 4)),
        pltpu.SemaphoreType.DMA((10,)),
        pltpu.SemaphoreType.DMA((NB + TOPC,)),
    ]
    anyspec = pl.BlockSpec(memory_space=pl.ANY)
    return pl.pallas_call(
        kernel,
        in_specs=[anyspec] * 11,
        out_specs=anyspec,
        out_shape=jax.ShapeDtypeStruct((D, S), BF),
        scratch_shapes=scratch,
        compiler_params=pltpu.CompilerParams(vmem_limit_bytes=opts.get('vmem', 110) * 1024 * 1024, flags=flags),
        name='adaln_gqa_moe',
        interpret=opts.get('interpret', False),
    )


def build_fn(T=256, CK=512, flags=None, **opts):
    def fn(A_x, A_k_cache, A_v_cache, A_wq, A_wo, B_x, B_w_r, B_w_gate, B_w_up, B_w_down, c, w_mod):
        B, S, D = A_x.shape
        _, HKV, SK, DH = A_k_cache.shape
        F = B_w_gate.shape[1]
        call = _build(S, SK, D, HKV, DH, F, T, CK, flags, opts)
        outT = call(
            A_x.reshape(S, D).T, A_k_cache.reshape(HKV, SK, DH), A_v_cache.reshape(HKV, SK, DH),
            A_wq, A_wo.T, B_w_r, B_w_gate, B_w_up, B_w_down.T, c, w_mod)
        return outT.T.reshape(B, S, D)
    return fn


_IMPL = build_fn(flags={"XLA_TPU_FORCE_LP_LLO_SCHEDULER": True}, )


@jax.jit
def pallas_adaLN_cond__gqa_block_cached__moe_arch_mod__prompt_kernel(
        A_x, A_k_cache, A_v_cache, A_wq, A_wo, B_x, B_w_r, B_w_gate, B_w_up, B_w_down, c, w_mod):
    return _IMPL(A_x, A_k_cache, A_v_cache, A_wq, A_wo, B_x, B_w_r, B_w_gate, B_w_up, B_w_down, c, w_mod)
```

```python
import functools

import jax
import jax.numpy as jnp
from jax import lax
import jax.experimental.pallas as pl
import jax.experimental.pallas.tpu as pltpu

BF = jnp.bfloat16
F32 = jnp.float32
NT = (((1,), (1,)), ((), ()))
LOG2E = 1.4426950408889634
EPS = 1e-5
TOPC = 8
LANES = 128


def _build(S, SK, D, HKV, DH, F, T, CK, flags, opts):
    REP = 2
    R = REP * T
    NB = S // T
    TPB = T // LANES
    NTILE = S // LANES
    NC = SK // CK
    HD = REP * DH
    NP = HKV // 2
    qscale = (DH ** -0.5) * LOG2E
    PH = opts.get('ph', [0, 0, 0, 0, 1, 1, 1, 0])
    NL = opts.get('nl', 0)
    FC = opts.get('fc', 48)
    assert HKV % 2 == 0 and TPB == 2 and D % FC == 0 and FC % 16 == 0 and NB >= 3
    assert S & (S - 1) == 0 and NP & (NP - 1) == 0
    LOG_NP = NP.bit_length() - 1

    def kernel(xT_hbm, k_hbm, v_hbm, wq_hbm, woT_hbm, wr_hbm, wg_hbm, wu_hbm, wdT_hbm, c_hbm, wm_hbm,
               outT_hbm,
               xT_v, k_v, v_v, wq_v, woT_v, wg_v, wu_v, wdT_v, wm_v, c_v, wr_v,
               modr_s, colf_s, h_s, s_s0, s_s1, m_s0, m_s1, o_s0, o_s1, acc_s, zero_s, h2_s, r_s,
               outT_v, flag_s, hot_s, of_s0, of_s1, l_s0, l_s1,
               sem_w, sem_first, sem_misc, sem_out):
        s_s = (s_s0, s_s1)
        m_s = (m_s0, m_s1)
        o_s = (o_s0, o_s1)
        of_s = (of_s0, of_s1)
        l_s = (l_s0, l_s1)
        if opts.get('prof'):
            scope = jax.named_scope
        else:
            import contextlib
            scope = lambda name: contextlib.nullcontext()

        def cp_wq(p):
            return pltpu.make_async_copy(wq_hbm.at[:, pl.ds(p * 2 * HD, 2 * HD)], wq_v.at[p], sem_w.at[0, p])

        def cp_k(p):
            return pltpu.make_async_copy(k_hbm.at[pl.ds(2 * p, 2)], k_v.at[pl.ds(2 * p, 2)], sem_w.at[1, p])

        def cp_v(p):
            return pltpu.make_async_copy(v_hbm.at[pl.ds(2 * p, 2)], v_v.at[pl.ds(2 * p, 2)], sem_w.at[2, p])

        def cp_wo(p):
            return pltpu.make_async_copy(woT_hbm.at[:, pl.ds(p * 2 * HD, 2 * HD)], woT_v.at[p], sem_w.at[3, p])

        def cols(src, dst, lo, n, sem):
            return pltpu.make_async_copy(src.at[:, pl.ds(lo, n)], dst.at[:, pl.ds(lo, n)], sem)

        def head(src, dst, g, sem):
            return pltpu.make_async_copy(src.at[pl.ds(g, 1)], dst.at[pl.ds(g, 1)], sem)

        def half(src, dst, g, sem):
            lo = (g % 2) * HD
            return pltpu.make_async_copy(src.at[:, pl.ds(g * HD, HD)], dst.at[g // 2, :, pl.ds(lo, HD)], sem)

        cp_wq0 = [half(wq_hbm, wq_v, g, sem_first.at[0, g]) for g in range(4)]
        cp_k0 = [head(k_hbm, k_v, g, sem_first.at[1, g]) for g in range(4)]
        cp_v0 = [head(v_hbm, v_v, g, sem_first.at[2, g]) for g in range(4)]
        cp_wo0 = [half(woT_hbm, woT_v, g, sem_first.at[3, g]) for g in range(2)]
        cp_wm1 = cols(wm_hbm, wm_v, 0, 2 * D, sem_misc.at[0])
        cp_wm2 = cols(wm_hbm, wm_v, 2 * D, 4 * D, sem_misc.at[1])
        cp_x0 = cols(xT_hbm, xT_v, 0, T, sem_misc.at[2])
        cp_x1 = cols(xT_hbm, xT_v, T, T, sem_misc.at[3])
        cp_x2 = cols(xT_hbm, xT_v, 2 * T, S - 2 * T, sem_misc.at[4])
        cp_wg = pltpu.make_async_copy(wg_hbm, wg_v, sem_misc.at[5])
        cp_wu = pltpu.make_async_copy(wu_hbm, wu_v, sem_misc.at[6])
        cp_wd = pltpu.make_async_copy(wdT_hbm, wdT_v, sem_misc.at[7])
        cp_c = pltpu.make_async_copy(c_hbm, c_v, sem_misc.at[8])
        cp_wr = pltpu.make_async_copy(wr_hbm, wr_v, sem_misc.at[9])

        def cp_out(t):
            cs = pl.ds(pl.multiple_of(t * T, T), T)
            return pltpu.make_async_copy(outT_v.at[:, cs], outT_hbm.at[:, cs], sem_out.at[t])

        def cp_fix(i, tile):
            cs = pl.ds(pl.multiple_of(tile * LANES, LANES), LANES)
            return pltpu.make_async_copy(outT_v.at[:, cs], outT_hbm.at[:, cs], sem_out.at[NB + i])

        def in_own_block(fn):
            def body(i, carry):
                fn()
                return carry
            lax.fori_loop(0, zero_s[0] + 1, body, 0)

        zero_s[0] = 0
        for cp in (cp_c, cp_wr, cp_x0, cp_wm1, cp_wq0[0], cp_k0[0]):
            cp.start()
        in_own_block(lambda: [cp.start() for cp in (cp_wq0[1], cp_k0[1], cp_v0[0])])
        in_own_block(lambda: [cp.start() for cp in (cp_wq0[2], cp_k0[2], cp_v0[1], cp_wo0[0])])
        in_own_block(lambda: [cp.start() for cp in (cp_x1, cp_wq0[3], cp_k0[3], cp_v0[2], cp_wo0[1], cp_v0[3])])

        def request_pairs():
            for p0 in range(2, NP):
                cp_wq(p0).start()
                cp_k(p0).start()
                cp_wo(p0 - 1).start()
                cp_v(p0).start()
            cp_wo(NP - 1).start()
        in_own_block(request_pairs)

        def fold(a):
            n = a.shape[0]
            while n > 8:
                if n % 16 == 0:
                    n //= 2
                    a = a[0:n] + a[n:2 * n]
                else:
                    r = a[0:8]
                    for i in range(1, n // 8):
                        r = r + a[8 * i:8 * i + 8]
                    a, n = r, 8
            return a

        def total(a):
            return jnp.sum(a, axis=0, keepdims=True) * (1.0 / D)

        def x_rows(lo, n, tile):
            col = pl.ds(pl.multiple_of(tile * LANES, LANES), LANES)
            return xT_v[pl.ds(lo, n), col].astype(F32)

        def stat_pieces(load_a, load_b, st):
            def sum_piece(lo):
                def run():
                    part = fold(load_a(lo, FC))
                    st['s'] = part if lo == 0 else st['s'] + part
                    if lo + FC == D:
                        st['mu'] = total(st['s'])
                return run

            def var_piece(lo):
                def run():
                    xc = load_b(lo, FC) - st['mu']
                    part = fold(xc * xc)
                    st['q'] = part if lo == 0 else st['q'] + part
                    if lo + FC == D:
                        st['rstd'] = lax.rsqrt(total(st['q']) + EPS)
                return run
            return [sum_piece(lo) for lo in range(0, D, FC)] + [var_piece(lo) for lo in range(0, D, FC)]

        def ln1_pieces(tile, row_dst, raw=False):
            st = {}
            row = pl.ds(pl.multiple_of(row_dst, LANES), LANES)
            ld = lambda lo, n: x_rows(lo, n, tile)

            def apply_piece(lo):
                def run():
                    n = min(LANES, D - lo)
                    hn = ((ld(lo, n) - st['mu']) * st['rstd']).T
                    if raw:
                        s_s0[row, pl.ds(lo, n)] = hn
                    else:
                        hh = hn * modr_s[1, 0:1, pl.ds(lo, n)] + modr_s[0, 0:1, pl.ds(lo, n)]
                        h_s[row, pl.ds(lo, n)] = hh.astype(BF)
                return run
            return stat_pieces(ld, ld, st), [apply_piece(lo) for lo in range(0, D, LANES)]

        def ln2_pieces(tile, slot, half, acc_val=None, st=None, live=None):
            st = {} if st is None else st
            col = pl.ds(pl.multiple_of(tile * LANES, LANES), LANES)
            acol = pl.ds(half * LANES if isinstance(half, int) else pl.multiple_of(half * LANES, LANES), LANES)

            def load_a(lo, n):
                rows = pl.ds(lo, n)
                av = acc_s[slot, rows, acol] if acc_val is None else acc_val[lo:lo + n, :]
                dx = colf_s[0, rows, :] * av
                if live is not None:
                    dx = jnp.where(live, dx, 0.0)
                x2 = (x_rows(lo, n, tile) + dx).astype(BF)
                xT_v[rows, col] = x2
                return x2.astype(F32)

            def load_b(lo, n):
                return x_rows(lo, n, tile)

            def apply_piece(lo):
                def run():
                    rows = pl.ds(lo, FC)
                    x2 = load_b(lo, FC)
                    h2 = ((x2 - st['mu']) * st['rstd'] * colf_s[2, rows, :] + colf_s[1, rows, :]).astype(BF)
                    h2_s[rows, col] = h2
                    h2 = h2.astype(F32)
                    outT_v[rows, col] = (x2 + colf_s[3, rows, :] * h2).astype(BF)
                    if opts.get('rv', 1):
                        part = fold(h2 * colf_s[4, rows, :])
                        st['r'] = part if lo == 0 else st['r'] + part
                        if lo + FC == D:
                            r_s[tile] = jnp.broadcast_to(jnp.sum(st['r'], axis=0, keepdims=True), (8, LANES))
                return run
            sp = stat_pieces(load_a, load_b, st)
            if acc_val is not None:
                run_all(sp[:D // FC])
                sp = sp[D // FC:]
            return sp + [apply_piece(lo) for lo in range(0, D, FC)]

        def interleave(a, b):
            return [f for pair_ in zip(a, b) for f in pair_]

        def run_all(pieces):
            for f in pieces:
                f()

        def anchor(v, z):
            xT_v[0:16, pl.ds(pl.multiple_of(S + z * LANES, LANES), LANES)] = v.astype(BF)
            colf_s[5 + z, 0:8, :] = v[0:8]

        def r_tile(tile):
            col = pl.multiple_of(tile * LANES, LANES)
            wr16 = jnp.broadcast_to(wr_v[...].reshape(1, D), (16, D))
            rr = jnp.dot(wr16, h2_s[:, pl.ds(col, LANES)], preferred_element_type=F32)
            r_s[tile] = rr[0:8, :]

        def step(ua, up, uo, par, extra=None, pieces=None, ck=None, nl_in=None, nl_out=None, o_sink=None,
                 o_init=False):
            pieces = list(pieces or [])
            nl_in = NL if nl_in is None else nl_in
            nl_out = NL if nl_out is None else nl_out
            CK = ck or (opts.get('ckp', 2048) if pieces else opts.get('cki', 2048))
            NC = SK // CK
            nslot = 2 * SK // 512
            slots = [i for i in range(nslot) if PH[i]]
            state = {'slot': 0}

            def place(v):
                for c0 in range(0, v.shape[1], 512):
                    ph = state['slot']
                    state['slot'] += 1
                    if not pieces or ph not in slots:
                        continue
                    left = len([q for q in slots if q >= ph])
                    npc = -(-len(pieces) // left)
                    mine = [pieces.pop(0) for _ in range(npc)]
                    for i, f in enumerate(mine):
                        r0 = ((i * R // len(mine)) // 16) * 16
                        anchor(v[r0:r0 + 16, c0:c0 + LANES], zero_s[0])
                        f()

            OP = opts.get('opos', 'start')
            st = {}

            def ldkv(ref, g, c):
                if opts.get('u32'):
                    return pltpu.bitcast(ref.bitcast(jnp.uint32)[g, pl.ds(c * (CK // 2), CK // 2), :], BF)
                return ref[g, pl.ds(c * CK, CK), :]

            def do_q():
                hslot, pa = ua
                hrow = pl.multiple_of(hslot * T, T)
                if opts.get('ksplit', 1):
                    k0 = (D // LANES) * LANES
                    qf = jnp.dot(h_s[pl.ds(hrow, T), pl.ds(k0, D - k0)], wq_v[pa, pl.ds(k0, D - k0), pl.ds(par * HD, HD)],
                                 preferred_element_type=F32)
                    qf = qf + jnp.dot(h_s[pl.ds(hrow, T), pl.ds(0, k0)], wq_v[pa, pl.ds(0, k0), pl.ds(par * HD, HD)],
                                      preferred_element_type=F32)
                    qf = qf * qscale
                else:
                    qf = jnp.dot(h_s[pl.ds(hrow, T), :], wq_v[pa, :, pl.ds(par * HD, HD)],
                                 preferred_element_type=F32) * qscale
                qb = qf.astype(BF)
                st['q2'] = jnp.concatenate([qb[:, r * DH:(r + 1) * DH] for r in range(REP)], axis=0)

            def do_o():
                aslot, po = uo
                if nl_in:
                    if nl_in == 1:
                        lsum = jnp.sum(l_s[par][...], axis=-1, keepdims=True)
                    else:
                        lsum = l_s[par][...]
                    ob = (of_s[par][...] * pltpu.reciprocal(lsum, approx=False, full_range=False)).astype(BF)
                    o2 = jnp.concatenate([ob[r * T:(r + 1) * T, :] for r in range(REP)], axis=1)
                else:
                    o2 = o_s[par][...]
                y = lax.dot_general(woT_v[po, :, pl.ds(par * HD, HD)], o2, NT,
                                    preferred_element_type=F32)
                if o_init is True:
                    acc_s[aslot] = y
                elif o_init is not None and o_init is not False:
                    acc_s[aslot] = jnp.where(o_init, 0.0, acc_s[aslot]) + y
                elif o_sink is None:
                    acc_s[aslot] = acc_s[aslot] + y
                else:
                    o_sink(acc_s[aslot] + y)

            def do_m():
                if opts.get('mend'):
                    st['mrow'] = m_s[1 - par][...]
                else:
                    st['mrow'] = jnp.max(m_s[1 - par][...], axis=-1, keepdims=True)

            def do_p(c):
                keys = pl.ds(c * CK, CK)
                sv = s_s[1 - par][:, keys]
                mrow = st['mrow']
                if opts.get('mend'):
                    mrow = jnp.concatenate([mrow] * (CK // LANES), axis=1)
                p = jnp.exp2(sv - mrow)
                ll = p[:, 0:LANES]
                for jj in range(1, CK // LANES):
                    ll = ll + p[:, jj * LANES:(jj + 1) * LANES]
                st['l'] = ll if c == 0 else st['l'] + ll
                o = jnp.dot(p.astype(BF), ldkv(v_v, up, c), preferred_element_type=F32)
                st['o'] = o if c == 0 else st['o'] + o
                place(p if opts.get('anchp', CK > 512) else o)

            def do_s(c):
                keys = pl.ds(c * CK, CK)
                s = lax.dot_general(st['q2'], ldkv(k_v, 2 * ua[1] + par, c), NT, preferred_element_type=F32)
                s_s[par][:, keys] = s
                mm = s[:, 0:LANES]
                for jj in range(1, CK // LANES):
                    mm = jnp.maximum(mm, s[:, jj * LANES:(jj + 1) * LANES])
                st['m'] = mm if c == 0 else jnp.maximum(st['m'], mm)
                place(s)

            def do_norm():
                if nl_out:
                    of_s[1 - par][...] = st['o']
                    if nl_out == 1:
                        l_s[1 - par][...] = st['l']
                    else:
                        l_s[1 - par][...] = jnp.broadcast_to(jnp.sum(st['l'], axis=-1, keepdims=True), (R, LANES))
                    return
                lsum = jnp.sum(st['l'], axis=-1, keepdims=True)
                ob = (st['o'] * pltpu.reciprocal(lsum, approx=False, full_range=False)).astype(BF)
                for r in range(REP):
                    o_s[1 - par][:, r * DH:(r + 1) * DH] = ob[r * T:(r + 1) * T, :]

            if OP == 'first' and uo is not None:
                do_o()
            if opts.get('mfirst', 1) and up is not None:
                do_m()
            if ua is not None:
                do_q()
            if OP == 'start' and uo is not None:
                do_o()
            if not opts.get('mfirst', 1) and up is not None:
                do_m()
            for c in range(NC):
                if opts.get('sfirst') and c > 0:
                    if ua is not None:
                        do_s(c - 1)
                if up is not None:
                    do_p(c)
                if not opts.get('sfirst') and ua is not None:
                    do_s(c)
                if OP == c and uo is not None:
                    do_o()
            if opts.get('sfirst'):
                if opts.get('normlast') and ua is not None:
                    do_s(NC - 1)
                if up is not None:
                    do_norm()
                if not opts.get('normlast') and ua is not None:
                    do_s(NC - 1)
            elif up is not None:
                do_norm()
            if OP == 'end' and uo is not None:
                do_o()
            if ua is not None:
                if opts.get('mend'):
                    m_s[par][...] = jnp.broadcast_to(jnp.max(st['m'], axis=-1, keepdims=True), (R, LANES))
                else:
                    m_s[par][...] = st['m']
            if extra is not None:
                extra()


        acc_s[1] = jnp.zeros((D, T), F32)
        colf_s[0:4] = jnp.zeros((4, D, LANES), F32)
        cp_c.wait()
        cp_wr.wait()
        cc = jnp.broadcast_to(c_v[...].astype(F32), (8, D))
        sc = (cc * jax.nn.sigmoid(cc)).astype(BF)
        colf_s[4] = jnp.broadcast_to(wr_v[...].reshape(1, D).astype(F32), (LANES, D)).T

        with scope('ln1_first'):
            cp_x0.wait()
            first_ln = [ln1_pieces(i, i * LANES, raw=True) for i in range(TPB)]
            run_all(interleave(first_ln[0][0], first_ln[1][0]))
            run_all(interleave(first_ln[0][1], first_ln[1][1]))
            cp_wm1.wait()
            mod1 = jnp.dot(sc, wm_v[:, pl.ds(0, 2 * D)], preferred_element_type=F32)
            sa = mod1[:, 0:D]
            ca1 = mod1[:, D:2 * D] + 1.0
            modr_s[0] = sa
            modr_s[1] = ca1
            h_s[0:T, :] = (s_s0[0:T, 0:D] * ca1[0:1, :] + sa[0:1, :]).astype(BF)

        in_own_block(lambda: [cp.start() for cp in (cp_x2, cp_wm2, cp_wg, cp_wu, cp_wd)])

        def pair_units(t, p):
            return ((t + (p >> LOG_NP)) & 1, p & (NP - 1)), (t & 1, p - 1)

        def pair(t, p, pieces=(None, None), extra=None, first=None):
            ua, uo = pair_units(t, p)
            step(ua, 2 * p - 1, uo, 0, pieces=pieces[0], o_init=first)
            step(ua, (2 * p) & (HKV - 1), uo, 1, pieces=pieces[1], extra=extra)

        def ln1_block(tsrc, tdst):
            la = [ln1_pieces(tsrc * TPB + i, (tdst & 1) * T + i * LANES) for i in range(TPB)]
            return interleave(la[0][0] + la[0][1], la[1][0] + la[1][1])

        with scope('fill'):
            cp_wq0[0].wait()
            cp_k0[0].wait()
            step((0, 0), None, None, 0)
            cp_wq0[1].wait()
            cp_k0[1].wait()
            cp_v0[0].wait()
            step((0, 0), 0, None, 1)
            ua, uo = pair_units(0, 1)
            for cp in (cp_wq0[2], cp_k0[2], cp_v0[1], cp_wo0[0]):
                cp.wait()
            step(ua, 1, uo, 0, o_init=True)
            for cp in (cp_x1, cp_wq0[3], cp_k0[3], cp_v0[2], cp_wo0[1]):
                cp.wait()
            step(ua, 2, uo, 1, pieces=ln1_block(1, 1))
            cp_v0[3].wait()

        def weight_waits(t, p):
            first = t == 0

            @pl.when(jnp.logical_and(first, p < NP))
            def _():
                cp_wq(p).wait()
                cp_k(p).wait()
                cp_v(p).wait()

            @pl.when(first)
            def _():
                cp_wo(p - 1).wait()

        def block(t, carry):
            last = (t == NB - 1).astype(jnp.int32)

            def loaded(i, carry2):
                weight_waits(t, i + 1)
                half = jnp.minimum(i, TPB - 1)
                live = jnp.logical_and(t > 0, i < TPB)
                p1 = sum(ln1_pieces(jnp.minimum(t + 1, NB - 1) * TPB + half, ((t + 1) & 1) * T + half * LANES), [])
                p2 = ln2_pieces(jnp.maximum(t - 1, 0) * TPB + half, (t + 1) & 1, half, live=live)
                pair(t, i + 1, pieces=(p1, p2), first=i == 0)
                return carry2

            with scope('loaded'):
                lax.fori_loop((t == 0).astype(jnp.int32), TPB + last, loaded, 0)

            @pl.when(t > 0)
            def _():
                cp_out(t - 1).start()

            def inner(b, carry2):
                p = 2 * b + TPB + 1 + last
                weight_waits(t, p)
                weight_waits(t, p + 1)
                pair(t, p)
                pair(t, p + 1)
                return carry2

            with scope('inner'):
                lax.fori_loop(0, (NP - TPB) // 2 - last, inner, 0)

            def mod_rest(i, carry2):
                cp_x2.wait()
                cp_wm2.wait()
                for k2 in range(4):
                    lo = (2 + k2) * D // LANES * LANES
                    hi = -(-((3 + k2) * D) // LANES) * LANES
                    row = jnp.dot(sc, wm_v[:, pl.ds(lo, hi - lo)], preferred_element_type=F32)[0:1, :]
                    if k2 == 2:
                        row = row + 1.0
                    off = (2 + k2) * D - lo
                    colf_s[k2] = jnp.broadcast_to(row, (LANES, hi - lo)).T[off:off + D, :]
                return carry2
            with scope('mod_rest'):
                lax.fori_loop(0, (t == 0).astype(jnp.int32), mod_rest, 0)
            return carry

        lax.fori_loop(0, NB, block, 0)
        if opts.get('dead'):
            def dead(i, c):
                for u in range(opts['dead']):
                    step(None, None, (0, i), u & 1) if opts.get('small') else step((0, i), 1, (0, i), u & 1)
                return c
            lax.fori_loop(0, zero_s[0], dead, 0)
        with scope('drain'):
            tl = NB - 1
            step(None, HKV - 1, ((NB - 1) % 2, NP - 1), 0, nl_out=0)
            sums = []

            def first_sweep(a):
                for i in range(TPB):
                    st = {}
                    st['rest'] = ln2_pieces(tl * TPB + i, None, i, a[:, i * LANES:(i + 1) * LANES], st)
                    sums.append(st)
            step(None, None, ((NB - 1) % 2, NP - 1), 1, nl_in=0, o_sink=first_sweep)

        with scope('ln2_tail'):
            if not opts.get('tloop', 1):
                run_all(interleave(sums[0]['rest'], sums[1]['rest']))
            else:
                TC = opts.get('tc', 96)
                cols_ = [pl.ds((tl * TPB + i) * LANES, LANES) for i in range(TPB)]
                mus = [st['mu'] for st in sums]

                def var_body(k, qs):
                    rows = pl.ds(pl.multiple_of(k * TC, TC), TC)
                    out = []
                    for i in range(TPB):
                        xc = xT_v[rows, cols_[i]].astype(F32) - mus[i]
                        out.append(qs[i] + fold(xc * xc))
                    return tuple(out)
                qs = lax.fori_loop(0, D // TC, var_body, (jnp.zeros((8, LANES), F32),) * TPB)
                rstds = [lax.rsqrt(total(q) + EPS) for q in qs]

                def apply_body(k, rs):
                    rows = pl.ds(pl.multiple_of(k * TC, TC), TC)
                    out = []
                    for i in range(TPB):
                        x2 = xT_v[rows, cols_[i]].astype(F32)
                        h2 = ((x2 - mus[i]) * rstds[i] * colf_s[2, rows, :] + colf_s[1, rows, :]).astype(BF)
                        h2_s[rows, cols_[i]] = h2
                        h2 = h2.astype(F32)
                        outT_v[rows, cols_[i]] = (x2 + colf_s[3, rows, :] * h2).astype(BF)
                        out.append(rs[i] + fold(h2 * colf_s[4, rows, :]))
                    return tuple(out)
                rs = lax.fori_loop(0, D // TC, apply_body, (jnp.zeros((8, LANES), F32),) * TPB)
                for i in range(TPB):
                    r_s[tl * TPB + i] = jnp.broadcast_to(jnp.sum(rs[i], axis=0, keepdims=True), (8, LANES))
            cp_out(tl).start()

        with scope('topk'):
            lane = lax.broadcasted_iota(jnp.int32, (8, LANES), 1)
            sub = lax.broadcasted_iota(jnp.int32, (8, LANES), 0)
            keys = []
            for i in range(NTILE):
                rv = r_s[i]
                tok = lane + i * LANES
                code = jnp.where(rv < 0.0, tok, (S - 1) - tok)
                mag = jnp.clip(jnp.abs(rv), 1.1754944e-38, 3.0e38)
                bits = (lax.bitcast_convert_type(mag, jnp.int32) & jnp.int32(-S)) | code
                kf = lax.bitcast_convert_type(bits, F32)
                keys.append(jnp.where(rv < 0.0, -kf, kf))
            keys0 = list(keys)
            msel = jnp.zeros((8, LANES), F32)
            for i in range(TOPC):
                tree = list(keys)
                while len(tree) > 1:
                    tree = [jnp.maximum(tree[2 * a], tree[2 * a + 1]) for a in range(len(tree) // 2)]
                mx = jnp.max(tree[0], axis=1, keepdims=True)
                msel = jnp.where(sub == i, mx, msel)
                if i + 1 < TOPC:
                    keys = [jnp.where(kk == mx, -jnp.inf, kk) for kk in keys]
            hot = [jnp.where(kk == msel, 1.0, 0.0) for kk in keys0]
            oht = jnp.concatenate(hot, axis=1).astype(BF)
            mbits = lax.bitcast_convert_type(msel, jnp.int32)
            rsel = lax.bitcast_convert_type(mbits & jnp.int32(-S), F32)[:, 0:1]
            code = mbits & jnp.int32(S - 1)
            tile_of = jnp.where(msel < 0.0, code, (S - 1) - code) // LANES
            for i in range(TOPC):
                flag_s[NTILE + i] = jnp.max(tile_of[i:i + 1, 0:1])
            for i in range(TOPC):
                fresh = jnp.int32(1)
                for j in range(i):
                    fresh = fresh & (flag_s[NTILE + j] != flag_s[NTILE + i]).astype(jnp.int32)
                flag_s[i] = fresh
            for i in range(NTILE):
                hot_s[i] = jnp.concatenate([hot[i], hot[i]], axis=0).astype(BF)[0:16]

        with scope('ffn'):
            xsel = lax.dot_general(oht, h2_s[...], NT, preferred_element_type=F32).astype(BF)
            cp_wg.wait()
            cp_wu.wait()
            cp_wd.wait()
            gg = jnp.dot(xsel, wg_v[...], preferred_element_type=F32)
            uu = jnp.dot(xsel, wu_v[...], preferred_element_type=F32)
            act = (gg * jax.nn.sigmoid(gg) * uu).astype(BF)
            yy = lax.dot_general(act, wdT_v[...], NT, preferred_element_type=F32)
            yy = yy * jax.nn.sigmoid(rsel)
            yT = yy.T.astype(BF)

        with scope('final'):
            for i in range(NB):
                cp_out(i).wait()
            yT2 = jnp.concatenate([yT, jnp.zeros_like(yT)], axis=1)

            for i in range(TOPC):
                @pl.when(flag_s[i] > 0)
                def _():
                    tile = flag_s[NTILE + i]
                    cs = pl.ds(pl.multiple_of(tile * LANES, LANES), LANES)
                    upd = jnp.dot(yT2, hot_s[tile], preferred_element_type=F32)
                    outT_v[:, cs] = (xT_v[:, cs].astype(F32)
                                     + colf_s[3] * (h2_s[:, cs].astype(F32) + upd)).astype(BF)
                    cp_fix(i, tile).start()
            for i in range(TOPC):
                @pl.when(flag_s[i] > 0)
                def _():
                    cp_fix(i, flag_s[NTILE + i]).wait()

    scratch = [
        pltpu.VMEM((D, S + LANES), BF),
        pltpu.VMEM((HKV, SK, DH), BF),
        pltpu.VMEM((HKV, SK, DH), BF),
        pltpu.VMEM((NP, D, 2 * HD), BF),
        pltpu.VMEM((NP, D, 2 * HD), BF),
        pltpu.VMEM((D, F), BF),
        pltpu.VMEM((D, F), BF),
        pltpu.VMEM((D, F), BF),
        pltpu.VMEM((D, 6 * D), BF),
        pltpu.VMEM((1, D), BF),
        pltpu.VMEM((D,), BF),
        pltpu.VMEM((2, 8, D), F32),
        pltpu.VMEM((6, D, LANES), F32),
        pltpu.VMEM((2 * T, D), BF),
        pltpu.VMEM((R, SK), F32),
        pltpu.VMEM((R, SK), F32),
        pltpu.VMEM((R, LANES), F32),
        pltpu.VMEM((R, LANES), F32),
        pltpu.VMEM((T, HD), BF),
        pltpu.VMEM((T, HD), BF),
        pltpu.VMEM((2, D, T), F32),
        pltpu.SMEM((1,), jnp.int32),
        pltpu.VMEM((D, S), BF),
        pltpu.VMEM((NTILE, 8, LANES), F32),
        pltpu.VMEM((D, S), BF),
        pltpu.SMEM((NTILE + TOPC,), jnp.int32),
        pltpu.VMEM((NTILE, 16, LANES), BF),
        pltpu.VMEM((R, LANES), F32), pltpu.VMEM((R, LANES), F32), pltpu.VMEM((R, LANES), F32), pltpu.VMEM((R, LANES), F32),
        pltpu.SemaphoreType.DMA((4, NP)),
        pltpu.SemaphoreType.DMA((4, 4)),
        pltpu.SemaphoreType.DMA((10,)),
        pltpu.SemaphoreType.DMA((NB + TOPC,)),
    ]
    anyspec = pl.BlockSpec(memory_space=pl.ANY)
    return pl.pallas_call(
        kernel,
        in_specs=[anyspec] * 11,
        out_specs=anyspec,
        out_shape=jax.ShapeDtypeStruct((D, S), BF),
        scratch_shapes=scratch,
        compiler_params=pltpu.CompilerParams(vmem_limit_bytes=opts.get('vmem', 110) * 1024 * 1024, flags=flags),
        name='adaln_gqa_moe',
        interpret=opts.get('interpret', False),
    )


def build_fn(T=256, CK=512, flags=None, **opts):
    def fn(A_x, A_k_cache, A_v_cache, A_wq, A_wo, B_x, B_w_r, B_w_gate, B_w_up, B_w_down, c, w_mod):
        B, S, D = A_x.shape
        _, HKV, SK, DH = A_k_cache.shape
        F = B_w_gate.shape[1]
        call = _build(S, SK, D, HKV, DH, F, T, CK, flags, opts)
        outT = call(
            A_x.reshape(S, D).T, A_k_cache.reshape(HKV, SK, DH), A_v_cache.reshape(HKV, SK, DH),
            A_wq, A_wo.T, B_w_r, B_w_gate, B_w_up, B_w_down.T, c, w_mod)
        return outT.T.reshape(B, S, D)
    return fn


_IMPL = build_fn(flags={"XLA_TPU_FORCE_LP_LLO_SCHEDULER": True}, )


@jax.jit
def pallas_adaLN_cond__gqa_block_cached__moe_arch_mod__prompt_kernel(
        A_x, A_k_cache, A_v_cache, A_wq, A_wo, B_x, B_w_r, B_w_gate, B_w_up, B_w_down, c, w_mod):
    return _IMPL(A_x, A_k_cache, A_v_cache, A_wq, A_wo, B_x, B_w_r, B_w_gate, B_w_up, B_w_down, c, w_mod)
```

```python
import functools

import jax
import jax.numpy as jnp
from jax import lax
import jax.experimental.pallas as pl
import jax.experimental.pallas.tpu as pltpu

BF = jnp.bfloat16
F32 = jnp.float32
NT = (((1,), (1,)), ((), ()))
LOG2E = 1.4426950408889634
EPS = 1e-5
TOPC = 8
LANES = 128


def _build(S, SK, D, HKV, DH, F, T, CK, flags, opts):
    REP = 2
    R = REP * T
    NB = S // T
    TPB = T // LANES
    NTILE = S // LANES
    NC = SK // CK
    HD = REP * DH
    NP = HKV // 2
    qscale = (DH ** -0.5) * LOG2E
    PH = opts.get('ph', [0, 0, 0, 0, 1, 1, 1, 0])
    NL = opts.get('nl', 0)
    FC = opts.get('fc', 48)
    assert HKV % 2 == 0 and TPB == 2 and D % FC == 0 and FC % 16 == 0 and NB >= 3
    assert S & (S - 1) == 0 and NP & (NP - 1) == 0
    LOG_NP = NP.bit_length() - 1

    def kernel(xT_hbm, k_hbm, v_hbm, wq_hbm, woT_hbm, wr_hbm, wg_hbm, wu_hbm, wdT_hbm, c_hbm, wm_hbm,
               outT_hbm,
               xT_v, k_v, v_v, wq_v, woT_v, wg_v, wu_v, wdT_v, wm_v, c_v, wr_v,
               modr_s, colf_s, h_s, s_s0, s_s1, m_s0, m_s1, o_s0, o_s1, acc_s, zero_s, h2_s, r_s,
               outT_v, flag_s, hot_s, of_s0, of_s1, l_s0, l_s1,
               sem_w, sem_first, sem_misc, sem_out):
        s_s = (s_s0, s_s1)
        m_s = (m_s0, m_s1)
        o_s = (o_s0, o_s1)
        of_s = (of_s0, of_s1)
        l_s = (l_s0, l_s1)
        if opts.get('prof'):
            scope = jax.named_scope
        else:
            import contextlib
            scope = lambda name: contextlib.nullcontext()

        def cp_wq(p):
            return pltpu.make_async_copy(wq_hbm.at[:, pl.ds(p * 2 * HD, 2 * HD)], wq_v.at[p], sem_w.at[0, p])

        def cp_k(p):
            return pltpu.make_async_copy(k_hbm.at[pl.ds(2 * p, 2)], k_v.at[pl.ds(2 * p, 2)], sem_w.at[1, p])

        def cp_v(p):
            return pltpu.make_async_copy(v_hbm.at[pl.ds(2 * p, 2)], v_v.at[pl.ds(2 * p, 2)], sem_w.at[2, p])

        def cp_wo(p):
            return pltpu.make_async_copy(woT_hbm.at[:, pl.ds(p * 2 * HD, 2 * HD)], woT_v.at[p], sem_w.at[3, p])

        def cols(src, dst, lo, n, sem):
            return pltpu.make_async_copy(src.at[:, pl.ds(lo, n)], dst.at[:, pl.ds(lo, n)], sem)

        def head(src, dst, g, sem):
            return pltpu.make_async_copy(src.at[pl.ds(g, 1)], dst.at[pl.ds(g, 1)], sem)

        def half(src, dst, g, sem):
            lo = (g % 2) * HD
            return pltpu.make_async_copy(src.at[:, pl.ds(g * HD, HD)], dst.at[g // 2, :, pl.ds(lo, HD)], sem)

        cp_wq0 = [half(wq_hbm, wq_v, g, sem_first.at[0, g]) for g in range(4)]
        cp_k0 = [head(k_hbm, k_v, g, sem_first.at[1, g]) for g in range(4)]
        cp_v0 = [head(v_hbm, v_v, g, sem_first.at[2, g]) for g in range(4)]
        cp_wo0 = [half(woT_hbm, woT_v, g, sem_first.at[3, g]) for g in range(2)]
        cp_wm1 = cols(wm_hbm, wm_v, 0, 2 * D, sem_misc.at[0])
        cp_wm2 = cols(wm_hbm, wm_v, 2 * D, 4 * D, sem_misc.at[1])
        cp_x0 = cols(xT_hbm, xT_v, 0, T, sem_misc.at[2])
        cp_x1 = cols(xT_hbm, xT_v, T, T, sem_misc.at[3])
        cp_x2 = cols(xT_hbm, xT_v, 2 * T, S - 2 * T, sem_misc.at[4])
        cp_wg = pltpu.make_async_copy(wg_hbm, wg_v, sem_misc.at[5])
        cp_wu = pltpu.make_async_copy(wu_hbm, wu_v, sem_misc.at[6])
        cp_wd = pltpu.make_async_copy(wdT_hbm, wdT_v, sem_misc.at[7])
        cp_c = pltpu.make_async_copy(c_hbm, c_v, sem_misc.at[8])
        cp_wr = pltpu.make_async_copy(wr_hbm, wr_v, sem_misc.at[9])

        def cp_out(t):
            cs = pl.ds(pl.multiple_of(t * T, T), T)
            return pltpu.make_async_copy(outT_v.at[:, cs], outT_hbm.at[:, cs], sem_out.at[t])

        def cp_fix(i, tile):
            cs = pl.ds(pl.multiple_of(tile * LANES, LANES), LANES)
            return pltpu.make_async_copy(outT_v.at[:, cs], outT_hbm.at[:, cs], sem_out.at[NB + i])

        def in_own_block(fn):
            def body(i, carry):
                fn()
                return carry
            lax.fori_loop(0, zero_s[0] + 1, body, 0)

        zero_s[0] = 0
        for cp in (cp_c, cp_wr, cp_x0, cp_wm1, cp_wq0[0], cp_k0[0]):
            cp.start()
        in_own_block(lambda: [cp.start() for cp in (cp_wq0[1], cp_k0[1], cp_v0[0])])
        in_own_block(lambda: [cp.start() for cp in (cp_wq0[2], cp_k0[2], cp_v0[1], cp_wo0[0])])
        in_own_block(lambda: [cp.start() for cp in (cp_x1, cp_wq0[3], cp_k0[3], cp_v0[2], cp_wo0[1], cp_v0[3])])

        def request_pairs():
            for p0 in range(2, NP):
                cp_wq(p0).start()
                cp_k(p0).start()
                cp_wo(p0 - 1).start()
                cp_v(p0).start()
            cp_wo(NP - 1).start()
        in_own_block(request_pairs)

        def fold(a):
            n = a.shape[0]
            while n > 8:
                if n % 16 == 0:
                    n //= 2
                    a = a[0:n] + a[n:2 * n]
                else:
                    r = a[0:8]
                    for i in range(1, n // 8):
                        r = r + a[8 * i:8 * i + 8]
                    a, n = r, 8
            return a

        def total(a):
            return jnp.sum(a, axis=0, keepdims=True) * (1.0 / D)

        def x_rows(lo, n, tile):
            col = pl.ds(pl.multiple_of(tile * LANES, LANES), LANES)
            return xT_v[pl.ds(lo, n), col].astype(F32)

        def stat_pieces(load_a, load_b, st):
            def sum_piece(lo):
                def run():
                    part = fold(load_a(lo, FC))
                    st['s'] = part if lo == 0 else st['s'] + part
                    if lo + FC == D:
                        st['mu'] = total(st['s'])
                return run

            def var_piece(lo):
                def run():
                    xc = load_b(lo, FC) - st['mu']
                    part = fold(xc * xc)
                    st['q'] = part if lo == 0 else st['q'] + part
                    if lo + FC == D:
                        st['rstd'] = lax.rsqrt(total(st['q']) + EPS)
                return run
            return [sum_piece(lo) for lo in range(0, D, FC)] + [var_piece(lo) for lo in range(0, D, FC)]

        def ln1_pieces(tile, row_dst, raw=False):
            st = {}
            row = pl.ds(pl.multiple_of(row_dst, LANES), LANES)
            ld = lambda lo, n: x_rows(lo, n, tile)

            def apply_piece(lo):
                def run():
                    n = min(LANES, D - lo)
                    hn = ((ld(lo, n) - st['mu']) * st['rstd']).T
                    if raw:
                        s_s0[row, pl.ds(lo, n)] = hn
                    else:
                        hh = hn * modr_s[1, 0:1, pl.ds(lo, n)] + modr_s[0, 0:1, pl.ds(lo, n)]
                        h_s[row, pl.ds(lo, n)] = hh.astype(BF)
                return run
            return stat_pieces(ld, ld, st), [apply_piece(lo) for lo in range(0, D, LANES)]

        def ln2_pieces(tile, slot, half, acc_val=None, st=None, live=None):
            st = {} if st is None else st
            col = pl.ds(pl.multiple_of(tile * LANES, LANES), LANES)
            acol = pl.ds(half * LANES if isinstance(half, int) else pl.multiple_of(half * LANES, LANES), LANES)

            def load_a(lo, n):
                rows = pl.ds(lo, n)
                av = acc_s[slot, rows, acol] if acc_val is None else acc_val[lo:lo + n, :]
                dx = colf_s[0, rows, :] * av
                if live is not None:
                    dx = jnp.where(live, dx, 0.0)
                x2 = (x_rows(lo, n, tile) + dx).astype(BF)
                xT_v[rows, col] = x2
                return x2.astype(F32)

            def load_b(lo, n):
                return x_rows(lo, n, tile)

            def apply_piece(lo):
                def run():
                    rows = pl.ds(lo, FC)
                    x2 = load_b(lo, FC)
                    h2 = ((x2 - st['mu']) * st['rstd'] * colf_s[2, rows, :] + colf_s[1, rows, :]).astype(BF)
                    h2_s[rows, col] = h2
                    h2 = h2.astype(F32)
                    outT_v[rows, col] = (x2 + colf_s[3, rows, :] * h2).astype(BF)
                    if opts.get('rv', 1):
                        part = fold(h2 * colf_s[4, rows, :])
                        st['r'] = part if lo == 0 else st['r'] + part
                        if lo + FC == D:
                            r_s[tile] = jnp.broadcast_to(jnp.sum(st['r'], axis=0, keepdims=True), (8, LANES))
                return run
            sp = stat_pieces(load_a, load_b, st)
            if acc_val is not None:
                run_all(sp[:D // FC])
                sp = sp[D // FC:]
            return sp + [apply_piece(lo) for lo in range(0, D, FC)]

        def interleave(a, b):
            return [f for pair_ in zip(a, b) for f in pair_]

        def run_all(pieces):
            for f in pieces:
                f()

        def anchor(v, z):
            xT_v[0:16, pl.ds(pl.multiple_of(S + z * LANES, LANES), LANES)] = v.astype(BF)
            colf_s[5 + z, 0:8, :] = v[0:8]

        def r_tile(tile):
            col = pl.multiple_of(tile * LANES, LANES)
            wr16 = jnp.broadcast_to(wr_v[...].reshape(1, D), (16, D))
            rr = jnp.dot(wr16, h2_s[:, pl.ds(col, LANES)], preferred_element_type=F32)
            r_s[tile] = rr[0:8, :]

        def step(ua, up, uo, par, extra=None, pieces=None, ck=None, nl_in=None, nl_out=None, o_sink=None,
                 o_init=False):
            pieces = list(pieces or [])
            nl_in = NL if nl_in is None else nl_in
            nl_out = NL if nl_out is None else nl_out
            CK = ck or (opts.get('ckp', 2048) if pieces else opts.get('cki', 2048))
            NC = SK // CK
            nslot = 2 * SK // 512
            slots = [i for i in range(nslot) if PH[i]]
            state = {'slot': 0}

            def place(v):
                for c0 in range(0, v.shape[1], 512):
                    ph = state['slot']
                    state['slot'] += 1
                    if not pieces or ph not in slots:
                        continue
                    left = len([q for q in slots if q >= ph])
                    npc = -(-len(pieces) // left)
                    mine = [pieces.pop(0) for _ in range(npc)]
                    for i, f in enumerate(mine):
                        r0 = ((i * R // len(mine)) // 16) * 16
                        anchor(v[r0:r0 + 16, c0:c0 + LANES], zero_s[0])
                        f()

            OP = opts.get('opos', 'start')
            st = {}

            def ldkv(ref, g, c):
                if opts.get('u32'):
                    return pltpu.bitcast(ref.bitcast(jnp.uint32)[g, pl.ds(c * (CK // 2), CK // 2), :], BF)
                return ref[g, pl.ds(c * CK, CK), :]

            def do_q():
                hslot, pa = ua
                hrow = pl.multiple_of(hslot * T, T)
                if opts.get('ksplit', 1):
                    k0 = (D // LANES) * LANES
                    qf = jnp.dot(h_s[pl.ds(hrow, T), pl.ds(k0, D - k0)], wq_v[pa, pl.ds(k0, D - k0), pl.ds(par * HD, HD)],
                                 preferred_element_type=F32)
                    qf = qf + jnp.dot(h_s[pl.ds(hrow, T), pl.ds(0, k0)], wq_v[pa, pl.ds(0, k0), pl.ds(par * HD, HD)],
                                      preferred_element_type=F32)
                    qf = qf * qscale
                else:
                    qf = jnp.dot(h_s[pl.ds(hrow, T), :], wq_v[pa, :, pl.ds(par * HD, HD)],
                                 preferred_element_type=F32) * qscale
                qb = qf.astype(BF)
                st['q2'] = jnp.concatenate([qb[:, r * DH:(r + 1) * DH] for r in range(REP)], axis=0)

            def do_o():
                aslot, po = uo
                if nl_in:
                    if nl_in == 1:
                        lsum = jnp.sum(l_s[par][...], axis=-1, keepdims=True)
                    else:
                        lsum = l_s[par][...]
                    ob = (of_s[par][...] * pltpu.reciprocal(lsum, approx=False, full_range=False)).astype(BF)
                    o2 = jnp.concatenate([ob[r * T:(r + 1) * T, :] for r in range(REP)], axis=1)
                else:
                    o2 = o_s[par][...]
                y = lax.dot_general(woT_v[po, :, pl.ds(par * HD, HD)], o2, NT,
                                    preferred_element_type=F32)
                if o_init is True:
                    acc_s[aslot] = y
                elif o_init is not None and o_init is not False:
                    acc_s[aslot] = jnp.where(o_init, 0.0, acc_s[aslot]) + y
                elif o_sink is None:
                    acc_s[aslot] = acc_s[aslot] + y
                else:
                    o_sink(acc_s[aslot] + y)

            def do_m():
                if opts.get('mend'):
                    st['mrow'] = m_s[1 - par][...]
                else:
                    st['mrow'] = jnp.max(m_s[1 - par][...], axis=-1, keepdims=True)

            def do_p(c):
                keys = pl.ds(c * CK, CK)
                sv = s_s[1 - par][:, keys]
                mrow = st['mrow']
                if opts.get('mend'):
                    mrow = jnp.concatenate([mrow] * (CK // LANES), axis=1)
                p = jnp.exp2(sv - mrow)
                ll = p[:, 0:LANES]
                for jj in range(1, CK // LANES):
                    ll = ll + p[:, jj * LANES:(jj + 1) * LANES]
                st['l'] = ll if c == 0 else st['l'] + ll
                o = jnp.dot(p.astype(BF), ldkv(v_v, up, c), preferred_element_type=F32)
                st['o'] = o if c == 0 else st['o'] + o
                place(p if opts.get('anchp', CK > 512) else o)

            def do_s(c):
                keys = pl.ds(c * CK, CK)
                s = lax.dot_general(st['q2'], ldkv(k_v, 2 * ua[1] + par, c), NT, preferred_element_type=F32)
                s_s[par][:, keys] = s
                mm = s[:, 0:LANES]
                for jj in range(1, CK // LANES):
                    mm = jnp.maximum(mm, s[:, jj * LANES:(jj + 1) * LANES])
                st['m'] = mm if c == 0 else jnp.maximum(st['m'], mm)
                place(s)

            def do_norm():
                if nl_out:
                    of_s[1 - par][...] = st['o']
                    if nl_out == 1:
                        l_s[1 - par][...] = st['l']
                    else:
                        l_s[1 - par][...] = jnp.broadcast_to(jnp.sum(st['l'], axis=-1, keepdims=True), (R, LANES))
                    return
                lsum = jnp.sum(st['l'], axis=-1, keepdims=True)
                ob = (st['o'] * pltpu.reciprocal(lsum, approx=False, full_range=False)).astype(BF)
                for r in range(REP):
                    o_s[1 - par][:, r * DH:(r + 1) * DH] = ob[r * T:(r + 1) * T, :]

            if OP == 'first' and uo is not None:
                do_o()
            if opts.get('mfirst', 1) and up is not None:
                do_m()
            if ua is not None:
                do_q()
            if OP == 'start' and uo is not None:
                do_o()
            if not opts.get('mfirst', 1) and up is not None:
                do_m()
            for c in range(NC):
                if opts.get('sfirst') and c > 0:
                    if ua is not None:
                        do_s(c - 1)
                if up is not None:
                    do_p(c)
                if not opts.get('sfirst') and ua is not None:
                    do_s(c)
                if OP == c and uo is not None:
                    do_o()
            if opts.get('sfirst'):
                if opts.get('normlast') and ua is not None:
                    do_s(NC - 1)
                if up is not None:
                    do_norm()
                if not opts.get('normlast') and ua is not None:
                    do_s(NC - 1)
            elif up is not None:
                do_norm()
            if OP == 'end' and uo is not None:
                do_o()
            if ua is not None:
                if opts.get('mend'):
                    m_s[par][...] = jnp.broadcast_to(jnp.max(st['m'], axis=-1, keepdims=True), (R, LANES))
                else:
                    m_s[par][...] = st['m']
            if extra is not None:
                extra()


        acc_s[1] = jnp.zeros((D, T), F32)
        colf_s[0:4] = jnp.zeros((4, D, LANES), F32)
        cp_c.wait()
        cp_wr.wait()
        cc = jnp.broadcast_to(c_v[...].astype(F32), (8, D))
        sc = (cc * jax.nn.sigmoid(cc)).astype(BF)
        colf_s[4] = jnp.broadcast_to(wr_v[...].reshape(1, D).astype(F32), (LANES, D)).T

        with scope('ln1_first'):
            cp_x0.wait()
            first_ln = [ln1_pieces(i, i * LANES, raw=True) for i in range(TPB)]
            run_all(interleave(first_ln[0][0], first_ln[1][0]))
            run_all(interleave(first_ln[0][1], first_ln[1][1]))
            cp_wm1.wait()
            mod1 = jnp.dot(sc, wm_v[:, pl.ds(0, 2 * D)], preferred_element_type=F32)
            sa = mod1[:, 0:D]
            ca1 = mod1[:, D:2 * D] + 1.0
            modr_s[0] = sa
            modr_s[1] = ca1
            h_s[0:T, :] = (s_s0[0:T, 0:D] * ca1[0:1, :] + sa[0:1, :]).astype(BF)

        in_own_block(lambda: [cp.start() for cp in (cp_x2, cp_wm2, cp_wg, cp_wu, cp_wd)])

        def pair_units(t, p):
            return ((t + (p >> LOG_NP)) & 1, p & (NP - 1)), (t & 1, p - 1)

        def pair(t, p, pieces=(None, None), extra=None, first=None):
            ua, uo = pair_units(t, p)
            step(ua, 2 * p - 1, uo, 0, pieces=pieces[0], o_init=first)
            step(ua, (2 * p) & (HKV - 1), uo, 1, pieces=pieces[1], extra=extra)

        def ln1_block(tsrc, tdst):
            la = [ln1_pieces(tsrc * TPB + i, (tdst & 1) * T + i * LANES) for i in range(TPB)]
            return interleave(la[0][0] + la[0][1], la[1][0] + la[1][1])

        with scope('fill'):
            cp_wq0[0].wait()
            cp_k0[0].wait()
            step((0, 0), None, None, 0)
            cp_wq0[1].wait()
            cp_k0[1].wait()
            cp_v0[0].wait()
            step((0, 0), 0, None, 1)
            ua, uo = pair_units(0, 1)
            for cp in (cp_wq0[2], cp_k0[2], cp_v0[1], cp_wo0[0]):
                cp.wait()
            step(ua, 1, uo, 0, o_init=True)
            for cp in (cp_x1, cp_wq0[3], cp_k0[3], cp_v0[2], cp_wo0[1]):
                cp.wait()
            step(ua, 2, uo, 1, pieces=ln1_block(1, 1))
            cp_v0[3].wait()

        def weight_waits(t, p, n):
            def run(q, carry):
                @pl.when(q < NP)
                def _():
                    cp_wq(q).wait()
                    cp_k(q).wait()
                    cp_v(q).wait()
                cp_wo(q - 1).wait()
                return carry
            lax.fori_loop(p, jnp.where(t == 0, p + n, p), run, 0)

        def block(t, carry):
            last = (t == NB - 1).astype(jnp.int32)

            def loaded(i, carry2):
                weight_waits(t, i + 1, 1)
                half = jnp.minimum(i, TPB - 1)
                live = jnp.logical_and(t > 0, i < TPB)
                p1 = sum(ln1_pieces(jnp.minimum(t + 1, NB - 1) * TPB + half, ((t + 1) & 1) * T + half * LANES), [])
                p2 = ln2_pieces(jnp.maximum(t - 1, 0) * TPB + half, (t + 1) & 1, half, live=live)
                pair(t, i + 1, pieces=(p1, p2), first=i == 0)
                return carry2

            with scope('loaded'):
                lax.fori_loop((t == 0).astype(jnp.int32), TPB + last, loaded, 0)

            @pl.when(t > 0)
            def _():
                cp_out(t - 1).start()

            def inner(b, carry2):
                p = 2 * b + TPB + 1 + last
                weight_waits(t, p, 2)
                pair(t, p)
                pair(t, p + 1)
                return carry2

            with scope('inner'):
                lax.fori_loop(0, (NP - TPB) // 2 - last, inner, 0)

            def mod_rest(i, carry2):
                cp_x2.wait()
                cp_wm2.wait()
                for k2 in range(4):
                    lo = (2 + k2) * D // LANES * LANES
                    hi = -(-((3 + k2) * D) // LANES) * LANES
                    row = jnp.dot(sc, wm_v[:, pl.ds(lo, hi - lo)], preferred_element_type=F32)[0:1, :]
                    if k2 == 2:
                        row = row + 1.0
                    off = (2 + k2) * D - lo
                    colf_s[k2] = jnp.broadcast_to(row, (LANES, hi - lo)).T[off:off + D, :]
                return carry2
            with scope('mod_rest'):
                lax.fori_loop(0, (t == 0).astype(jnp.int32), mod_rest, 0)
            return carry

        lax.fori_loop(0, NB, block, 0)
        if opts.get('dead'):
            def dead(i, c):
                for u in range(opts['dead']):
                    step(None, None, (0, i), u & 1) if opts.get('small') else step((0, i), 1, (0, i), u & 1)
                return c
            lax.fori_loop(0, zero_s[0], dead, 0)
        with scope('drain'):
            tl = NB - 1
            step(None, HKV - 1, ((NB - 1) % 2, NP - 1), 0, nl_out=0)
            sums = []

            def first_sweep(a):
                for i in range(TPB):
                    st = {}
                    st['rest'] = ln2_pieces(tl * TPB + i, None, i, a[:, i * LANES:(i + 1) * LANES], st)
                    sums.append(st)
            step(None, None, ((NB - 1) % 2, NP - 1), 1, nl_in=0, o_sink=first_sweep)

        with scope('ln2_tail'):
            if not opts.get('tloop', 1):
                run_all(interleave(sums[0]['rest'], sums[1]['rest']))
            else:
                TC = opts.get('tc', 96)
                cols_ = [pl.ds((tl * TPB + i) * LANES, LANES) for i in range(TPB)]
                mus = [st['mu'] for st in sums]

                def var_body(k, qs):
                    rows = pl.ds(pl.multiple_of(k * TC, TC), TC)
                    out = []
                    for i in range(TPB):
                        xc = xT_v[rows, cols_[i]].astype(F32) - mus[i]
                        out.append(qs[i] + fold(xc * xc))
                    return tuple(out)
                qs = lax.fori_loop(0, D // TC, var_body, (jnp.zeros((8, LANES), F32),) * TPB)
                rstds = [lax.rsqrt(total(q) + EPS) for q in qs]

                def apply_body(k, rs):
                    rows = pl.ds(pl.multiple_of(k * TC, TC), TC)
                    out = []
                    for i in range(TPB):
                        x2 = xT_v[rows, cols_[i]].astype(F32)
                        h2 = ((x2 - mus[i]) * rstds[i] * colf_s[2, rows, :] + colf_s[1, rows, :]).astype(BF)
                        h2_s[rows, cols_[i]] = h2
                        h2 = h2.astype(F32)
                        outT_v[rows, cols_[i]] = (x2 + colf_s[3, rows, :] * h2).astype(BF)
                        out.append(rs[i] + fold(h2 * colf_s[4, rows, :]))
                    return tuple(out)
                rs = lax.fori_loop(0, D // TC, apply_body, (jnp.zeros((8, LANES), F32),) * TPB)
                for i in range(TPB):
                    r_s[tl * TPB + i] = jnp.broadcast_to(jnp.sum(rs[i], axis=0, keepdims=True), (8, LANES))
            cp_out(tl).start()

        with scope('topk'):
            lane = lax.broadcasted_iota(jnp.int32, (8, LANES), 1)
            sub = lax.broadcasted_iota(jnp.int32, (8, LANES), 0)
            keys = []
            for i in range(NTILE):
                rv = r_s[i]
                tok = lane + i * LANES
                code = jnp.where(rv < 0.0, tok, (S - 1) - tok)
                mag = jnp.clip(jnp.abs(rv), 1.1754944e-38, 3.0e38)
                bits = (lax.bitcast_convert_type(mag, jnp.int32) & jnp.int32(-S)) | code
                kf = lax.bitcast_convert_type(bits, F32)
                keys.append(jnp.where(rv < 0.0, -kf, kf))
            keys0 = list(keys)
            msel = jnp.zeros((8, LANES), F32)
            for i in range(TOPC):
                tree = list(keys)
                while len(tree) > 1:
                    tree = [jnp.maximum(tree[2 * a], tree[2 * a + 1]) for a in range(len(tree) // 2)]
                mx = jnp.max(tree[0], axis=1, keepdims=True)
                msel = jnp.where(sub == i, mx, msel)
                if i + 1 < TOPC:
                    keys = [jnp.where(kk == mx, -jnp.inf, kk) for kk in keys]
            hot = [jnp.where(kk == msel, 1.0, 0.0) for kk in keys0]
            oht = jnp.concatenate(hot, axis=1).astype(BF)
            mbits = lax.bitcast_convert_type(msel, jnp.int32)
            rsel = lax.bitcast_convert_type(mbits & jnp.int32(-S), F32)[:, 0:1]
            code = mbits & jnp.int32(S - 1)
            tile_of = jnp.where(msel < 0.0, code, (S - 1) - code) // LANES
            for i in range(TOPC):
                flag_s[NTILE + i] = jnp.max(tile_of[i:i + 1, 0:1])
            for i in range(TOPC):
                fresh = jnp.int32(1)
                for j in range(i):
                    fresh = fresh & (flag_s[NTILE + j] != flag_s[NTILE + i]).astype(jnp.int32)
                flag_s[i] = fresh
            for i in range(NTILE):
                hot_s[i] = jnp.concatenate([hot[i], jnp.zeros_like(hot[i])], axis=0).astype(BF)

        with scope('ffn'):
            if opts.get('sg', 1):
                row16 = lax.broadcasted_iota(jnp.int32, (16, LANES), 0)
                xsel = None
                for i in range(TOPC):
                    tile = flag_s[NTILE + i]
                    cs = pl.ds(pl.multiple_of(tile * LANES, LANES), LANES)
                    one = jnp.where(row16 == i, hot_s[tile], jnp.zeros((16, LANES), BF))
                    part = lax.dot_general(one, h2_s[:, cs], NT, preferred_element_type=F32)
                    xsel = part if xsel is None else xsel + part
                xsel = xsel.astype(BF)
            else:
                xsel = lax.dot_general(oht, h2_s[...], NT, preferred_element_type=F32).astype(BF)
            cp_wg.wait()
            cp_wu.wait()
            cp_wd.wait()
            gg = jnp.dot(xsel, wg_v[...], preferred_element_type=F32)
            uu = jnp.dot(xsel, wu_v[...], preferred_element_type=F32)
            act = (gg * jax.nn.sigmoid(gg) * uu).astype(BF)
            yy = lax.dot_general(act, wdT_v[...], NT, preferred_element_type=F32)
            yy = yy[0:8] * jax.nn.sigmoid(rsel)
            yT = yy.T.astype(BF)

        with scope('final'):
            for i in range(NB):
                cp_out(i).wait()
            yT2 = jnp.concatenate([yT, jnp.zeros_like(yT)], axis=1)

            for i in range(TOPC):
                @pl.when(flag_s[i] > 0)
                def _():
                    tile = flag_s[NTILE + i]
                    cs = pl.ds(pl.multiple_of(tile * LANES, LANES), LANES)
                    upd = jnp.dot(yT2, hot_s[tile], preferred_element_type=F32)
                    outT_v[:, cs] = (xT_v[:, cs].astype(F32)
                                     + colf_s[3] * (h2_s[:, cs].astype(F32) + upd)).astype(BF)
                    cp_fix(i, tile).start()
            for i in range(TOPC):
                @pl.when(flag_s[i] > 0)
                def _():
                    cp_fix(i, flag_s[NTILE + i]).wait()

    scratch = [
        pltpu.VMEM((D, S + LANES), BF),
        pltpu.VMEM((HKV, SK, DH), BF),
        pltpu.VMEM((HKV, SK, DH), BF),
        pltpu.VMEM((NP, D, 2 * HD), BF),
        pltpu.VMEM((NP, D, 2 * HD), BF),
        pltpu.VMEM((D, F), BF),
        pltpu.VMEM((D, F), BF),
        pltpu.VMEM((D, F), BF),
        pltpu.VMEM((D, 6 * D), BF),
        pltpu.VMEM((1, D), BF),
        pltpu.VMEM((D,), BF),
        pltpu.VMEM((2, 8, D), F32),
        pltpu.VMEM((6, D, LANES), F32),
        pltpu.VMEM((2 * T, D), BF),
        pltpu.VMEM((R, SK), F32),
        pltpu.VMEM((R, SK), F32),
        pltpu.VMEM((R, LANES), F32),
        pltpu.VMEM((R, LANES), F32),
        pltpu.VMEM((T, HD), BF),
        pltpu.VMEM((T, HD), BF),
        pltpu.VMEM((2, D, T), F32),
        pltpu.SMEM((1,), jnp.int32),
        pltpu.VMEM((D, S), BF),
        pltpu.VMEM((NTILE, 8, LANES), F32),
        pltpu.VMEM((D, S), BF),
        pltpu.SMEM((NTILE + TOPC,), jnp.int32),
        pltpu.VMEM((NTILE, 16, LANES), BF),
        pltpu.VMEM((R, LANES), F32), pltpu.VMEM((R, LANES), F32), pltpu.VMEM((R, LANES), F32), pltpu.VMEM((R, LANES), F32),
        pltpu.SemaphoreType.DMA((4, NP)),
        pltpu.SemaphoreType.DMA((4, 4)),
        pltpu.SemaphoreType.DMA((10,)),
        pltpu.SemaphoreType.DMA((NB + TOPC,)),
    ]
    anyspec = pl.BlockSpec(memory_space=pl.ANY)
    return pl.pallas_call(
        kernel,
        in_specs=[anyspec] * 11,
        out_specs=anyspec,
        out_shape=jax.ShapeDtypeStruct((D, S), BF),
        scratch_shapes=scratch,
        compiler_params=pltpu.CompilerParams(vmem_limit_bytes=opts.get('vmem', 110) * 1024 * 1024, flags=flags),
        name='adaln_gqa_moe',
        interpret=opts.get('interpret', False),
    )


def build_fn(T=256, CK=512, flags=None, **opts):
    def fn(A_x, A_k_cache, A_v_cache, A_wq, A_wo, B_x, B_w_r, B_w_gate, B_w_up, B_w_down, c, w_mod):
        B, S, D = A_x.shape
        _, HKV, SK, DH = A_k_cache.shape
        F = B_w_gate.shape[1]
        call = _build(S, SK, D, HKV, DH, F, T, CK, flags, opts)
        outT = call(
            A_x.reshape(S, D).T, A_k_cache.reshape(HKV, SK, DH), A_v_cache.reshape(HKV, SK, DH),
            A_wq, A_wo.T, B_w_r, B_w_gate, B_w_up, B_w_down.T, c, w_mod)
        return outT.T.reshape(B, S, D)
    return fn


_IMPL = build_fn(flags={"XLA_TPU_FORCE_LP_LLO_SCHEDULER": True}, )


@jax.jit
def pallas_adaLN_cond__gqa_block_cached__moe_arch_mod__prompt_kernel(
        A_x, A_k_cache, A_v_cache, A_wq, A_wo, B_x, B_w_r, B_w_gate, B_w_up, B_w_down, c, w_mod):
    return _IMPL(A_x, A_k_cache, A_v_cache, A_wq, A_wo, B_x, B_w_r, B_w_gate, B_w_up, B_w_down, c, w_mod)
```

```python
import jax
import jax.numpy as jnp
from jax import lax
import jax.experimental.pallas as pl
import jax.experimental.pallas.tpu as pltpu

BF = jnp.bfloat16
F32 = jnp.float32
NT = (((1,), (1,)), ((), ()))
LOG2E = 1.4426950408889634
EPS = 1e-5
TOPC = 8
LANES = 128


def _build(S, SK, D, HKV, DH, F):
    REP = 2
    T = 256
    R = REP * T
    NB = S // T
    TPB = T // LANES
    NTILE = S // LANES
    HD = REP * DH
    NP = HKV // 2
    qscale = (DH ** -0.5) * LOG2E
    FC = 48
    assert HKV % 2 == 0 and TPB == 2 and D % FC == 0 and FC % 16 == 0 and NB >= 3
    assert S & (S - 1) == 0 and NP & (NP - 1) == 0
    LOG_NP = NP.bit_length() - 1

    def kernel(xT_hbm, k_hbm, v_hbm, wq_hbm, woT_hbm, wr_hbm, wg_hbm, wu_hbm, wdT_hbm, c_hbm, wm_hbm,
               outT_hbm,
               xT_v, k_v, v_v, wq_v, woT_v, wg_v, wu_v, wdT_v, wm_v, c_v, wr_v,
               modr_s, colf_s, h_s, s_s0, s_s1, m_s0, m_s1, o_s0, o_s1, acc_s, zero_s, h2_s, r_s,
               outT_v, flag_s, hot_s,
               sem_w, sem_first, sem_misc, sem_out):
        s_s = (s_s0, s_s1)
        m_s = (m_s0, m_s1)
        o_s = (o_s0, o_s1)

        def cp_wq(p):
            return pltpu.make_async_copy(wq_hbm.at[:, pl.ds(p * 2 * HD, 2 * HD)], wq_v.at[p], sem_w.at[0, p])

        def cp_k(p):
            return pltpu.make_async_copy(k_hbm.at[pl.ds(2 * p, 2)], k_v.at[pl.ds(2 * p, 2)], sem_w.at[1, p])

        def cp_v(p):
            return pltpu.make_async_copy(v_hbm.at[pl.ds(2 * p, 2)], v_v.at[pl.ds(2 * p, 2)], sem_w.at[2, p])

        def cp_wo(p):
            return pltpu.make_async_copy(woT_hbm.at[:, pl.ds(p * 2 * HD, 2 * HD)], woT_v.at[p], sem_w.at[3, p])

        def cols(src, dst, lo, n, sem):
            return pltpu.make_async_copy(src.at[:, pl.ds(lo, n)], dst.at[:, pl.ds(lo, n)], sem)

        def head(src, dst, g, sem):
            return pltpu.make_async_copy(src.at[pl.ds(g, 1)], dst.at[pl.ds(g, 1)], sem)

        def half(src, dst, g, sem):
            lo = (g % 2) * HD
            return pltpu.make_async_copy(src.at[:, pl.ds(g * HD, HD)], dst.at[g // 2, :, pl.ds(lo, HD)], sem)

        cp_wq0 = [half(wq_hbm, wq_v, g, sem_first.at[0, g]) for g in range(4)]
        cp_k0 = [head(k_hbm, k_v, g, sem_first.at[1, g]) for g in range(4)]
        cp_v0 = [head(v_hbm, v_v, g, sem_first.at[2, g]) for g in range(4)]
        cp_wo0 = [half(woT_hbm, woT_v, g, sem_first.at[3, g]) for g in range(2)]
        cp_wm1 = cols(wm_hbm, wm_v, 0, 2 * D, sem_misc.at[0])
        cp_wm2 = cols(wm_hbm, wm_v, 2 * D, 4 * D, sem_misc.at[1])
        cp_x0 = cols(xT_hbm, xT_v, 0, T, sem_misc.at[2])
        cp_x1 = cols(xT_hbm, xT_v, T, T, sem_misc.at[3])
        cp_x2 = cols(xT_hbm, xT_v, 2 * T, S - 2 * T, sem_misc.at[4])
        cp_wg = pltpu.make_async_copy(wg_hbm, wg_v, sem_misc.at[5])
        cp_wu = pltpu.make_async_copy(wu_hbm, wu_v, sem_misc.at[6])
        cp_wd = pltpu.make_async_copy(wdT_hbm, wdT_v, sem_misc.at[7])
        cp_c = pltpu.make_async_copy(c_hbm, c_v, sem_misc.at[8])
        cp_wr = pltpu.make_async_copy(wr_hbm, wr_v, sem_misc.at[9])

        def cp_out(t):
            cs = pl.ds(pl.multiple_of(t * T, T), T)
            return pltpu.make_async_copy(outT_v.at[:, cs], outT_hbm.at[:, cs], sem_out.at[t])

        def cp_fix(i, tile):
            cs = pl.ds(pl.multiple_of(tile * LANES, LANES), LANES)
            return pltpu.make_async_copy(outT_v.at[:, cs], outT_hbm.at[:, cs], sem_out.at[NB + i])

        def in_own_block(fn):
            def body(i, carry):
                fn()
                return carry
            lax.fori_loop(0, zero_s[0] + 1, body, 0)

        zero_s[0] = 0
        for cp in (cp_c, cp_wr, cp_x0, cp_wm1, cp_wq0[0], cp_k0[0]):
            cp.start()
        in_own_block(lambda: [cp.start() for cp in (cp_wq0[1], cp_k0[1], cp_v0[0])])
        in_own_block(lambda: [cp.start() for cp in (cp_wq0[2], cp_k0[2], cp_v0[1], cp_wo0[0])])
        in_own_block(lambda: [cp.start() for cp in (cp_x1, cp_wq0[3], cp_k0[3], cp_v0[2], cp_wo0[1], cp_v0[3])])

        def request_pairs():
            for p0 in range(2, NP):
                cp_wq(p0).start()
                cp_k(p0).start()
                cp_wo(p0 - 1).start()
                cp_v(p0).start()
            cp_wo(NP - 1).start()
        in_own_block(request_pairs)

        def fold(a):
            n = a.shape[0]
            while n > 8:
                if n % 16 == 0:
                    n //= 2
                    a = a[0:n] + a[n:2 * n]
                else:
                    r = a[0:8]
                    for i in range(1, n // 8):
                        r = r + a[8 * i:8 * i + 8]
                    a, n = r, 8
            return a

        def total(a):
            return jnp.sum(a, axis=0, keepdims=True) * (1.0 / D)

        def x_rows(lo, n, tile):
            col = pl.ds(pl.multiple_of(tile * LANES, LANES), LANES)
            return xT_v[pl.ds(lo, n), col].astype(F32)

        def stat_pieces(load_a, load_b, st):
            def sum_piece(lo):
                def run():
                    part = fold(load_a(lo, FC))
                    st['s'] = part if lo == 0 else st['s'] + part
                    if lo + FC == D:
                        st['mu'] = total(st['s'])
                return run

            def var_piece(lo):
                def run():
                    xc = load_b(lo, FC) - st['mu']
                    part = fold(xc * xc)
                    st['q'] = part if lo == 0 else st['q'] + part
                    if lo + FC == D:
                        st['rstd'] = lax.rsqrt(total(st['q']) + EPS)
                return run
            return [sum_piece(lo) for lo in range(0, D, FC)] + [var_piece(lo) for lo in range(0, D, FC)]

        def ln1_pieces(tile, row_dst, raw=False):
            st = {}
            row = pl.ds(pl.multiple_of(row_dst, LANES), LANES)
            ld = lambda lo, n: x_rows(lo, n, tile)

            def apply_piece(lo):
                def run():
                    n = min(LANES, D - lo)
                    hn = ((ld(lo, n) - st['mu']) * st['rstd']).T
                    if raw:
                        s_s0[row, pl.ds(lo, n)] = hn
                    else:
                        hh = hn * modr_s[1, 0:1, pl.ds(lo, n)] + modr_s[0, 0:1, pl.ds(lo, n)]
                        h_s[row, pl.ds(lo, n)] = hh.astype(BF)
                return run
            return stat_pieces(ld, ld, st), [apply_piece(lo) for lo in range(0, D, LANES)]

        def ln2_pieces(tile, slot, half, acc_val=None, st=None, live=None):
            st = {} if st is None else st
            col = pl.ds(pl.multiple_of(tile * LANES, LANES), LANES)
            acol = pl.ds(half * LANES if isinstance(half, int) else pl.multiple_of(half * LANES, LANES), LANES)

            def load_a(lo, n):
                rows = pl.ds(lo, n)
                av = acc_s[slot, rows, acol] if acc_val is None else acc_val[lo:lo + n, :]
                dx = colf_s[0, rows, :] * av
                if live is not None:
                    dx = jnp.where(live, dx, 0.0)
                x2 = (x_rows(lo, n, tile) + dx).astype(BF)
                xT_v[rows, col] = x2
                return x2.astype(F32)

            def load_b(lo, n):
                return x_rows(lo, n, tile)

            def apply_piece(lo):
                def run():
                    rows = pl.ds(lo, FC)
                    x2 = load_b(lo, FC)
                    h2 = ((x2 - st['mu']) * st['rstd'] * colf_s[2, rows, :] + colf_s[1, rows, :]).astype(BF)
                    h2_s[rows, col] = h2
                    h2 = h2.astype(F32)
                    outT_v[rows, col] = (x2 + colf_s[3, rows, :] * h2).astype(BF)
                    part = fold(h2 * colf_s[4, rows, :])
                    st['r'] = part if lo == 0 else st['r'] + part
                    if lo + FC == D:
                        r_s[tile] = jnp.broadcast_to(jnp.sum(st['r'], axis=0, keepdims=True), (8, LANES))
                return run
            sp = stat_pieces(load_a, load_b, st)
            if acc_val is not None:
                run_all(sp[:D // FC])
                sp = sp[D // FC:]
            return sp + [apply_piece(lo) for lo in range(0, D, FC)]

        def interleave(a, b):
            return [f for pair_ in zip(a, b) for f in pair_]

        def run_all(pieces):
            for f in pieces:
                f()

        def anchor(v, z):
            xT_v[0:16, pl.ds(pl.multiple_of(S + z * LANES, LANES), LANES)] = v.astype(BF)
            colf_s[5 + z, 0:8, :] = v[0:8]

        def step(ua, up, uo, par, pieces=None, o_init=False, o_sink=None):
            pieces = list(pieces or [])

            def place(s):
                rounds = SK // 512 - 1
                for rd in range(rounds):
                    npc = -(-len(pieces) // (rounds - rd))
                    mine = [pieces.pop(0) for _ in range(npc)]
                    for i, f in enumerate(mine):
                        r0 = ((i * R // len(mine)) // 16) * 16
                        anchor(s[r0:r0 + 16, rd * 512:rd * 512 + LANES], zero_s[0])
                        f()

            def chain(op, a):
                r = a[:, 0:LANES]
                for j in range(1, a.shape[1] // LANES):
                    r = op(r, a[:, j * LANES:(j + 1) * LANES])
                return r

            if up is not None:
                mrow = jnp.max(m_s[1 - par][...], axis=-1, keepdims=True)
            if ua is not None:
                hslot, pa = ua
                hrow = pl.ds(pl.multiple_of(hslot * T, T), T)
                hcol = pl.ds(par * HD, HD)
                k0 = (D // LANES) * LANES
                qf = jnp.dot(h_s[hrow, pl.ds(k0, D - k0)], wq_v[pa, pl.ds(k0, D - k0), hcol],
                             preferred_element_type=F32)
                qf = qf + jnp.dot(h_s[hrow, pl.ds(0, k0)], wq_v[pa, pl.ds(0, k0), hcol], preferred_element_type=F32)
                qb = (qf * qscale).astype(BF)
                q2 = jnp.concatenate([qb[:, r * DH:(r + 1) * DH] for r in range(REP)], axis=0)
            if uo is not None:
                aslot, po = uo
                y = lax.dot_general(woT_v[po, :, pl.ds(par * HD, HD)], o_s[par][...], NT,
                                    preferred_element_type=F32)
                if o_init is True:
                    acc_s[aslot] = y
                elif o_init is not False:
                    acc_s[aslot] = jnp.where(o_init, 0.0, acc_s[aslot]) + y
                elif o_sink is None:
                    acc_s[aslot] = acc_s[aslot] + y
                else:
                    o_sink(acc_s[aslot] + y)
            if up is not None:
                p = jnp.exp2(s_s[1 - par][...] - mrow)
                lsum = chain(jnp.add, p)
                o = jnp.dot(p.astype(BF), v_v[up], preferred_element_type=F32)
            if ua is not None:
                s = lax.dot_general(q2, k_v[2 * pa + par], NT, preferred_element_type=F32)
                s_s[par][...] = s
                mrun = chain(jnp.maximum, s)
                place(s)
            if up is not None:
                lsum = jnp.sum(lsum, axis=-1, keepdims=True)
                ob = (o * pltpu.reciprocal(lsum, approx=False, full_range=False)).astype(BF)
                for r in range(REP):
                    o_s[1 - par][:, r * DH:(r + 1) * DH] = ob[r * T:(r + 1) * T, :]
            if ua is not None:
                m_s[par][...] = mrun


        acc_s[1] = jnp.zeros((D, T), F32)
        colf_s[0:4] = jnp.zeros((4, D, LANES), F32)
        cp_c.wait()
        cp_wr.wait()
        cc = jnp.broadcast_to(c_v[...].astype(F32), (8, D))
        sc = (cc * jax.nn.sigmoid(cc)).astype(BF)
        colf_s[4] = jnp.broadcast_to(wr_v[...].reshape(1, D).astype(F32), (LANES, D)).T

        cp_x0.wait()
        first_ln = [ln1_pieces(i, i * LANES, raw=True) for i in range(TPB)]
        run_all(interleave(first_ln[0][0], first_ln[1][0]))
        run_all(interleave(first_ln[0][1], first_ln[1][1]))
        cp_wm1.wait()
        mod1 = jnp.dot(sc, wm_v[:, pl.ds(0, 2 * D)], preferred_element_type=F32)
        sa = mod1[:, 0:D]
        ca1 = mod1[:, D:2 * D] + 1.0
        modr_s[0] = sa
        modr_s[1] = ca1
        h_s[0:T, :] = (s_s0[0:T, 0:D] * ca1[0:1, :] + sa[0:1, :]).astype(BF)

        in_own_block(lambda: [cp.start() for cp in (cp_x2, cp_wm2, cp_wg, cp_wu, cp_wd)])

        def pair_units(t, p):
            return ((t + (p >> LOG_NP)) & 1, p & (NP - 1)), (t & 1, p - 1)

        def pair(t, p, pieces=(None, None), first=False):
            ua, uo = pair_units(t, p)
            step(ua, 2 * p - 1, uo, 0, pieces=pieces[0], o_init=first)
            step(ua, (2 * p) & (HKV - 1), uo, 1, pieces=pieces[1])

        def ln1_block(tsrc, tdst):
            la = [ln1_pieces(tsrc * TPB + i, (tdst & 1) * T + i * LANES) for i in range(TPB)]
            return interleave(la[0][0] + la[0][1], la[1][0] + la[1][1])

        cp_wq0[0].wait()
        cp_k0[0].wait()
        step((0, 0), None, None, 0)
        cp_wq0[1].wait()
        cp_k0[1].wait()
        cp_v0[0].wait()
        step((0, 0), 0, None, 1)
        ua, uo = pair_units(0, 1)
        for cp in (cp_wq0[2], cp_k0[2], cp_v0[1], cp_wo0[0]):
            cp.wait()
        step(ua, 1, uo, 0, o_init=True)
        for cp in (cp_x1, cp_wq0[3], cp_k0[3], cp_v0[2], cp_wo0[1]):
            cp.wait()
        step(ua, 2, uo, 1, pieces=ln1_block(1, 1))
        cp_v0[3].wait()

        def weight_waits(t, p, n):
            def run(q, carry):
                @pl.when(q < NP)
                def _():
                    cp_wq(q).wait()
                    cp_k(q).wait()
                    cp_v(q).wait()
                cp_wo(q - 1).wait()
                return carry
            lax.fori_loop(p, jnp.where(t == 0, p + n, p), run, 0)

        def block(t, carry):
            last = (t == NB - 1).astype(jnp.int32)

            def loaded(i, carry2):
                weight_waits(t, i + 1, 1)
                half = jnp.minimum(i, TPB - 1)
                live = jnp.logical_and(t > 0, i < TPB)
                p1 = sum(ln1_pieces(jnp.minimum(t + 1, NB - 1) * TPB + half, ((t + 1) & 1) * T + half * LANES), [])
                p2 = ln2_pieces(jnp.maximum(t - 1, 0) * TPB + half, (t + 1) & 1, half, live=live)
                pair(t, i + 1, pieces=(p1, p2), first=i == 0)
                return carry2

            lax.fori_loop((t == 0).astype(jnp.int32), TPB + last, loaded, 0)

            @pl.when(t > 0)
            def _():
                cp_out(t - 1).start()

            def inner(b, carry2):
                p = 2 * b + TPB + 1 + last
                weight_waits(t, p, 2)
                pair(t, p)
                pair(t, p + 1)
                return carry2

            lax.fori_loop(0, (NP - TPB) // 2 - last, inner, 0)

            def mod_rest(i, carry2):
                cp_x2.wait()
                cp_wm2.wait()
                for k2 in range(4):
                    lo = (2 + k2) * D // LANES * LANES
                    hi = -(-((3 + k2) * D) // LANES) * LANES
                    row = jnp.dot(sc, wm_v[:, pl.ds(lo, hi - lo)], preferred_element_type=F32)[0:1, :]
                    if k2 == 2:
                        row = row + 1.0
                    off = (2 + k2) * D - lo
                    colf_s[k2] = jnp.broadcast_to(row, (LANES, hi - lo)).T[off:off + D, :]
                return carry2
            lax.fori_loop(0, (t == 0).astype(jnp.int32), mod_rest, 0)
            return carry

        lax.fori_loop(0, NB, block, 0)
        tl = NB - 1
        step(None, HKV - 1, ((NB - 1) % 2, NP - 1), 0)
        sums = []

        def first_sweep(a):
            for i in range(TPB):
                st = {}
                ln2_pieces(tl * TPB + i, None, i, a[:, i * LANES:(i + 1) * LANES], st)
                sums.append(st)
        step(None, None, ((NB - 1) % 2, NP - 1), 1, o_sink=first_sweep)

        TC = 96
        cols_ = [pl.ds((tl * TPB + i) * LANES, LANES) for i in range(TPB)]
        mus = [st['mu'] for st in sums]

        def var_body(k, qs):
            rows = pl.ds(pl.multiple_of(k * TC, TC), TC)
            out = []
            for i in range(TPB):
                xc = xT_v[rows, cols_[i]].astype(F32) - mus[i]
                out.append(qs[i] + fold(xc * xc))
            return tuple(out)
        qs = lax.fori_loop(0, D // TC, var_body, (jnp.zeros((8, LANES), F32),) * TPB)
        rstds = [lax.rsqrt(total(q) + EPS) for q in qs]

        def apply_body(k, rs):
            rows = pl.ds(pl.multiple_of(k * TC, TC), TC)
            out = []
            for i in range(TPB):
                x2 = xT_v[rows, cols_[i]].astype(F32)
                h2 = ((x2 - mus[i]) * rstds[i] * colf_s[2, rows, :] + colf_s[1, rows, :]).astype(BF)
                h2_s[rows, cols_[i]] = h2
                h2 = h2.astype(F32)
                outT_v[rows, cols_[i]] = (x2 + colf_s[3, rows, :] * h2).astype(BF)
                out.append(rs[i] + fold(h2 * colf_s[4, rows, :]))
            return tuple(out)
        rs = lax.fori_loop(0, D // TC, apply_body, (jnp.zeros((8, LANES), F32),) * TPB)
        for i in range(TPB):
            r_s[tl * TPB + i] = jnp.broadcast_to(jnp.sum(rs[i], axis=0, keepdims=True), (8, LANES))
        cp_out(tl).start()

        lane = lax.broadcasted_iota(jnp.int32, (8, LANES), 1)
        sub = lax.broadcasted_iota(jnp.int32, (8, LANES), 0)
        keys = []
        for i in range(NTILE):
            rv = r_s[i]
            tok = lane + i * LANES
            code = jnp.where(rv < 0.0, tok, (S - 1) - tok)
            mag = jnp.clip(jnp.abs(rv), 1.1754944e-38, 3.0e38)
            bits = (lax.bitcast_convert_type(mag, jnp.int32) & jnp.int32(-S)) | code
            kf = lax.bitcast_convert_type(bits, F32)
            keys.append(jnp.where(rv < 0.0, -kf, kf))
        keys0 = list(keys)
        msel = jnp.zeros((8, LANES), F32)
        for i in range(TOPC):
            tree = list(keys)
            while len(tree) > 1:
                tree = [jnp.maximum(tree[2 * a], tree[2 * a + 1]) for a in range(len(tree) // 2)]
            mx = jnp.max(tree[0], axis=1, keepdims=True)
            msel = jnp.where(sub == i, mx, msel)
            if i + 1 < TOPC:
                keys = [jnp.where(kk == mx, -jnp.inf, kk) for kk in keys]
        hot = [jnp.where(kk == msel, 1.0, 0.0) for kk in keys0]
        mbits = lax.bitcast_convert_type(msel, jnp.int32)
        rsel = lax.bitcast_convert_type(mbits & jnp.int32(-S), F32)[:, 0:1]
        code = mbits & jnp.int32(S - 1)
        tile_of = jnp.where(msel < 0.0, code, (S - 1) - code) // LANES
        for i in range(TOPC):
            flag_s[NTILE + i] = jnp.max(tile_of[i:i + 1, 0:1])
        for i in range(TOPC):
            fresh = jnp.int32(1)
            for j in range(i):
                fresh = fresh & (flag_s[NTILE + j] != flag_s[NTILE + i]).astype(jnp.int32)
            flag_s[i] = fresh
        for i in range(NTILE):
            hot_s[i] = jnp.concatenate([hot[i], jnp.zeros_like(hot[i])], axis=0).astype(BF)

        row16 = lax.broadcasted_iota(jnp.int32, (16, LANES), 0)
        xsel = None
        for i in range(TOPC):
            tile = flag_s[NTILE + i]
            cs = pl.ds(pl.multiple_of(tile * LANES, LANES), LANES)
            one = jnp.where(row16 == i, hot_s[tile], jnp.zeros((16, LANES), BF))
            part = lax.dot_general(one, h2_s[:, cs], NT, preferred_element_type=F32)
            xsel = part if xsel is None else xsel + part
        xsel = xsel.astype(BF)
        cp_wg.wait()
        cp_wu.wait()
        cp_wd.wait()
        gg = jnp.dot(xsel, wg_v[...], preferred_element_type=F32)
        uu = jnp.dot(xsel, wu_v[...], preferred_element_type=F32)
        act = (gg * jax.nn.sigmoid(gg) * uu).astype(BF)
        yy = lax.dot_general(act, wdT_v[...], NT, preferred_element_type=F32)
        yy = yy[0:8] * jax.nn.sigmoid(rsel)
        yT = yy.T.astype(BF)

        for i in range(NB):
            cp_out(i).wait()
        yT2 = jnp.concatenate([yT, jnp.zeros_like(yT)], axis=1)

        for i in range(TOPC):
            @pl.when(flag_s[i] > 0)
            def _():
                tile = flag_s[NTILE + i]
                cs = pl.ds(pl.multiple_of(tile * LANES, LANES), LANES)
                upd = jnp.dot(yT2, hot_s[tile], preferred_element_type=F32)
                outT_v[:, cs] = (xT_v[:, cs].astype(F32)
                                 + colf_s[3] * (h2_s[:, cs].astype(F32) + upd)).astype(BF)
                cp_fix(i, tile).start()
        for i in range(TOPC):
            @pl.when(flag_s[i] > 0)
            def _():
                cp_fix(i, flag_s[NTILE + i]).wait()

    scratch = [
        pltpu.VMEM((D, S + LANES), BF),
        pltpu.VMEM((HKV, SK, DH), BF),
        pltpu.VMEM((HKV, SK, DH), BF),
        pltpu.VMEM((NP, D, 2 * HD), BF),
        pltpu.VMEM((NP, D, 2 * HD), BF),
        pltpu.VMEM((D, F), BF),
        pltpu.VMEM((D, F), BF),
        pltpu.VMEM((D, F), BF),
        pltpu.VMEM((D, 6 * D), BF),
        pltpu.VMEM((1, D), BF),
        pltpu.VMEM((D,), BF),
        pltpu.VMEM((2, 8, D), F32),
        pltpu.VMEM((6, D, LANES), F32),
        pltpu.VMEM((2 * T, D), BF),
        pltpu.VMEM((R, SK), F32),
        pltpu.VMEM((R, SK), F32),
        pltpu.VMEM((R, LANES), F32),
        pltpu.VMEM((R, LANES), F32),
        pltpu.VMEM((T, HD), BF),
        pltpu.VMEM((T, HD), BF),
        pltpu.VMEM((2, D, T), F32),
        pltpu.SMEM((1,), jnp.int32),
        pltpu.VMEM((D, S), BF),
        pltpu.VMEM((NTILE, 8, LANES), F32),
        pltpu.VMEM((D, S), BF),
        pltpu.SMEM((NTILE + TOPC,), jnp.int32),
        pltpu.VMEM((NTILE, 16, LANES), BF),
        pltpu.SemaphoreType.DMA((4, NP)),
        pltpu.SemaphoreType.DMA((4, 4)),
        pltpu.SemaphoreType.DMA((10,)),
        pltpu.SemaphoreType.DMA((NB + TOPC,)),
    ]
    anyspec = pl.BlockSpec(memory_space=pl.ANY)
    return pl.pallas_call(
        kernel,
        in_specs=[anyspec] * 11,
        out_specs=anyspec,
        out_shape=jax.ShapeDtypeStruct((D, S), BF),
        scratch_shapes=scratch,
        compiler_params=pltpu.CompilerParams(
            vmem_limit_bytes=110 * 1024 * 1024,
            flags={"XLA_TPU_FORCE_LP_LLO_SCHEDULER": True}),
        name='adaln_gqa_moe',
    )


@jax.jit
def pallas_adaLN_cond__gqa_block_cached__moe_arch_mod__prompt_kernel(
        A_x, A_k_cache, A_v_cache, A_wq, A_wo, B_x, B_w_r, B_w_gate, B_w_up, B_w_down, c, w_mod):
    del B_x
    B, S, D = A_x.shape
    _, HKV, SK, DH = A_k_cache.shape
    F = B_w_gate.shape[1]
    outT = _build(S, SK, D, HKV, DH, F)(
        A_x.reshape(S, D).T, A_k_cache.reshape(HKV, SK, DH), A_v_cache.reshape(HKV, SK, DH),
        A_wq, A_wo.T, B_w_r, B_w_gate, B_w_up, B_w_down.T, c, w_mod)
    return outT.T.reshape(B, S, D)
```
